```python
import jax
import jax.numpy as jnp

def _softmax(x, axis=-1):
    return jax.nn.softmax(x, axis=axis)

def _gelu(x):
    return jax.nn.gelu(x, approximate=True)

def _silu(x):
    return jax.nn.silu(x)

def _sigmoid(x):
    return jax.nn.sigmoid(x)

def _layernorm(x, axis=-1, eps=1e-05):
    m = jnp.mean(x, axis=axis, keepdims=True)
    v = jnp.var(x, axis=axis, keepdims=True)
    return (x - m) / jnp.sqrt(v + eps)

def _scatter_add(tgt, idx, src, axis=0):
    return tgt.at[idx].add(src)

def _segment_sum(src, seg, n):
    return jax.ops.segment_sum(src, seg, n)

class _Rng:

    def __init__(self, key):
        self._k = key

    def _next(self):
        self._k, sub = jax.random.split(self._k)
        return sub

    def normal(self, shape):
        return jax.random.normal(self._next(), shape, dtype=jnp.bfloat16)

    def randint(self, lo, hi, shape):
        return jax.random.randint(self._next(), shape, lo, hi, dtype=jnp.int32)

    def uniform(self, shape, lo=0.0, hi=1.0):
        return jax.random.uniform(self._next(), shape, jnp.bfloat16, lo, hi)

    def permutation(self, n):
        return jax.random.permutation(self._next(), n)
kernel_name = 'interleave_layers__linear_kernel_hedgehog__memory_aug_recurrent_mem_tr__prompt'

def setup_inputs():
    _rng = _Rng(jax.random.key(int.from_bytes(__import__("os").urandom(4), "little")))
    _w = lambda a: (lambda t: t.astype(jnp.bfloat16) if jnp.issubdtype(t.dtype, jnp.floating) else t)(jnp.asarray(a))

    def _A_setup():
        B, S, D, H = (1, 2048, 640, 32)
        Dh = D // H
        return {'x': _w((lambda *s: _rng.normal(s) * 0.05)(B, S, D)), 'wqkv': _w((lambda *s: _rng.normal(s) * 0.05)(D, 3 * D)), 'w_phi': _w((lambda *s: _rng.normal(s) * 0.05)(H, Dh, Dh) * Dh ** (-0.5)), 'wo': _w((lambda *s: _rng.normal(s) * 0.05)(D, D))}
    _A_in = _A_setup()

    def _B_setup():
        B, S, Dm = (1, 2048, 640)
        H, Dh = (32, 192)
        M, seg = (8, 32)
        seg = min(seg, S)
        S = S // seg * seg
        return {'x': _w((lambda *s: _rng.normal(s) * 0.05)(B, S, Dm)), 'mem0': _w((lambda *s: _rng.normal(s) * 0.05)(B, M, Dm)), 'Wq': _w((lambda *s: _rng.normal(s) * 0.05)(Dm, H, Dh) * Dm ** (-0.5)), 'Wk': _w((lambda *s: _rng.normal(s) * 0.05)(Dm, H, Dh) * Dm ** (-0.5)), 'Wv': _w((lambda *s: _rng.normal(s) * 0.05)(Dm, H, Dh) * Dm ** (-0.5)), 'Wo': _w((lambda *s: _rng.normal(s) * 0.05)(H, Dh, Dm) * (H * Dh) ** (-0.5)), 'seg_len': seg}
    _B_in = _B_setup()
    return {'A_x': _A_in['x'], 'A_wqkv': _A_in['wqkv'], 'A_w_phi': _A_in['w_phi'], 'A_wo': _A_in['wo'], 'B_x': _B_in['x'], 'B_mem0': _B_in['mem0'], 'B_Wq': _B_in['Wq'], 'B_Wk': _B_in['Wk'], 'B_Wv': _B_in['Wv'], 'B_Wo': _B_in['Wo'], 'B_seg_len': _B_in['seg_len']}

def reference(A_x, A_wqkv, A_w_phi, A_wo, B_x, B_mem0, B_Wq, B_Wk, B_Wv, B_Wo, B_seg_len):

    def _A_ref(x, wqkv, w_phi, wo):
        B, S, D = x.shape
        H = 32
        Dh = D // H
        qkv = (lambda x, *d: x.transpose(*d))((x @ wqkv).reshape(B, S, 3, H, Dh), 2, 0, 3, 1, 4)
        q, k, v = (qkv[0], qkv[1], qkv[2])
        pq = jnp.einsum('bhsd,hdf->bhsf', q, w_phi)
        pk = jnp.einsum('bhsd,hdf->bhsf', k, w_phi)
        phi_q = jnp.concatenate([_softmax(pq, axis=-1), _softmax(-pq, axis=-1)], axis=-1)
        phi_k = jnp.concatenate([_softmax(pk, axis=-1), _softmax(-pk, axis=-1)], axis=-1)
        kv = jnp.einsum('bhsf,bhsd->bhfd', phi_k, v)
        z = jnp.einsum('bhsf->bhf', phi_k)
        num = jnp.einsum('bhqf,bhfd->bhqd', phi_q, kv)
        den = jnp.einsum('bhqf,bhf->bhq', phi_q, z)[..., None] + 1e-06
        o = num / den
        return (lambda x, *d: x.transpose(*d))(o, 0, 2, 1, 3).reshape(B, S, D) @ wo

    def _B_ref(x, mem0, Wq, Wk, Wv, Wo, seg_len):
        B, S, Dm = x.shape
        H, Dh = (Wq.shape[1], Wq.shape[2])
        M = mem0.shape[1]
        scale = Dh ** (-0.5)
        n_seg = S // seg_len
        L = M + seg_len
        idx = jnp.arange(L)
        mask = (idx[:, None] < M) | (idx[:, None] >= idx[None, :])
        mem = mem0
        outs = []
        for s in range(n_seg):
            xs = x[:, s * seg_len:(s + 1) * seg_len, :].copy()
            h = jnp.concatenate([mem, xs], axis=1)
            q = jnp.einsum('btd,dhe->bhte', h, Wq)
            k = jnp.einsum('btd,dhe->bhte', h, Wk)
            v = jnp.einsum('btd,dhe->bhte', h, Wv)
            scores = jnp.einsum('bhqe,bhke->bhqk', q, k) * scale
            scores = jnp.where(mask[None, None], scores, -1000000000.0)
            p = _softmax(scores, axis=-1)
            o = jnp.einsum('bhqk,bhke->bhqe', p, v)
            o = jnp.einsum('bhte,hed->btd', o, Wo)
            mem = o[:, :M, :].copy()
            outs.append(o[:, M:, :])
        return jnp.concatenate(outs, axis=1)
    x = A_x
    x = x + _A_ref(_layernorm(x, axis=-1), A_wqkv, A_w_phi, A_wo)
    x = x + _B_ref(_layernorm(x, axis=-1), B_mem0, B_Wq, B_Wk, B_Wv, B_Wo, B_seg_len)
    x = x + _A_ref(_layernorm(x, axis=-1), A_wqkv, A_w_phi, A_wo)
    x = x + _B_ref(_layernorm(x, axis=-1), B_mem0, B_Wq, B_Wk, B_Wv, B_Wo, B_seg_len)
    return x
```

```python
import jax
import jax.numpy as jnp
from jax import lax
import jax.experimental.pallas as pl
import jax.experimental.pallas.tpu as pltpu

f32, bf16, u32, i32 = jnp.float32, jnp.bfloat16, jnp.uint32, jnp.int32

S, D = 2048, 640
HA, DA = 32, 20
NPA = HA // 2
RA = 2 * DA
GA = 4
TC = 256
NCH = S // TC
HB, DB, MEM, SEG = 32, 192, 8, 32
HD = HB * DB
L = MEM + SEG
NPB = HB // 2
PW = 2 * DB
SCALE = DB ** -0.5
TRC = 768

_NT = (((1,), (1,)), ((), ()))


def _dot(a, b):
    return jnp.dot(a, b, preferred_element_type=f32)


def _dot_nt(a, b):
    return lax.dot_general(a, b, _NT, preferred_element_type=f32)


def _pack(x):
    return pltpu.bitcast(x.astype(bf16), u32)


def _unpack(x):
    return pltpu.bitcast(x, bf16)


def _ln(x):
    m = jnp.mean(x, axis=-1, keepdims=True)
    xc = x - m
    v = jnp.mean(xc * xc, axis=-1, keepdims=True)
    return xc * lax.rsqrt(v + 1e-5)


def _fold(op, p):
    r = p[0:8]
    for j in range(1, 5):
        r = op(r, p[8 * j:8 * j + 8])
    r = op(r, pltpu.roll(r, 2, 0))
    return op(r, pltpu.roll(r, 4, 0))


def _tile5(r):
    return jnp.concatenate([r] * 5, axis=0)


def _phi(p):
    ep = jnp.exp(p - _tile5(_fold(jnp.maximum, p)))
    en = jnp.exp(_tile5(_fold(jnp.minimum, p)) - p)
    ep = ep * _tile5(1.0 / _fold(jnp.add, ep))
    en = en * _tile5(1.0 / _fold(jnp.add, en))
    return jnp.concatenate([ep, en], axis=0).astype(bf16)


def _bd(k):
    lo = lax.broadcasted_iota(i32, (L, 128), 1) < 64
    z = jnp.zeros((L, 128), f32)
    mid = k[:, 128:256]
    top = jnp.concatenate([k[:, 0:128], jnp.where(lo, mid, z), z], axis=1)
    bot = jnp.concatenate([z, jnp.where(lo, z, mid), k[:, 256:384]], axis=1)
    return jnp.concatenate([top, bot], axis=0).astype(bf16)


def _probs(qb, kbd):
    s = _dot_nt(qb, kbd) * SCALE
    r = lax.broadcasted_iota(i32, (L, 2 * L), 0)
    c = lax.broadcasted_iota(i32, (L, 2 * L), 1)
    first = c < L
    mask = (r < MEM) | (r >= jnp.where(first, c, c - L))
    s = jnp.where(mask, s, -1000000000.0)
    neg = jnp.full_like(s, -jnp.inf)
    ma = jnp.max(jnp.where(first, s, neg), axis=-1, keepdims=True)
    mb = jnp.max(jnp.where(first, neg, s), axis=-1, keepdims=True)
    e = jnp.exp(s - jnp.where(first, ma, mb))
    z = jnp.zeros_like(e)
    sa = jnp.sum(jnp.where(first, e, z), axis=-1, keepdims=True)
    sb = jnp.sum(jnp.where(first, z, e), axis=-1, keepdims=True)
    return (e * (1.0 / jnp.where(first, sa, sb))).astype(bf16)


def _kernel(x_in, wqkv, phiu, wo_a, mem0, wqt_hbm, wkt_hbm, wvt_hbm, wo_hbm, out_ref,
            x_ref, wat_ref, wop_ref, phiq_ref, kv_ref, kvm_ref,
            stage_ref, wb_ref, wo_ref, mem_ref, sv_ref, osv_ref, o_ref, sems):
    big = (wqt_hbm, wkt_hbm, wvt_hbm, wo_hbm)
    copies = [pltpu.make_async_copy(big[n], stage_ref.at[n], sems.at[n]) for n in range(4)]
    for cp in copies:
        cp.start()

    x_ref[...] = x_in[...].astype(f32)

    for g in range(GA):
        c0 = 128 * ((160 * g) // 128)
        col = lax.broadcasted_iota(i32, (RA, 256), 1) + c0
        row = lax.broadcasted_iota(i32, (RA, 256), 0)
        ecol = lax.broadcasted_iota(i32, (DA, 256), 1) + c0
        erow = lax.broadcasted_iota(i32, (DA, 256), 0)
        emat = jnp.where(ecol - DA * ((ecol * 3277) >> 16) == erow, 1.0, 0.0).astype(bf16)
        urep = _dot(phiu[160 * g:160 * g + 160, :], emat)
        phit, perm = [], []
        for pp in range(4):
            lo = (8 * g + 2 * pp + (row & 1)) * DA
            phit.append(jnp.where((col >= lo) & (col < lo + DA), urep[RA * pp:RA * pp + RA], 0.0))
            perm.append(jnp.where(col == lo + (row >> 1), 1.0, 0.0))
        phit = jnp.concatenate(phit, axis=0).astype(bf16)
        perm = jnp.concatenate(perm, axis=0).astype(bf16)
        wat_ref[0, g] = _pack(_dot_nt(phit, wqkv[:, c0:c0 + 256]))
        wat_ref[1, g] = _pack(_dot_nt(phit, wqkv[:, D + c0:D + c0 + 256]))
        wat_ref[2, g] = _pack(_dot_nt(perm, wqkv[:, 2 * D + c0:2 * D + c0 + 256]))
        wop_ref[80 * g:80 * g + 80, :] = _pack(_dot(perm, wo_a[c0:c0 + 256, :]))

    def layer_a():
        kv_ref[...] = jnp.zeros(kv_ref.shape, f32)

        def phase1(c, carry):
            r0 = pl.multiple_of(c * TC, TC)
            xn = _ln(x_ref[pl.ds(r0, TC), :]).astype(bf16)
            ones = jnp.ones((8, TC), f32)
            for g in range(GA):
                pq = _dot_nt(_unpack(wat_ref[0, g]), xn)
                pk = _dot_nt(_unpack(wat_ref[1, g]), xn)
                vt = _dot_nt(_unpack(wat_ref[2, g]), xn)
                for pp in range(4):
                    p = 4 * g + pp
                    sl = slice(RA * pp, RA * pp + RA)
                    phiq_ref[c, p] = pltpu.bitcast(_phi(pq[sl]), u32)
                    vext = jnp.concatenate([vt[sl], ones], axis=0).astype(bf16)
                    kv_ref[p] += _dot_nt(vext, _phi(pk[sl]))
            return carry

        lax.fori_loop(0, NCH, phase1, 0)

        same = ((lax.broadcasted_iota(i32, (RA + 8, 2 * RA), 0) & 1)
                == (lax.broadcasted_iota(i32, (RA + 8, 2 * RA), 1) & 1))
        for p in range(NPA):
            kvm_ref[p] = _pack(jnp.where(same, kv_ref[p], 0.0))

        def phase2(c, carry):
            r0 = pl.multiple_of(c * TC, TC)
            ot = []
            for p in range(NPA):
                ne = _dot(_unpack(kvm_ref[p]), _unpack(phiq_ref[c, p]))
                ot.append(ne[0:RA] * _tile5(1.0 / (ne[RA:RA + 8] + 1e-6)))
            o = jnp.concatenate(ot, axis=0).T.astype(bf16)
            x_ref[pl.ds(r0, TC), :] += _dot(o, _unpack(wop_ref[...]))
            return carry

        lax.fori_loop(0, NCH, phase2, 0)

    def prep_b():
        for n in range(3):
            copies[n].wait()

            def tr(j, carry):
                r0 = pl.multiple_of(j * TRC, TRC)
                t = stage_ref[n, pl.ds(r0, TRC), :].T
                wb_ref[n, j] = pltpu.bitcast(t, u32)
                return carry

            lax.fori_loop(0, HD // TRC, tr, 0)
        copies[3].wait()

        def cpy(j, carry):
            r0 = pl.multiple_of(j * TRC, TRC)
            wo_ref[pl.ds(pl.multiple_of(j * (TRC // 2), TRC // 2), TRC // 2), :] = pltpu.bitcast(
                stage_ref[3, pl.ds(r0, TRC), :], u32)
            return carry

        lax.fori_loop(0, HD // TRC, cpy, 0)

    def b_step(h, is_a):
        st = {}
        nrow = 16 if is_a else 24

        def proj(p, which):
            c0 = p * PW
            w = wb_ref[which, c0 // TRC, :, c0 % TRC:c0 % TRC + PW]
            y = _dot(h, _unpack(w))
            if is_a:
                sv_ref[which, :, c0:c0 + PW] = y[L:L + 8]
                y = y[0:L]
            else:
                y = jnp.concatenate([y[0:8], sv_ref[which, :, c0:c0 + PW], y[8:32]], axis=0)
            st[(p, which)] = y.astype(bf16) if which == 0 else _bd(y)

        def do_qk(p):
            st[(p, 'p')] = _probs(st.pop((p, 0)), st.pop((p, 1)))

        def do_pv(p):
            c0 = p * PW
            o = _dot(st.pop((p, 'p')), st.pop((p, 2)))
            if is_a:
                osv_ref[:, c0:c0 + PW] = o[32:L]
                o = o[0:32]
            else:
                o = jnp.concatenate([o, osv_ref[:, c0:c0 + PW]], axis=0)
            o_ref[0:nrow, c0:c0 + PW] = _pack(o)

        def do_o(p0, p1):
            y = _dot(_unpack(o_ref[0:nrow, p0 * PW:p1 * PW]),
                     _unpack(wo_ref[p0 * PW // 2:p1 * PW // 2, :]))
            st['y'] = y if 'y' not in st else st['y'] + y

        for s in range(NPB):
            proj(s, 0)
            if s >= 1:
                do_qk(s - 1)
            proj(s, 1)
            if s >= 2:
                do_pv(s - 2)
            proj(s, 2)
        do_o(0, 3)
        do_qk(NPB - 1)
        do_pv(NPB - 2)
        do_o(3, 9)
        do_pv(NPB - 1)
        do_o(9, 14)
        do_o(14, 16)
        return st['y']

    def layer_b():
        mem_ref[...] = mem0[...].astype(f32)

        def body(j, carry):
            r0 = pl.multiple_of(j * 64, 64)
            xn = _ln(x_ref[pl.ds(r0, 64), :])
            y = b_step(jnp.concatenate([mem_ref[...], xn[0:L]], axis=0).astype(bf16), True)
            x_ref[pl.ds(r0, 24), :] += y[8:32]
            y = b_step(jnp.concatenate([y[0:8], xn[L:64]], axis=0).astype(bf16), False)
            mem_ref[...] = y[0:8]
            x_ref[pl.ds(r0 + 32, 32), :] += y[8:L]
            x_ref[pl.ds(r0 + 24, 8), :] += y[L:L + 8]
            return carry

        lax.fori_loop(0, S // 64, body, 0)

    def layer(li, carry):
        layer_a()

        @pl.when(li == 0)
        def _():
            prep_b()

        layer_b()
        return carry

    lax.fori_loop(0, 2, layer, 0)
    out_ref[...] = x_ref[...].astype(bf16)


@jax.jit
def pallas_interleave_layers__linear_kernel_hedgehog__memory_aug_recurrent_mem_tr__prompt_kernel(
    A_x: jax.Array,
    A_wqkv: jax.Array,
    A_w_phi: jax.Array,
    A_wo: jax.Array,
    B_x: jax.Array,
    B_mem0: jax.Array,
    B_Wq: jax.Array,
    B_Wk: jax.Array,
    B_Wv: jax.Array,
    B_Wo: jax.Array,
    B_seg_len: jax.Array,
):
    del B_x, B_seg_len
    x = A_x.reshape(S, D)
    phiu = A_w_phi.reshape(NPA, 2, DA, DA).transpose(0, 3, 1, 2).reshape(HA * DA, DA)
    wqt = B_Wq.transpose(1, 2, 0).reshape(HD, D)
    wkt = B_Wk.transpose(1, 2, 0).reshape(HD, D)
    wvt = B_Wv.transpose(1, 2, 0).reshape(HD, D)
    wo = B_Wo.reshape(HD, D)
    vmem = pl.BlockSpec(memory_space=pltpu.VMEM)
    hbm = pl.BlockSpec(memory_space=pl.ANY)
    out = pl.pallas_call(
        _kernel,
        out_shape=jax.ShapeDtypeStruct((S, D), bf16),
        in_specs=[vmem, vmem, vmem, vmem, vmem, hbm, hbm, hbm, hbm],
        out_specs=vmem,
        scratch_shapes=[
            pltpu.VMEM((S, D), f32),
            pltpu.VMEM((3, GA, 80, D), u32),
            pltpu.VMEM((D // 2, D), u32),
            pltpu.VMEM((NCH, NPA, RA, TC), u32),
            pltpu.VMEM((NPA, RA + 8, 2 * RA), f32),
            pltpu.VMEM((NPA, (RA + 8) // 2, 2 * RA), u32),
            pltpu.VMEM((4, HD, D), bf16),
            pltpu.VMEM((3, HD // TRC, D // 2, TRC), u32),
            pltpu.VMEM((HD // 2, D), u32),
            pltpu.VMEM((MEM, D), f32),
            pltpu.VMEM((3, 8, HD), f32),
            pltpu.VMEM((8, HD), f32),
            pltpu.VMEM((24, HD), u32),
            pltpu.SemaphoreType.DMA((4,)),
        ],
        compiler_params=pltpu.CompilerParams(vmem_limit_bytes=120 * 1024 * 1024),
    )(x, A_wqkv, phiu, A_wo, B_mem0.reshape(MEM, D), wqt, wkt, wvt, wo)
    return out.reshape(1, S, D)
```

```python
import functools
import os

import jax
import jax.numpy as jnp
from jax import lax
import jax.experimental.pallas as pl
import jax.experimental.pallas.tpu as pltpu

f32, bf16, u32, i32 = jnp.float32, jnp.bfloat16, jnp.uint32, jnp.int32

S, D = 2048, 640
HA, DA = 32, 20
NPA = HA // 2
RA = 2 * DA
GA = 4
TC = 256
NCH = S // TC
HB, DB, MEM, SEG = 32, 192, 8, 32
HD = HB * DB
L = MEM + SEG
NPB = HB // 2
PW = 2 * DB
SCALE = DB ** -0.5
TRC = 768
NTR = HD // TRC
NB = S // 64
assert NTR == NCH

SCH_A = tuple(int(v) for v in os.environ.get("SCH_A", "0,0,0,4,6,6,12").split(","))
SCH_B = tuple(int(v) for v in os.environ.get("SCH_B", "1,0,1,3,1,4,6").split(","))

_NT = (((1,), (1,)), ((), ()))


def _dot(a, b):
    return jnp.dot(a, b, preferred_element_type=f32)


def _dot_nt(a, b):
    return lax.dot_general(a, b, _NT, preferred_element_type=f32)


def _pack(x):
    return pltpu.bitcast(x.astype(bf16), u32)


def _unpack(x):
    return pltpu.bitcast(x, bf16)


def _ln(x):
    m = jnp.mean(x, axis=-1, keepdims=True)
    xc = x - m
    r = lax.rsqrt(jnp.mean(xc * xc, axis=-1, keepdims=True) + 1e-5)
    return x * r - m * r


def _fold(op, p):
    r = p[0:8]
    for j in range(1, 5):
        r = op(r, p[8 * j:8 * j + 8])
    r = op(r, pltpu.roll(r, 2, 0))
    return op(r, pltpu.roll(r, 4, 0))


def _tile5(r):
    return jnp.concatenate([r] * 5, axis=0)


def _phi(p):
    ep = jnp.exp(p - _tile5(_fold(jnp.maximum, p)))
    en = jnp.exp(_tile5(_fold(jnp.minimum, p)) - p)
    ep = ep * _tile5(1.0 / _fold(jnp.add, ep))
    en = en * _tile5(1.0 / _fold(jnp.add, en))
    return jnp.concatenate([ep, en], axis=0).astype(bf16)


def _split(k):
    lo = lax.broadcasted_iota(i32, (L, 128), 1) < 64
    z = jnp.zeros((L, 128), f32)
    mid = k[:, 128:256]
    outer = jnp.concatenate([k[:, 0:128], k[:, 256:384]], axis=0).astype(bf16)
    mid = jnp.concatenate([jnp.where(lo, mid, z), jnp.where(lo, z, mid)], axis=0).astype(bf16)
    return outer, mid


def _probs(q, k):
    r = lax.broadcasted_iota(i32, (L, 2 * L), 0)
    c = lax.broadcasted_iota(i32, (L, 2 * L), 1)
    first = c < L
    so = _dot_nt(q[0], k[0])
    s = jnp.where(first, so[0:L], so[L:2 * L]) + _dot_nt(q[1], k[1])
    s = s * SCALE
    mask = (r < MEM) | (r >= jnp.where(first, c, c - L))
    s = jnp.where(mask, s, -1000000000.0)
    neg = jnp.full_like(s, -jnp.inf)
    ma = jnp.max(jnp.where(first, s, neg), axis=-1, keepdims=True)
    mb = jnp.max(jnp.where(first, neg, s), axis=-1, keepdims=True)
    e = jnp.exp(s - jnp.where(first, ma, mb))
    z = jnp.zeros_like(e)
    ea = jnp.where(first, e, z)
    eb = jnp.where(first, z, e)
    pa = ea * (1.0 / jnp.sum(ea, axis=-1, keepdims=True))
    pb = eb * (1.0 / jnp.sum(eb, axis=-1, keepdims=True))
    return jnp.concatenate([pa, pb], axis=0).astype(bf16), (pa + pb).astype(bf16)


def _pv(p, v):
    oo = _dot(p[0], v[0])
    return jnp.concatenate([oo[0:L], _dot(p[1], v[1]), oo[L:2 * L]], axis=1)


def _kernel(x_hbm, wqkv_hbm, phiu, woa_hbm, mem0, wqt_hbm, wkt_hbm, wvt_hbm, wo_hbm, out_ref,
            xin_ref, wqkv, wo_a, x_ref, xna_ref, xnb_ref, xa_ref, xb_ref, yb_ref, oa_ref, wat_ref, wop_ref, phiq_ref, kv_ref,
            kvm_ref, stage_ref, wb_ref, wo_ref, mem_ref, sv_ref, osv_ref, o_ref, sems):
    cp_wqkv = pltpu.make_async_copy(wqkv_hbm, wqkv, sems.at[0])
    cp_woa = pltpu.make_async_copy(woa_hbm, wo_a, sems.at[1])
    cp_x = pltpu.make_async_copy(x_hbm, xin_ref, sems.at[2])
    cp_wo = [pltpu.make_async_copy(wo_hbm.at[:, pl.ds(128 * n, 128)], wo_ref.at[n], sems.at[3 + n])
             for n in range(D // 128)]
    big = (wqt_hbm, wkt_hbm, wvt_hbm)

    def cp_w(n, j):
        rows = pl.ds(pl.multiple_of(j * TRC, TRC), TRC)
        return pltpu.make_async_copy(big[n].at[rows, :], stage_ref.at[n, rows, :], sems.at[8 + n * NTR + j])

    cp_wqkv.start()
    cp_woa.start()
    cp_x.start()
    for j in range(NTR):
        for n in range(3):
            cp_w(n, j).start()
    for cp in cp_wo:
        cp.start()

    with jax.named_scope("wait_wqkv"):
        cp_wqkv.wait()
    with jax.named_scope("wait_woa"):
        cp_woa.wait()
    for g in range(GA):
        c0 = 128 * ((160 * g) // 128)
        col = lax.broadcasted_iota(i32, (RA, 256), 1) + c0
        row = lax.broadcasted_iota(i32, (RA, 256), 0)
        ecol = lax.broadcasted_iota(i32, (DA, 256), 1) + c0
        erow = lax.broadcasted_iota(i32, (DA, 256), 0)
        emat = jnp.where(ecol - DA * ((ecol * 3277) >> 16) == erow, 1.0, 0.0).astype(bf16)
        urep = _dot(phiu[160 * g:160 * g + 160, :], emat)
        phit, perm = [], []
        for pp in range(4):
            lo = (8 * g + 2 * pp + (row & 1)) * DA
            phit.append(jnp.where((col >= lo) & (col < lo + DA), urep[RA * pp:RA * pp + RA], 0.0))
            perm.append(jnp.where(col == lo + (row >> 1), 1.0, 0.0))
        phit = jnp.concatenate(phit, axis=0).astype(bf16)
        perm = jnp.concatenate(perm, axis=0).astype(bf16)
        wat_ref[0, g] = _pack(_dot_nt(phit, wqkv[:, c0:c0 + 256]))
        wat_ref[1, g] = _pack(_dot_nt(phit, wqkv[:, D + c0:D + c0 + 256]))
        wat_ref[2, g] = _pack(_dot_nt(perm, wqkv[:, 2 * D + c0:2 * D + c0 + 256]))
        wop_ref[80 * g:80 * g + 80, :] = _pack(_dot(perm, wo_a[c0:c0 + 256, :]))

    with jax.named_scope("wait_x"):
        cp_x.wait()

    def init_x(c, carry):
        r0 = pl.multiple_of(c * TC, TC)
        x = xin_ref[pl.ds(r0, TC), :].astype(f32)
        x_ref[pl.ds(r0, TC), :] = x
        xna_ref[pl.ds(pl.multiple_of(c * (TC // 2), TC // 2), TC // 2), :] = _pack(_ln(x))
        return carry

    with jax.named_scope("init_x"):
        lax.fori_loop(0, NCH, init_x, 0)

    def a_phase1(with_transposes):
        def body(c, carry):
            if with_transposes:
                for n in range(3):
                    cp_w(n, c).wait()
            xn = _unpack(xna_ref[pl.ds(pl.multiple_of(c * (TC // 2), TC // 2), TC // 2), :])
            ones = jnp.ones((8, TC), f32)
            for g in range(GA):
                pq = _dot_nt(_unpack(wat_ref[0, g]), xn)
                pk = _dot_nt(_unpack(wat_ref[1, g]), xn)
                vt = _dot_nt(_unpack(wat_ref[2, g]), xn)
                for pp in range(4):
                    p = 4 * g + pp
                    sl = slice(RA * pp, RA * pp + RA)
                    phiq_ref[c, p] = pltpu.bitcast(_phi(pq[sl]), u32)
                    vext = jnp.concatenate([vt[sl], ones], axis=0).astype(bf16)
                    kv_ref[p] += _dot_nt(vext, _phi(pk[sl]))
                if with_transposes and g < 3:
                    t = stage_ref[g, pl.ds(pl.multiple_of(c * TRC, TRC), TRC), :].T
                    wb_ref[g, c] = pltpu.bitcast(t, u32)
            return carry

        lax.fori_loop(0, NCH, body, 0)

    def a_phase2():
        same = ((lax.broadcasted_iota(i32, (RA + 8, 2 * RA), 0) & 1)
                == (lax.broadcasted_iota(i32, (RA + 8, 2 * RA), 1) & 1))
        for p in range(NPA):
            kvm_ref[p] = _pack(jnp.where(same, kv_ref[p], 0.0))

        def body(c, carry):
            ot = []
            for p in range(NPA):
                ne = _dot(_unpack(kvm_ref[p]), _unpack(phiq_ref[c, p]))
                ot.append(ne[0:RA] * _tile5(1.0 / (ne[RA:RA + 8] + 1e-6)))
            o = jnp.concatenate(ot, axis=0).T
            oa_ref[pl.ds(pl.multiple_of(c * (TC // 2), TC // 2), TC // 2), :] = _pack(o)
            return carry

        lax.fori_loop(0, NCH, body, 0)

    def a_finish(jr, jw):
        y = _dot(_unpack(oa_ref[pl.ds(pl.multiple_of(jr * 32, 32), 32), :]), _unpack(wop_ref[...]))
        x = x_ref[pl.ds(pl.multiple_of(jr * 64, 64), 64), :] + y
        x_ref[pl.ds(pl.multiple_of(jw * 64, 64), 64), :] = x
        xa_ref[...] = x

    def a_norm(i):
        xnb_ref[8 * i:8 * i + 8, :] = _ln(xa_ref[8 * i:8 * i + 8, :])

    def b_finish(jr, jw, i):
        x = x_ref[pl.ds(pl.multiple_of(jr * 64 + 16 * i, 16), 16), :] + yb_ref[16 * i:16 * i + 16, :]
        x_ref[pl.ds(pl.multiple_of(jw * 64 + 16 * i, 16), 16), :] = x
        out_ref[pl.ds(pl.multiple_of(jr * 64 + 16 * i, 16), 16), :] = x.astype(bf16)
        xb_ref[16 * i:16 * i + 16, :] = x
        xna_ref[pl.ds(pl.multiple_of(jr * 32 + 8 * i, 8), 8), :] = _pack(_ln(xb_ref[16 * i:16 * i + 16, :]))

    wo32 = wo_ref.bitcast(u32)

    def b_step(h, is_a, side):
        st = {}
        nrow = 16 if is_a else 24

        def proj(p, which):
            c0 = p * PW
            w = wb_ref[which, c0 // TRC, :, c0 % TRC:c0 % TRC + PW]
            y = _dot(h, _unpack(w))
            if is_a:
                sv_ref[which, :, c0:c0 + PW] = y[L:L + 8]
                y = y[0:L]
            else:
                y = jnp.concatenate([y[0:8], sv_ref[which, :, c0:c0 + PW], y[8:32]], axis=0)
            if which == 0:
                st[(p, which)] = (jnp.concatenate([y[:, 0:128], y[:, 256:384]], axis=0).astype(bf16),
                                  y[:, 128:256].astype(bf16))
            else:
                st[(p, which)] = _split(y)

        def do_qk(p):
            st[(p, 'p')] = _probs(st.pop((p, 0)), st.pop((p, 1)))

        def do_pv(p):
            c0 = p * PW
            o = _pv(st.pop((p, 'p')), st.pop((p, 2)))
            if is_a:
                osv_ref[:, c0:c0 + PW] = o[32:L]
                o = o[0:32]
            else:
                o = jnp.concatenate([o, osv_ref[:, c0:c0 + PW]], axis=0)
            o_ref[0:nrow, c0:c0 + PW] = _pack(o)

        def do_o(n):
            k0 = st.get('k', 0)
            k1 = min(k0 + n, HD // 128)
            if k0 == k1:
                return
            st['k'] = k1
            w = jnp.concatenate([wo32[t, k0 * 64:k1 * 64, :] for t in range(D // 128)], axis=1)
            y = _dot(_unpack(o_ref[0:nrow, k0 * 128:k1 * 128]), _unpack(w))
            st['y'] = y if 'y' not in st else st['y'] + y

        o1, o2, o3, olag, f1, f2, f3 = SCH_A if is_a else SCH_B
        for s in range(NPB):
            on = s >= olag
            proj(s, 0)
            if on:
                do_o(o1)
            if s >= 1:
                do_qk(s - 1)
            proj(s, 1)
            if on:
                do_o(o2)
            if s >= 2:
                do_pv(s - 2)
            proj(s, 2)
            if on:
                do_o(o3)
            if s in side:
                side[s]()
            assert st.get('k', 0) <= 3 * max(s - 2, 0)
        do_o(f1)
        do_qk(NPB - 1)
        do_o(f2)
        do_pv(NPB - 2)
        do_o(f3)
        assert st.get('k', 0) <= 3 * (NPB - 2)
        do_pv(NPB - 1)
        do_o(3 * (NPB - 1) - st['k'])
        do_o(3)
        return st['y']

    def layer_b():
        mem_ref[...] = mem0[...].astype(f32)
        yb_ref[...] = jnp.zeros(yb_ref.shape, f32)
        a_finish(0, 0)
        for i in range(8):
            a_norm(i)

        def body(j, carry):
            jp = jnp.maximum(j - 1, 0)
            jw = jnp.where(j == 0, NB, jp)
            side = {2 + 3 * i: functools.partial(b_finish, jp, jw, i) for i in range(4)}
            y = b_step(jnp.concatenate([mem_ref[...], xnb_ref[0:L, :]], axis=0).astype(bf16), True, side)
            h2 = jnp.concatenate([y[0:8], xnb_ref[L:64, :]], axis=0).astype(bf16)
            a_finish(jnp.minimum(j + 1, NB - 1), j + 1)
            yb_ref[0:24, :] = y[8:32]
            side = {3 + i: functools.partial(a_norm, i) for i in range(8)}
            y = b_step(h2, False, side)
            mem_ref[...] = y[0:8]
            yb_ref[32:64, :] = y[8:L]
            yb_ref[24:32, :] = y[L:L + 8]
            return carry

        lax.fori_loop(0, NB, body, 0)
        for i in range(4):
            b_finish(NB - 1, NB - 1, i)

    def layer(li, carry):
        kv_ref[...] = jnp.zeros(kv_ref.shape, f32)

        @pl.when(li == 0)
        def _():
            with jax.named_scope("a_p1_first"):
                a_phase1(True)

        @pl.when(li != 0)
        def _():
            with jax.named_scope("a_p1"):
                a_phase1(False)

        with jax.named_scope("a_p2"):
            a_phase2()

        @pl.when(li == 0)
        def _():
            with jax.named_scope("wait_wo"):
                for cp in cp_wo:
                    cp.wait()

        with jax.named_scope("layer_b"):
            layer_b()
        return carry

    lax.fori_loop(0, 2, layer, 0)


@jax.jit
def pallas_interleave_layers__linear_kernel_hedgehog__memory_aug_recurrent_mem_tr__prompt_kernel(
    A_x: jax.Array,
    A_wqkv: jax.Array,
    A_w_phi: jax.Array,
    A_wo: jax.Array,
    B_x: jax.Array,
    B_mem0: jax.Array,
    B_Wq: jax.Array,
    B_Wk: jax.Array,
    B_Wv: jax.Array,
    B_Wo: jax.Array,
    B_seg_len: jax.Array,
):
    del B_x, B_seg_len
    x = A_x.reshape(S, D)
    phiu = A_w_phi.reshape(NPA, 2, DA, DA).transpose(0, 3, 1, 2).reshape(HA * DA, DA)
    wqt = B_Wq.transpose(1, 2, 0).reshape(HD, D)
    wkt = B_Wk.transpose(1, 2, 0).reshape(HD, D)
    wvt = B_Wv.transpose(1, 2, 0).reshape(HD, D)
    wo = B_Wo.reshape(HD, D)
    vmem = pl.BlockSpec(memory_space=pltpu.VMEM)
    hbm = pl.BlockSpec(memory_space=pl.ANY)
    out = pl.pallas_call(
        _kernel,
        out_shape=jax.ShapeDtypeStruct((S, D), bf16),
        in_specs=[hbm, hbm, vmem, hbm, vmem, hbm, hbm, hbm, hbm],
        out_specs=vmem,
        scratch_shapes=[
            pltpu.VMEM((S, D), bf16),
            pltpu.VMEM((D, 3 * D), bf16),
            pltpu.VMEM((D, D), bf16),
            pltpu.VMEM((S + 64, D), f32),
            pltpu.VMEM((S // 2, D), u32),
            pltpu.VMEM((64, D), f32),
            pltpu.VMEM((64, D), f32),
            pltpu.VMEM((64, D), f32),
            pltpu.VMEM((64, D), f32),
            pltpu.VMEM((S // 2, D), u32),
            pltpu.VMEM((3, GA, 80, D), u32),
            pltpu.VMEM((D // 2, D), u32),
            pltpu.VMEM((NCH, NPA, RA, TC), u32),
            pltpu.VMEM((NPA, RA + 8, 2 * RA), f32),
            pltpu.VMEM((NPA, (RA + 8) // 2, 2 * RA), u32),
            pltpu.VMEM((3, HD, D), bf16),
            pltpu.VMEM((3, NTR, D // 2, TRC), u32),
            pltpu.VMEM((D // 128, HD, 128), bf16),
            pltpu.VMEM((MEM, D), f32),
            pltpu.VMEM((3, 8, HD), f32),
            pltpu.VMEM((8, HD), f32),
            pltpu.VMEM((24, HD), u32),
            pltpu.SemaphoreType.DMA((8 + 3 * NTR,)),
        ],
        compiler_params=pltpu.CompilerParams(vmem_limit_bytes=120 * 1024 * 1024),
    )(x, A_wqkv, phiu, A_wo, B_mem0.reshape(MEM, D), wqt, wkt, wvt, wo)
    return out.reshape(1, S, D)
```

```python
import functools
import os

import jax
import jax.numpy as jnp
from jax import lax
import jax.experimental.pallas as pl
import jax.experimental.pallas.tpu as pltpu

f32, bf16, u32, i32 = jnp.float32, jnp.bfloat16, jnp.uint32, jnp.int32

S, D = 2048, 640
HA, DA = 32, 20
NPA = HA // 2
RA = 2 * DA
GA = 4
TC = 256
NCH = S // TC
HB, DB, MEM, SEG = 32, 192, 8, 32
HD = HB * DB
L = MEM + SEG
NPB = HB // 2
PW = 2 * DB
SCALE = DB ** -0.5
TRC = 768
NTR = HD // TRC
NB = S // 64
assert NTR == NCH

SCH_A = tuple(int(v) for v in os.environ.get("SCH_A", "0,0,0,4,6,6,12").split(","))
SCH_B = tuple(int(v) for v in os.environ.get("SCH_B", "1,0,1,3,1,4,6").split(","))

P2U = int(os.environ.get("P2U", "1"))

_NT = (((1,), (1,)), ((), ()))


def _dot(a, b):
    return jnp.dot(a, b, preferred_element_type=f32)


def _dot_nt(a, b):
    return lax.dot_general(a, b, _NT, preferred_element_type=f32)


def _pack(x):
    return pltpu.bitcast(x.astype(bf16), u32)


def _unpack(x):
    return pltpu.bitcast(x, bf16)


def _ln(x):
    m = jnp.mean(x, axis=-1, keepdims=True)
    xc = x - m
    r = lax.rsqrt(jnp.mean(xc * xc, axis=-1, keepdims=True) + 1e-5)
    return x * r - m * r


def _fold(op, p):
    r = p[0:8]
    for j in range(1, 5):
        r = op(r, p[8 * j:8 * j + 8])
    r = op(r, pltpu.roll(r, 2, 0))
    return op(r, pltpu.roll(r, 4, 0))


def _tile5(r):
    return jnp.concatenate([r] * 5, axis=0)


def _phi(p):
    ep = jnp.exp(p - _tile5(_fold(jnp.maximum, p)))
    en = jnp.exp(_tile5(_fold(jnp.minimum, p)) - p)
    ep = ep * _tile5(1.0 / _fold(jnp.add, ep))
    en = en * _tile5(1.0 / _fold(jnp.add, en))
    return jnp.concatenate([ep, en], axis=0).astype(bf16)


def _split(k):
    lo = lax.broadcasted_iota(i32, (L, 128), 1) < 64
    z = jnp.zeros((L, 128), f32)
    mid = k[:, 128:256]
    outer = jnp.concatenate([k[:, 0:128], k[:, 256:384]], axis=0).astype(bf16)
    mid = jnp.concatenate([jnp.where(lo, mid, z), jnp.where(lo, z, mid)], axis=0).astype(bf16)
    return outer, mid


def _probs(q, k):
    r = lax.broadcasted_iota(i32, (L, 2 * L), 0)
    c = lax.broadcasted_iota(i32, (L, 2 * L), 1)
    first = c < L
    so = _dot_nt(q[0], k[0])
    s = jnp.where(first, so[0:L], so[L:2 * L]) + _dot_nt(q[1], k[1])
    s = s * SCALE
    mask = (r < MEM) | (r >= jnp.where(first, c, c - L))
    s = jnp.where(mask, s, -1000000000.0)
    neg = jnp.full_like(s, -jnp.inf)
    ma = jnp.max(jnp.where(first, s, neg), axis=-1, keepdims=True)
    mb = jnp.max(jnp.where(first, neg, s), axis=-1, keepdims=True)
    e = jnp.exp(s - jnp.where(first, ma, mb))
    z = jnp.zeros_like(e)
    ea = jnp.where(first, e, z)
    eb = jnp.where(first, z, e)
    pa = ea * (1.0 / jnp.sum(ea, axis=-1, keepdims=True))
    pb = eb * (1.0 / jnp.sum(eb, axis=-1, keepdims=True))
    return jnp.concatenate([pa, pb], axis=0).astype(bf16), (pa + pb).astype(bf16)


def _pv(p, v):
    oo = _dot(p[0], v[0])
    return jnp.concatenate([oo[0:L], _dot(p[1], v[1]), oo[L:2 * L]], axis=1)


def _kernel(x_hbm, wqkv_hbm, phi_ref, woa_hbm, mem0, wqt_hbm, wkt_hbm, wvt_hbm, wo_hbm, out_hbm,
            xin_ref, wqkv, wo_a, x_ref, xna_ref, xnb_ref, xa_ref, xb_ref, yb_ref, oa_ref, wat_ref,
            wop_ref, phiq_ref, kv_ref, kvm_ref, stage_ref, wb_ref, wo_ref, mem_ref, sv_ref, osv_ref,
            o_ref, sems):
    cp_wqkv = pltpu.make_async_copy(wqkv_hbm, wqkv, sems.at[0])
    cp_woa = pltpu.make_async_copy(woa_hbm, wo_a, sems.at[1])
    cp_x0 = pltpu.make_async_copy(x_hbm.at[pl.ds(0, 2 * TC), :], xin_ref.at[pl.ds(0, 2 * TC), :], sems.at[2])
    cp_x1 = pltpu.make_async_copy(x_hbm.at[pl.ds(2 * TC, S - 2 * TC), :],
                                  xin_ref.at[pl.ds(2 * TC, S - 2 * TC), :], sems.at[3])
    cp_wo = [pltpu.make_async_copy(wo_hbm.at[:, pl.ds(128 * n, 128)], wo_ref.at[n], sems.at[4 + n])
             for n in range(D // 128)]
    big = (wqt_hbm, wkt_hbm, wvt_hbm)

    def cp_w(n, j):
        rows = pl.ds(pl.multiple_of(j * TRC, TRC), TRC)
        return pltpu.make_async_copy(big[n].at[rows, :], stage_ref.at[n, rows, :], sems.at[10 + n * NTR + j])

    def cp_out(j, nblk):
        rows = pl.ds(pl.multiple_of(j * 64, 64), 64 * nblk)
        return pltpu.make_async_copy(xin_ref.at[rows, :], out_hbm.at[rows, :], sems.at[9])

    cp_wqkv.start()
    cp_x0.start()
    cp_x1.start()
    for j in range(NTR):
        for n in range(3):
            cp_w(n, j).start()
    cp_woa.start()
    for cp in cp_wo:
        cp.start()

    def init_x(c):
        x = xin_ref[pl.ds(pl.multiple_of(c * TC, TC), TC), :].astype(f32)
        x_ref[pl.ds(pl.multiple_of(c * TC, TC), TC), :] = x
        xna_ref[pl.ds(pl.multiple_of(c * (TC // 2), TC // 2), TC // 2), :] = _pack(_ln(x))

    def head_lo(g, pp):
        return (8 * g + 2 * pp + (lax.broadcasted_iota(i32, (RA, 256), 0) & 1)) * DA

    def perm_mat(g):
        col = lax.broadcasted_iota(i32, (RA, 256), 1) + 128 * ((160 * g) // 128)
        half = lax.broadcasted_iota(i32, (RA, 256), 0) >> 1
        return jnp.concatenate([jnp.where(col == head_lo(g, pp) + half, 1.0, 0.0) for pp in range(4)],
                               axis=0).astype(bf16)

    ecol = lax.broadcasted_iota(i32, (HA, D), 1) - DA * lax.broadcasted_iota(i32, (HA, D), 0)
    tp = _dot(phi_ref[0], jnp.where(ecol == 0, 1.0, 0.0).astype(bf16))
    for d in range(1, DA):
        tp = tp + _dot(phi_ref[d], jnp.where(ecol == d, 1.0, 0.0).astype(bf16))
    rep = jnp.where((lax.broadcasted_iota(i32, (RA, DA), 0) >> 1) == lax.broadcasted_iota(i32, (RA, DA), 1),
                    1.0, 0.0).astype(bf16)
    urep = _dot(rep, tp.astype(bf16))
    phit = []
    for g in range(GA):
        c0 = 128 * ((160 * g) // 128)
        col = lax.broadcasted_iota(i32, (RA, 256), 1) + c0
        phit.append(jnp.concatenate(
            [jnp.where((col >= head_lo(g, pp)) & (col < head_lo(g, pp) + DA), urep[:, c0:c0 + 256], 0.0)
             for pp in range(4)], axis=0).astype(bf16))

    with jax.named_scope("wait_wqkv"):
        cp_wqkv.wait()
        cp_x0.wait()
    for g in range(GA):
        c0 = 128 * ((160 * g) // 128)
        wat_ref[0, g] = _pack(_dot_nt(phit[g], wqkv[:, c0:c0 + 256]))
        wat_ref[1, g] = _pack(_dot_nt(phit[g], wqkv[:, D + c0:D + c0 + 256]))
        wat_ref[2, g] = _pack(_dot_nt(perm_mat(g), wqkv[:, 2 * D + c0:2 * D + c0 + 256]))
    init_x(0)
    init_x(1)
    with jax.named_scope("wait_x"):
        cp_x1.wait()

    def transpose_w(n, j):
        t = stage_ref[n, pl.ds(pl.multiple_of(j * TRC, TRC), TRC), :].T
        wb_ref[n, j] = pltpu.bitcast(t, u32)

    def a_phase1(lo, hi, first):
        def body(c, carry):
            if first:
                for n in range(3):
                    cp_w(n, c - 1).wait()
            xn = _unpack(xna_ref[pl.ds(pl.multiple_of(c * (TC // 2), TC // 2), TC // 2), :])
            ones = jnp.ones((8, TC), f32)
            for g in range(GA):
                pq = _dot_nt(_unpack(wat_ref[0, g]), xn)
                pk = _dot_nt(_unpack(wat_ref[1, g]), xn)
                vt = _dot_nt(_unpack(wat_ref[2, g]), xn)
                for pp in range(4):
                    p = 4 * g + pp
                    sl = slice(RA * pp, RA * pp + RA)
                    phiq_ref[c, p] = pltpu.bitcast(_phi(pq[sl]), u32)
                    vext = jnp.concatenate([vt[sl], ones], axis=0).astype(bf16)
                    kv_ref[p] += _dot_nt(vext, _phi(pk[sl]))
                if first and g < 3:
                    transpose_w(g, c - 1)
            if first:
                init_x(jnp.minimum(c + 1, NCH - 1))
            return carry

        lax.fori_loop(lo, hi, body, 0)

    def late_prep():
        cp_woa.wait()
        for n in range(3):
            cp_w(n, NTR - 1).wait()
        for g in range(GA):
            c0 = 128 * ((160 * g) // 128)
            wop_ref[80 * g:80 * g + 80, :] = _pack(_dot(perm_mat(g), wo_a[c0:c0 + 256, :]))
        for n in range(3):
            transpose_w(n, NTR - 1)

    def a_phase2():
        same = ((lax.broadcasted_iota(i32, (RA + 8, 2 * RA), 0) & 1)
                == (lax.broadcasted_iota(i32, (RA + 8, 2 * RA), 1) & 1))
        for p in range(NPA):
            kvm_ref[p] = _pack(jnp.where(same, kv_ref[p], 0.0))

        def body(c, carry):
            ot = []
            for p in range(NPA):
                ne = _dot(_unpack(kvm_ref[p]), _unpack(phiq_ref[c, p]))
                ot.append(ne[0:RA] * _tile5(1.0 / (ne[RA:RA + 8] + 1e-6)))
            o = jnp.concatenate(ot, axis=0).T
            oa_ref[pl.ds(pl.multiple_of(c * (TC // 2), TC // 2), TC // 2), :] = _pack(o)
            return carry

        lax.fori_loop(0, NCH, body, 0, unroll=P2U)

    def a_finish(jr, jw):
        y = _dot(_unpack(oa_ref[pl.ds(pl.multiple_of(jr * 32, 32), 32), :]), _unpack(wop_ref[...]))
        x = x_ref[pl.ds(pl.multiple_of(jr * 64, 64), 64), :] + y
        x_ref[pl.ds(pl.multiple_of(jw * 64, 64), 64), :] = x
        xa_ref[...] = x

    def a_norm(i):
        xnb_ref[8 * i:8 * i + 8, :] = _ln(xa_ref[8 * i:8 * i + 8, :])

    def b_finish(jr, jw, i):
        x = x_ref[pl.ds(pl.multiple_of(jr * 64 + 16 * i, 16), 16), :] + yb_ref[16 * i:16 * i + 16, :]
        x_ref[pl.ds(pl.multiple_of(jw * 64 + 16 * i, 16), 16), :] = x
        xin_ref[pl.ds(pl.multiple_of(jr * 64 + 16 * i, 16), 16), :] = x.astype(bf16)
        xb_ref[16 * i:16 * i + 16, :] = x
        xna_ref[pl.ds(pl.multiple_of(jr * 32 + 8 * i, 8), 8), :] = _pack(_ln(xb_ref[16 * i:16 * i + 16, :]))

    wo32 = wo_ref.bitcast(u32)

    def b_step(h, is_a, side, before_o=None):
        st = {}
        nrow = 16 if is_a else 24

        def proj(p, which):
            c0 = p * PW
            w = wb_ref[which, c0 // TRC, :, c0 % TRC:c0 % TRC + PW]
            y = _dot(h, _unpack(w))
            if is_a:
                sv_ref[which, :, c0:c0 + PW] = y[L:L + 8]
                y = y[0:L]
            else:
                y = jnp.concatenate([y[0:8], sv_ref[which, :, c0:c0 + PW], y[8:32]], axis=0)
            if which == 0:
                st[(p, which)] = (jnp.concatenate([y[:, 0:128], y[:, 256:384]], axis=0).astype(bf16),
                                  y[:, 128:256].astype(bf16))
            else:
                st[(p, which)] = _split(y)

        def do_qk(p):
            st[(p, 'p')] = _probs(st.pop((p, 0)), st.pop((p, 1)))

        def do_pv(p):
            c0 = p * PW
            o = _pv(st.pop((p, 'p')), st.pop((p, 2)))
            if is_a:
                osv_ref[:, c0:c0 + PW] = o[32:L]
                o = o[0:32]
            else:
                o = jnp.concatenate([o, osv_ref[:, c0:c0 + PW]], axis=0)
            o_ref[0:nrow, c0:c0 + PW] = _pack(o)

        def do_o(n):
            k0 = st.get('k', 0)
            k1 = min(k0 + n, HD // 128)
            if k0 == k1:
                return
            st['k'] = k1
            w = jnp.concatenate([wo32[t, k0 * 64:k1 * 64, :] for t in range(D // 128)], axis=1)
            y = _dot(_unpack(o_ref[0:nrow, k0 * 128:k1 * 128]), _unpack(w))
            st['y'] = y if 'y' not in st else st['y'] + y

        o1, o2, o3, olag, f1, f2, f3 = SCH_A if is_a else SCH_B
        for s in range(NPB):
            on = s >= olag
            proj(s, 0)
            if on:
                do_o(o1)
            if s >= 1:
                do_qk(s - 1)
            proj(s, 1)
            if on:
                do_o(o2)
            if s >= 2:
                do_pv(s - 2)
            proj(s, 2)
            if on:
                do_o(o3)
            if s in side:
                side[s]()
            assert st.get('k', 0) <= 3 * max(s - 2, 0)
        if before_o is not None:
            assert 'k' not in st
            before_o()
        do_o(f1)
        do_qk(NPB - 1)
        do_o(f2)
        do_pv(NPB - 2)
        do_o(f3)
        assert st.get('k', 0) <= 3 * (NPB - 2)
        do_pv(NPB - 1)
        do_o(3 * (NPB - 1) - st['k'])
        do_o(3)
        return st['y']

    def layer_b(li):
        mem_ref[...] = mem0[...].astype(f32)
        yb_ref[...] = jnp.zeros(yb_ref.shape, f32)
        a_finish(0, 0)
        for i in range(8):
            a_norm(i)

        @pl.when(li == 0)
        def _():
            for cp in cp_wo:
                cp.wait()

        def body(j, carry):
            @pl.when(jnp.logical_and(li == 1, j >= 2))
            def _():
                cp_out(j - 2, 1).start()

            jp = jnp.maximum(j - 1, 0)
            jw = jnp.where(j == 0, NB, jp)
            side = {2 + 3 * i: functools.partial(b_finish, jp, jw, i) for i in range(4)}
            y = b_step(jnp.concatenate([mem_ref[...], xnb_ref[0:L, :]], axis=0).astype(bf16), True, side)
            h2 = jnp.concatenate([y[0:8], xnb_ref[L:64, :]], axis=0).astype(bf16)
            a_finish(jnp.minimum(j + 1, NB - 1), j + 1)
            yb_ref[0:24, :] = y[8:32]
            side = {3 + i: functools.partial(a_norm, i) for i in range(8)}
            y = b_step(h2, False, side)
            mem_ref[...] = y[0:8]
            yb_ref[32:64, :] = y[8:L]
            yb_ref[24:32, :] = y[L:L + 8]
            return carry

        lax.fori_loop(0, NB, body, 0)
        for i in range(4):
            b_finish(NB - 1, NB - 1, i)

    def layer(li, carry):
        kv_ref[...] = jnp.zeros(kv_ref.shape, f32)
        split = jnp.where(li == 0, 1, NCH)
        with jax.named_scope("a_p1"):
            a_phase1(0, split, False)
        with jax.named_scope("a_p1_first"):
            a_phase1(split, NCH, True)
        with jax.named_scope("a_p2"):
            a_phase2()

        @pl.when(li == 0)
        def _():
            with jax.named_scope("late_prep"):
                late_prep()

        with jax.named_scope("layer_b"):
            layer_b(li)
        return carry

    lax.fori_loop(0, 2, layer, 0)
    cp_out(NB - 2, 2).start()
    cp_out(0, NB).wait()


@jax.jit
def pallas_interleave_layers__linear_kernel_hedgehog__memory_aug_recurrent_mem_tr__prompt_kernel(
    A_x: jax.Array,
    A_wqkv: jax.Array,
    A_w_phi: jax.Array,
    A_wo: jax.Array,
    B_x: jax.Array,
    B_mem0: jax.Array,
    B_Wq: jax.Array,
    B_Wk: jax.Array,
    B_Wv: jax.Array,
    B_Wo: jax.Array,
    B_seg_len: jax.Array,
):
    del B_x, B_seg_len
    x = A_x.reshape(S, D)
    phi = A_w_phi.transpose(1, 2, 0)
    wqt = B_Wq.transpose(1, 2, 0).reshape(HD, D)
    wkt = B_Wk.transpose(1, 2, 0).reshape(HD, D)
    wvt = B_Wv.transpose(1, 2, 0).reshape(HD, D)
    wo = B_Wo.reshape(HD, D)
    vmem = pl.BlockSpec(memory_space=pltpu.VMEM)
    hbm = pl.BlockSpec(memory_space=pl.ANY)
    out = pl.pallas_call(
        _kernel,
        out_shape=jax.ShapeDtypeStruct((S, D), bf16),
        in_specs=[hbm, hbm, vmem, hbm, vmem, hbm, hbm, hbm, hbm],
        out_specs=hbm,
        scratch_shapes=[
            pltpu.VMEM((S, D), bf16),
            pltpu.VMEM((D, 3 * D), bf16),
            pltpu.VMEM((D, D), bf16),
            pltpu.VMEM((S + 64, D), f32),
            pltpu.VMEM((S // 2, D), u32),
            pltpu.VMEM((64, D), f32),
            pltpu.VMEM((64, D), f32),
            pltpu.VMEM((64, D), f32),
            pltpu.VMEM((64, D), f32),
            pltpu.VMEM((S // 2, D), u32),
            pltpu.VMEM((3, GA, 80, D), u32),
            pltpu.VMEM((D // 2, D), u32),
            pltpu.VMEM((NCH, NPA, RA, TC), u32),
            pltpu.VMEM((NPA, RA + 8, 2 * RA), f32),
            pltpu.VMEM((NPA, (RA + 8) // 2, 2 * RA), u32),
            pltpu.VMEM((3, HD, D), bf16),
            pltpu.VMEM((3, NTR, D // 2, TRC), u32),
            pltpu.VMEM((D // 128, HD, 128), bf16),
            pltpu.VMEM((MEM, D), f32),
            pltpu.VMEM((3, 8, HD), f32),
            pltpu.VMEM((8, HD), f32),
            pltpu.VMEM((24, HD), u32),
            pltpu.SemaphoreType.DMA((10 + 3 * NTR,)),
        ],
        compiler_params=pltpu.CompilerParams(vmem_limit_bytes=120 * 1024 * 1024),
    )(x, A_wqkv, phi, A_wo, B_mem0.reshape(MEM, D), wqt, wkt, wvt, wo)
    return out.reshape(1, S, D)
```

```python
import functools
import os

import jax
import jax.numpy as jnp
from jax import lax
import jax.experimental.pallas as pl
import jax.experimental.pallas.tpu as pltpu

f32, bf16, u32, i32 = jnp.float32, jnp.bfloat16, jnp.uint32, jnp.int32

S, D = 2048, 640
HA, DA = 32, 20
NPA = HA // 2
RA = 2 * DA
GA = 4
TC = 256
NCH = S // TC
XCH = 512
HB, DB, MEM, SEG = 32, 192, 8, 32
HD = HB * DB
L = MEM + SEG
NPB = HB // 2
PW = 2 * DB
SCALE = DB ** -0.5
TRC = 768
NTR = HD // TRC
NB = S // 64
assert NTR == NCH

SCH_A = tuple(int(v) for v in os.environ.get("SCH_A", "0,0,0,4,6,6,12").split(","))
SCH_B = tuple(int(v) for v in os.environ.get("SCH_B", "1,0,1,3,1,4,6").split(","))

KVLAG = int(os.environ.get("KVLAG", "12"))
P1U = int(os.environ.get("P1U", "2"))

_NT = (((1,), (1,)), ((), ()))


def _dot(a, b):
    return jnp.dot(a, b, preferred_element_type=f32)


def _dot_nt(a, b):
    return lax.dot_general(a, b, _NT, preferred_element_type=f32)


def _pack(x):
    return pltpu.bitcast(x.astype(bf16), u32)


def _unpack(x):
    return pltpu.bitcast(x, bf16)


def _ln(x):
    m = jnp.mean(x, axis=-1, keepdims=True)
    xc = x - m
    r = lax.rsqrt(jnp.mean(xc * xc, axis=-1, keepdims=True) + 1e-5)
    return x * r - m * r


def _fold(op, p):
    r = p[0:8]
    for j in range(1, 5):
        r = op(r, p[8 * j:8 * j + 8])
    r = op(r, pltpu.roll(r, 2, 0))
    return op(r, pltpu.roll(r, 4, 0))


def _tile5(r):
    return jnp.concatenate([r] * 5, axis=0)


def _phi(p):
    ep = jnp.exp(p - _tile5(_fold(jnp.maximum, p)))
    en = jnp.exp(_tile5(_fold(jnp.minimum, p)) - p)
    ep = ep * _tile5(1.0 / _fold(jnp.add, ep))
    en = en * _tile5(1.0 / _fold(jnp.add, en))
    return jnp.concatenate([ep, en], axis=0).astype(bf16)


def _split(k):
    lo = lax.broadcasted_iota(i32, (L, 128), 1) < 64
    z = jnp.zeros((L, 128), f32)
    mid = k[:, 128:256]
    outer = jnp.concatenate([k[:, 0:128], k[:, 256:384]], axis=0).astype(bf16)
    mid = jnp.concatenate([jnp.where(lo, mid, z), jnp.where(lo, z, mid)], axis=0).astype(bf16)
    return outer, mid


def _probs(q, k):
    r = lax.broadcasted_iota(i32, (L, 2 * L), 0)
    c = lax.broadcasted_iota(i32, (L, 2 * L), 1)
    first = c < L
    so = _dot_nt(q[0], k[0])
    s = jnp.where(first, so[0:L], so[L:2 * L]) + _dot_nt(q[1], k[1])
    s = s * SCALE
    mask = (r < MEM) | (r >= jnp.where(first, c, c - L))
    s = jnp.where(mask, s, -1000000000.0)
    neg = jnp.full_like(s, -jnp.inf)
    ma = jnp.max(jnp.where(first, s, neg), axis=-1, keepdims=True)
    mb = jnp.max(jnp.where(first, neg, s), axis=-1, keepdims=True)
    e = jnp.exp(s - jnp.where(first, ma, mb))
    z = jnp.zeros_like(e)
    ea = jnp.where(first, e, z)
    eb = jnp.where(first, z, e)
    pa = ea * (1.0 / jnp.sum(ea, axis=-1, keepdims=True))
    pb = eb * (1.0 / jnp.sum(eb, axis=-1, keepdims=True))
    return jnp.concatenate([pa, pb], axis=0).astype(bf16), (pa + pb).astype(bf16)


def _pv(p, v):
    oo = _dot(p[0], v[0])
    return jnp.concatenate([oo[0:L], _dot(p[1], v[1]), oo[L:2 * L]], axis=1)


def _kernel(x_hbm, wqkv_hbm, phi_hbm, woa_hbm, mem0_hbm, wqt_hbm, wkt_hbm, wvt_hbm, wo_hbm, out_hbm,
            xin_ref, wqkv, phi_ref, wo_a, mem0, x_ref, xna_ref, xnb_ref, xa_ref, xb_ref, yb_ref, oa_ref,
            wat_ref, wop_ref, phiq_ref, kv_ref, kvm_ref, stage_ref, wb_ref, wo_ref, mem_ref, sv_ref,
            osv_ref, o_ref, sems):
    cp_phi = pltpu.make_async_copy(phi_hbm, phi_ref, sems.at[0])
    cp_mem0 = pltpu.make_async_copy(mem0_hbm, mem0, sems.at[1])
    cp_woa = pltpu.make_async_copy(woa_hbm, wo_a, sems.at[2])
    cp_wqkv = [pltpu.make_async_copy(wqkv_hbm.at[:, pl.ds(D * n, D)], wqkv.at[n], sems.at[4 + n])
               for n in range(3)]
    cp_wo = [pltpu.make_async_copy(wo_hbm.at[:, pl.ds(128 * n, 128)], wo_ref.at[n], sems.at[7 + n])
             for n in range(D // 128)]
    big = (wqt_hbm, wkt_hbm, wvt_hbm)

    def cp_x(j):
        rows = pl.ds(pl.multiple_of(j * XCH, XCH), XCH)
        return pltpu.make_async_copy(x_hbm.at[rows, :], xin_ref.at[rows, :], sems.at[12 + j])

    def cp_w(n, j):
        rows = pl.ds(pl.multiple_of(j * TRC, TRC), TRC)
        return pltpu.make_async_copy(big[n].at[rows, :], stage_ref.at[n, rows, :], sems.at[16 + n * NTR + j])

    def cp_out(j, nblk):
        rows = pl.ds(pl.multiple_of(j * 64, 64), 64 * nblk)
        return pltpu.make_async_copy(xin_ref.at[rows, :], out_hbm.at[rows, :], sems.at[3])

    cp_phi.start()
    for j in range(S // XCH):
        cp_x(j).start()
    for cp in cp_wqkv:
        cp.start()
    cp_mem0.start()
    for j in range(NTR):
        if j == NTR - 1:
            cp_woa.start()
        for n in range(3):
            cp_w(n, j).start()
    for cp in cp_wo:
        cp.start()

    def init_x(c, carry):
        with jax.named_scope("wait_x"):
            cp_x(c).wait()
        x = xin_ref[pl.ds(pl.multiple_of(c * XCH, XCH), XCH), :].astype(f32)
        x_ref[pl.ds(pl.multiple_of(c * XCH, XCH), XCH), :] = x
        xna_ref[pl.ds(pl.multiple_of(c * (XCH // 2), XCH // 2), XCH // 2), :] = _pack(_ln(x))
        return carry

    def head_lo(g, pp):
        return (8 * g + 2 * pp + (lax.broadcasted_iota(i32, (RA, 256), 0) & 1)) * DA

    def perm_mat(g):
        col = lax.broadcasted_iota(i32, (RA, 256), 1) + 128 * ((160 * g) // 128)
        half = lax.broadcasted_iota(i32, (RA, 256), 0) >> 1
        return jnp.concatenate([jnp.where(col == head_lo(g, pp) + half, 1.0, 0.0) for pp in range(4)],
                               axis=0).astype(bf16)

    with jax.named_scope("wait_phi"):
        cp_phi.wait()
    ecol = lax.broadcasted_iota(i32, (HA, D), 1) - DA * lax.broadcasted_iota(i32, (HA, D), 0)
    tp = _dot(phi_ref[0], jnp.where(ecol == 0, 1.0, 0.0).astype(bf16))
    for d in range(1, DA):
        tp = tp + _dot(phi_ref[d], jnp.where(ecol == d, 1.0, 0.0).astype(bf16))
    rep = jnp.where((lax.broadcasted_iota(i32, (RA, DA), 0) >> 1) == lax.broadcasted_iota(i32, (RA, DA), 1),
                    1.0, 0.0).astype(bf16)
    urep = _dot(rep, tp.astype(bf16))
    phit = []
    for g in range(GA):
        c0 = 128 * ((160 * g) // 128)
        col = lax.broadcasted_iota(i32, (RA, 256), 1) + c0
        phit.append(jnp.concatenate(
            [jnp.where((col >= head_lo(g, pp)) & (col < head_lo(g, pp) + DA), urep[:, c0:c0 + 256], 0.0)
             for pp in range(4)], axis=0).astype(bf16))

    with jax.named_scope("init_x"):
        lax.fori_loop(0, S // XCH, init_x, 0)
    with jax.named_scope("prep"):
        for n in range(3):
            with jax.named_scope("wait_wqkv"):
                cp_wqkv[n].wait()
            for g in range(GA):
                c0 = 128 * ((160 * g) // 128)
                lhs = phit[g] if n < 2 else perm_mat(g)
                wat_ref[n, g] = _pack(_dot_nt(lhs, wqkv[n, :, c0:c0 + 256]))
        cp_mem0.wait()

    def transpose_w(n, j):
        t = stage_ref[n, pl.ds(pl.multiple_of(j * TRC, TRC), TRC), :].T
        wb_ref[n, j] = pltpu.bitcast(t, u32)

    def a_phase1(lo, hi, first):
        def body(c, carry):
            if first:
                with jax.named_scope("wait_w"):
                    for n in range(3):
                        cp_w(n, c - 1).wait()
            xn = _unpack(xna_ref[pl.ds(pl.multiple_of(c * (TC // 2), TC // 2), TC // 2), :])
            ones = jnp.ones((8, TC), f32)
            pend = []

            def flush(n):
                while len(pend) > n:
                    p, vext, phik = pend.pop(0)
                    kv_ref[p] += _dot_nt(vext, phik)

            for g in range(GA):
                pq = _dot_nt(_unpack(wat_ref[0, g]), xn)
                flush(KVLAG)
                pk = _dot_nt(_unpack(wat_ref[1, g]), xn)
                vt = _dot_nt(_unpack(wat_ref[2, g]), xn)
                for pp in range(4):
                    p = 4 * g + pp
                    sl = slice(RA * pp, RA * pp + RA)
                    phiq_ref[c, p] = pltpu.bitcast(_phi(pq[sl]), u32)
                    vext = jnp.concatenate([vt[sl], ones], axis=0).astype(bf16)
                    pend.append((p, vext, _phi(pk[sl])))
                if first and g < 3:
                    transpose_w(g, c - 1)
            flush(0)
            return carry

        lax.fori_loop(lo, hi, body, 0, unroll=1 if (first or hi - lo == 1) else P1U)

    def a_phase2(first):
        if first:
            with jax.named_scope("wait_w7"):
                cp_woa.wait()
                for n in range(3):
                    cp_w(n, NTR - 1).wait()
            for g in range(GA):
                c0 = 128 * ((160 * g) // 128)
                wop_ref[80 * g:80 * g + 80, :] = _pack(_dot(perm_mat(g), wo_a[c0:c0 + 256, :]))
        same = ((lax.broadcasted_iota(i32, (RA + 8, 2 * RA), 0) & 1)
                == (lax.broadcasted_iota(i32, (RA + 8, 2 * RA), 1) & 1))
        for p in range(NPA):
            kvm_ref[p] = _pack(jnp.where(same, kv_ref[p], 0.0))

        def attend(c):
            ot = []
            for p in range(NPA):
                ne = _dot(_unpack(kvm_ref[p]), _unpack(phiq_ref[c, p]))
                ot.append(ne[0:RA] * _tile5(1.0 / (ne[RA:RA + 8] + 1e-6)))
            o = jnp.concatenate(ot, axis=0).T
            oa_ref[c * (TC // 2):(c + 1) * (TC // 2), :] = _pack(o)

        def project(c):
            for r in range(c * TC, (c + 1) * TC, 128):
                x_ref[r:r + 128, :] += _dot(_unpack(oa_ref[r // 2:r // 2 + 64, :]), _unpack(wop_ref[...]))

        for c in range(NCH + 1):
            if c < NCH:
                attend(c)
            if first and c >= 1:
                project(c - 1)
            if first and 2 <= c < 5:
                transpose_w(c - 2, NTR - 1)

    def a_finish(jr, jw):
        y = _dot(_unpack(oa_ref[pl.ds(pl.multiple_of(jr * 32, 32), 32), :]), _unpack(wop_ref[...]))
        x = x_ref[pl.ds(pl.multiple_of(jr * 64, 64), 64), :] + y
        x_ref[pl.ds(pl.multiple_of(jw * 64, 64), 64), :] = x
        xa_ref[...] = x

    def a_norm(first, j, i):
        if first:
            x = x_ref[pl.ds(pl.multiple_of(j * 64 + 8 * i, 8), 8), :]
        else:
            x = xa_ref[8 * i:8 * i + 8, :]
        xnb_ref[8 * i:8 * i + 8, :] = _ln(x)

    def b_finish(first, jr, jw, i):
        x = x_ref[pl.ds(pl.multiple_of(jr * 64 + 16 * i, 16), 16), :] + yb_ref[16 * i:16 * i + 16, :]
        if first:
            x_ref[pl.ds(pl.multiple_of(jw * 64 + 16 * i, 16), 16), :] = x
            xb_ref[16 * i:16 * i + 16, :] = x
            xna_ref[pl.ds(pl.multiple_of(jr * 32 + 8 * i, 8), 8), :] = _pack(_ln(xb_ref[16 * i:16 * i + 16, :]))
        else:
            xin_ref[pl.ds(pl.multiple_of(jr * 64 + 16 * i, 16), 16), :] = x.astype(bf16)

    wo32 = wo_ref.bitcast(u32)

    def b_step(h, is_a, side):
        st = {}
        nrow = 16 if is_a else 24

        def proj(p, which):
            c0 = p * PW
            w = wb_ref[which, c0 // TRC, :, c0 % TRC:c0 % TRC + PW]
            y = _dot(h, _unpack(w))
            if is_a:
                sv_ref[which, :, c0:c0 + PW] = y[L:L + 8]
                y = y[0:L]
            else:
                y = jnp.concatenate([y[0:8], sv_ref[which, :, c0:c0 + PW], y[8:32]], axis=0)
            if which == 0:
                st[(p, which)] = (jnp.concatenate([y[:, 0:128], y[:, 256:384]], axis=0).astype(bf16),
                                  y[:, 128:256].astype(bf16))
            else:
                st[(p, which)] = _split(y)

        def do_qk(p):
            st[(p, 'p')] = _probs(st.pop((p, 0)), st.pop((p, 1)))

        def do_pv(p):
            c0 = p * PW
            o = _pv(st.pop((p, 'p')), st.pop((p, 2)))
            if is_a:
                osv_ref[:, c0:c0 + PW] = o[32:L]
                o = o[0:32]
            else:
                o = jnp.concatenate([o, osv_ref[:, c0:c0 + PW]], axis=0)
            o_ref[0:nrow, c0:c0 + PW] = _pack(o)

        def do_o(n):
            k0 = st.get('k', 0)
            k1 = min(k0 + n, HD // 128)
            if k0 == k1:
                return
            st['k'] = k1
            w = jnp.concatenate([wo32[t, k0 * 64:k1 * 64, :] for t in range(D // 128)], axis=1)
            y = _dot(_unpack(o_ref[0:nrow, k0 * 128:k1 * 128]), _unpack(w))
            st['y'] = y if 'y' not in st else st['y'] + y

        o1, o2, o3, olag, f1, f2, f3 = SCH_A if is_a else SCH_B
        for s in range(NPB):
            on = s >= olag
            proj(s, 0)
            if on:
                do_o(o1)
            if s >= 1:
                do_qk(s - 1)
            proj(s, 1)
            if on:
                do_o(o2)
            if s >= 2:
                do_pv(s - 2)
            proj(s, 2)
            if on:
                do_o(o3)
            if s in side:
                side[s]()
            assert st.get('k', 0) <= 3 * max(s - 2, 0)
        do_o(f1)
        do_qk(NPB - 1)
        do_o(f2)
        do_pv(NPB - 2)
        do_o(f3)
        assert st.get('k', 0) <= 3 * (NPB - 2)
        do_pv(NPB - 1)
        do_o(3 * (NPB - 1) - st['k'])
        do_o(3)
        return st['y']

    def layer_b(first):
        mem_ref[...] = mem0[...].astype(f32)
        yb_ref[...] = jnp.zeros(yb_ref.shape, f32)
        if not first:
            a_finish(0, 0)
        for i in range(8):
            a_norm(first, 0, i)
        if first:
            with jax.named_scope("wait_wo"):
                for cp in cp_wo:
                    cp.wait()

        def body(j, carry):
            if not first:
                @pl.when(j >= 2)
                def _():
                    cp_out(j - 2, 1).start()

            jp = jnp.maximum(j - 1, 0)
            jw = jnp.where(j == 0, NB, jp)
            jn = jnp.minimum(j + 1, NB - 1)
            side = {2 + 3 * i: functools.partial(b_finish, first, jp, jw, i) for i in range(4)}
            y = b_step(jnp.concatenate([mem_ref[...], xnb_ref[0:L, :]], axis=0).astype(bf16), True, side)
            h2 = jnp.concatenate([y[0:8], xnb_ref[L:64, :]], axis=0).astype(bf16)
            if not first:
                a_finish(jn, j + 1)
            yb_ref[0:24, :] = y[8:32]
            side = {3 + i: functools.partial(a_norm, first, jn, i) for i in range(8)}
            y = b_step(h2, False, side)
            mem_ref[...] = y[0:8]
            yb_ref[32:64, :] = y[8:L]
            yb_ref[24:32, :] = y[L:L + 8]
            return carry

        with jax.named_scope("b_loop"):
            lax.fori_loop(0, NB, body, 0)
        for i in range(4):
            b_finish(first, NB - 1, NB - 1, i)

    for first in (True, False):
        kv_ref[...] = jnp.zeros(kv_ref.shape, f32)
        with jax.named_scope("a_p1"):
            a_phase1(0, 1 if first else NCH, False)
            if first:
                a_phase1(1, NCH, True)
        with jax.named_scope("a_p2"):
            a_phase2(first)
        with jax.named_scope("layer_b"):
            layer_b(first)

    cp_out(NB - 2, 2).start()
    cp_out(0, NB).wait()


@jax.jit
def pallas_interleave_layers__linear_kernel_hedgehog__memory_aug_recurrent_mem_tr__prompt_kernel(
    A_x: jax.Array,
    A_wqkv: jax.Array,
    A_w_phi: jax.Array,
    A_wo: jax.Array,
    B_x: jax.Array,
    B_mem0: jax.Array,
    B_Wq: jax.Array,
    B_Wk: jax.Array,
    B_Wv: jax.Array,
    B_Wo: jax.Array,
    B_seg_len: jax.Array,
):
    del B_x, B_seg_len
    x = A_x.reshape(S, D)
    phi = A_w_phi.transpose(1, 2, 0)
    wqt = B_Wq.transpose(1, 2, 0).reshape(HD, D)
    wkt = B_Wk.transpose(1, 2, 0).reshape(HD, D)
    wvt = B_Wv.transpose(1, 2, 0).reshape(HD, D)
    wo = B_Wo.reshape(HD, D)
    hbm = pl.BlockSpec(memory_space=pl.ANY)
    out = pl.pallas_call(
        _kernel,
        out_shape=jax.ShapeDtypeStruct((S, D), bf16),
        in_specs=[hbm] * 9,
        out_specs=hbm,
        scratch_shapes=[
            pltpu.VMEM((S, D), bf16),
            pltpu.VMEM((3, D, D), bf16),
            pltpu.VMEM((DA, DA, HA), bf16),
            pltpu.VMEM((D, D), bf16),
            pltpu.VMEM((MEM, D), bf16),
            pltpu.VMEM((S + 64, D), f32),
            pltpu.VMEM((S // 2, D), u32),
            pltpu.VMEM((64, D), f32),
            pltpu.VMEM((64, D), f32),
            pltpu.VMEM((64, D), f32),
            pltpu.VMEM((64, D), f32),
            pltpu.VMEM((S // 2, D), u32),
            pltpu.VMEM((3, GA, 80, D), u32),
            pltpu.VMEM((D // 2, D), u32),
            pltpu.VMEM((NCH, NPA, RA, TC), u32),
            pltpu.VMEM((NPA, RA + 8, 2 * RA), f32),
            pltpu.VMEM((NPA, (RA + 8) // 2, 2 * RA), u32),
            pltpu.VMEM((3, HD, D), bf16),
            pltpu.VMEM((3, NTR, D // 2, TRC), u32),
            pltpu.VMEM((D // 128, HD, 128), bf16),
            pltpu.VMEM((MEM, D), f32),
            pltpu.VMEM((3, 8, HD), f32),
            pltpu.VMEM((8, HD), f32),
            pltpu.VMEM((24, HD), u32),
            pltpu.SemaphoreType.DMA((16 + 3 * NTR,)),
        ],
        compiler_params=pltpu.CompilerParams(vmem_limit_bytes=120 * 1024 * 1024),
    )(x, A_wqkv, phi, A_wo, B_mem0.reshape(MEM, D), wqt, wkt, wvt, wo)
    return out.reshape(1, S, D)
```

```python
import functools
import os

import jax
import jax.numpy as jnp
from jax import lax
import jax.experimental.pallas as pl
import jax.experimental.pallas.tpu as pltpu

f32, bf16, u32, i32 = jnp.float32, jnp.bfloat16, jnp.uint32, jnp.int32

S, D = 2048, 640
HA, DA = 32, 20
NPA = HA // 2
RA = 2 * DA
GA = 4
TC = 256
NCH = S // TC
XCH = 512
HB, DB, MEM, SEG = 32, 192, 8, 32
HD = HB * DB
L = MEM + SEG
NPB = HB // 2
PW = 2 * DB
SCALE = DB ** -0.5
TRC = 768
NTR = HD // TRC
NB = S // 64
assert NTR == NCH

SCH_A = tuple(int(v) for v in os.environ.get("SCH_A", "0,0,0,4,6,6,12").split(","))
SCH_B = tuple(int(v) for v in os.environ.get("SCH_B", "1,0,1,3,1,4,6").split(","))

KVLAG = int(os.environ.get("KVLAG", "12"))
P1U = int(os.environ.get("P1U", "2"))

_NT = (((1,), (1,)), ((), ()))


def _dot(a, b):
    return jnp.dot(a, b, preferred_element_type=f32)


def _dot_nt(a, b):
    return lax.dot_general(a, b, _NT, preferred_element_type=f32)


def _pack(x):
    return pltpu.bitcast(x.astype(bf16), u32)


def _unpack(x):
    return pltpu.bitcast(x, bf16)


def _ln(x):
    m = jnp.mean(x, axis=-1, keepdims=True)
    xc = x - m
    r = lax.rsqrt(jnp.mean(xc * xc, axis=-1, keepdims=True) + 1e-5)
    return x * r - m * r


def _fold(op, p):
    r = p[0:8]
    for j in range(1, 5):
        r = op(r, p[8 * j:8 * j + 8])
    r = op(r, pltpu.roll(r, 2, 0))
    return op(r, pltpu.roll(r, 4, 0))


def _tile5(r):
    return jnp.concatenate([r] * 5, axis=0)


def _phi(p):
    ep = jnp.exp(p - _tile5(_fold(jnp.maximum, p)))
    en = jnp.exp(_tile5(_fold(jnp.minimum, p)) - p)
    ep = ep * _tile5(1.0 / _fold(jnp.add, ep))
    en = en * _tile5(1.0 / _fold(jnp.add, en))
    return jnp.concatenate([ep, en], axis=0).astype(bf16)


def _split(k):
    lo = lax.broadcasted_iota(i32, (L, 128), 1) < 64
    z = jnp.zeros((L, 128), f32)
    mid = k[:, 128:256]
    outer = jnp.concatenate([k[:, 0:128], k[:, 256:384]], axis=0).astype(bf16)
    mid = jnp.concatenate([jnp.where(lo, mid, z), jnp.where(lo, z, mid)], axis=0).astype(bf16)
    return outer, mid


def _probs(q, k):
    r = lax.broadcasted_iota(i32, (L, 2 * L), 0)
    c = lax.broadcasted_iota(i32, (L, 2 * L), 1)
    first = c < L
    so = _dot_nt(q[0], k[0])
    s = jnp.where(first, so[0:L], so[L:2 * L]) + _dot_nt(q[1], k[1])
    s = s * SCALE
    mask = (r < MEM) | (r >= jnp.where(first, c, c - L))
    s = jnp.where(mask, s, -1000000000.0)
    neg = jnp.full_like(s, -jnp.inf)
    ma = jnp.max(jnp.where(first, s, neg), axis=-1, keepdims=True)
    mb = jnp.max(jnp.where(first, neg, s), axis=-1, keepdims=True)
    e = jnp.exp(s - jnp.where(first, ma, mb))
    z = jnp.zeros_like(e)
    ea = jnp.where(first, e, z)
    eb = jnp.where(first, z, e)
    pa = ea * (1.0 / jnp.sum(ea, axis=-1, keepdims=True))
    pb = eb * (1.0 / jnp.sum(eb, axis=-1, keepdims=True))
    return jnp.concatenate([pa, pb], axis=0).astype(bf16), (pa + pb).astype(bf16)


def _pv(p, v):
    oo = _dot(p[0], v[0])
    return jnp.concatenate([oo[0:L], _dot(p[1], v[1]), oo[L:2 * L]], axis=1)


def _kernel(x_hbm, wqkv_hbm, phi_hbm, woa_hbm, mem0_hbm, wqt_hbm, wkt_hbm, wvt_hbm, wo_hbm, out_hbm,
            xin_ref, wqkv, phi_ref, wo_a, mem0, x_ref, xna_ref, xnb_ref, xa_ref, xb_ref, yb_ref, oa_ref,
            wat_ref, lhs_ref, phiq_ref, kv_ref, kvm_ref, stage_ref, wb_ref, wo_ref, mem_ref, sv_ref,
            osv_ref, o_ref, sems):
    cp_phi = pltpu.make_async_copy(phi_hbm, phi_ref, sems.at[0])
    cp_mem0 = pltpu.make_async_copy(mem0_hbm, mem0, sems.at[1])
    cp_woa = pltpu.make_async_copy(woa_hbm, wo_a, sems.at[2])
    cp_wo = [pltpu.make_async_copy(wo_hbm.at[:, pl.ds(128 * n, 128)], wo_ref.at[n], sems.at[7 + n])
             for n in range(D // 128)]
    big = (wqt_hbm, wkt_hbm, wvt_hbm)

    def cp_wqkv(n):
        return pltpu.make_async_copy(wqkv_hbm.at[:, pl.ds(pl.multiple_of(D * n, 128), D)], wqkv.at[n],
                                     sems.at[4 + n])

    def cp_x(j):
        rows = pl.ds(pl.multiple_of(j * XCH, XCH), XCH)
        return pltpu.make_async_copy(x_hbm.at[rows, :], xin_ref.at[rows, :], sems.at[12 + j])

    def cp_w(n, j):
        rows = pl.ds(pl.multiple_of(j * TRC, TRC), TRC)
        return pltpu.make_async_copy(big[n].at[rows, :], stage_ref.at[n, rows, :], sems.at[16 + n * NTR + j])

    def cp_out(j, nblk):
        rows = pl.ds(pl.multiple_of(j * 64, 64), 64 * nblk)
        return pltpu.make_async_copy(xin_ref.at[rows, :], out_hbm.at[rows, :], sems.at[3])

    cp_phi.start()
    for j in range(S // XCH):
        cp_x(j).start()
    for n in range(3):
        cp_wqkv(n).start()
    cp_mem0.start()
    for j in range(NTR):
        if j == NTR - 1:
            cp_woa.start()
        for n in range(3):
            cp_w(n, j).start()
    for cp in cp_wo:
        cp.start()

    def init_x(c, carry):
        with jax.named_scope("wait_x"):
            cp_x(c).wait()
        x = xin_ref[pl.ds(pl.multiple_of(c * XCH, XCH), XCH), :].astype(f32)
        x_ref[pl.ds(pl.multiple_of(c * XCH, XCH), XCH), :] = x
        xna_ref[pl.ds(pl.multiple_of(c * (XCH // 2), XCH // 2), XCH // 2), :] = _pack(_ln(x))
        return carry

    with jax.named_scope("wait_phi"):
        cp_phi.wait()
    ecol = lax.broadcasted_iota(i32, (HA, D), 1) - DA * lax.broadcasted_iota(i32, (HA, D), 0)
    tp = _dot(phi_ref[0], jnp.where(ecol == 0, 1.0, 0.0).astype(bf16))
    for d in range(1, DA):
        tp = tp + _dot(phi_ref[d], jnp.where(ecol == d, 1.0, 0.0).astype(bf16))
    rep = jnp.where((lax.broadcasted_iota(i32, (RA, DA), 0) >> 1) == lax.broadcasted_iota(i32, (RA, DA), 1),
                    1.0, 0.0).astype(bf16)
    urep = _dot(rep, tp.astype(bf16))
    for g in range(GA):
        col = lax.broadcasted_iota(i32, (RA, 256), 1) + 128 * g
        par = lax.broadcasted_iota(i32, (RA, 256), 0) & 1
        for pp in range(4):
            lo = (8 * g + 2 * pp + par) * DA
            blk = jnp.where((col >= lo) & (col < lo + DA), urep[:, 128 * g:128 * g + 256], 0.0)
            lhs_ref[0, g, RA * pp:RA * pp + RA, :] = blk
        lhs_ref[1, g] = jnp.where(lax.broadcasted_iota(i32, (160, 256), 1) + 128 * g
                                  == lax.broadcasted_iota(i32, (160, 256), 0) + 160 * g, 1.0, 0.0)

    with jax.named_scope("init_x"):
        lax.fori_loop(0, S // XCH, init_x, 0)

    def prep(n, carry):
        with jax.named_scope("wait_wqkv"):
            cp_wqkv(n).wait()
        for g in range(GA):
            wat_ref[n, g] = _pack(_dot_nt(lhs_ref[n // 2, g].astype(bf16), wqkv[n, :, 128 * g:128 * g + 256]))
        return carry

    with jax.named_scope("prep"):
        lax.fori_loop(0, 3, prep, 0)
        cp_mem0.wait()

    def transpose_w(n, p):
        t = stage_ref[n, pl.ds(pl.multiple_of(p * PW, PW), PW), :].T
        wb_ref[n, p] = pltpu.bitcast(t, u32)

    def a_phase1(first):
        def body(c, carry):
            if first:
                ct = jnp.where(c == 0, NTR, c - 1)

                @pl.when(c > 0)
                def _():
                    with jax.named_scope("wait_w"):
                        for n in range(3):
                            cp_w(n, c - 1).wait()

            xn = _unpack(xna_ref[pl.ds(pl.multiple_of(c * (TC // 2), TC // 2), TC // 2), :])
            ones = jnp.ones((8, TC), f32)
            pend = []

            def flush(n):
                while len(pend) > n:
                    p, vext, phik = pend.pop(0)
                    kv_ref[p] += _dot_nt(vext, phik)

            for g in range(GA):
                pq = _dot_nt(_unpack(wat_ref[0, g]), xn)
                flush(KVLAG)
                pk = _dot_nt(_unpack(wat_ref[1, g]), xn)
                vt = _dot_nt(_unpack(wat_ref[2, g]), xn)
                for pp in range(4):
                    p = 4 * g + pp
                    sl = slice(RA * pp, RA * pp + RA)
                    phiq_ref[c, p] = pltpu.bitcast(_phi(pq[sl]), u32)
                    vext = jnp.concatenate([vt[sl], ones], axis=0).astype(bf16)
                    pend.append((p, vext, _phi(pk[sl])))
                if first and g < 3:
                    transpose_w(g, 2 * ct)
                    transpose_w(g, 2 * ct + 1)
            flush(0)
            return carry

        lax.fori_loop(0, NCH, body, 0, unroll=1 if first else P1U)

    def a_phase2(first):
        r = lax.broadcasted_iota(i32, (RA + 8, 2 * RA), 0)
        rb = jnp.where(((r >= DA) & (r < RA)) | (r >= RA + 4), 1, 0)
        same = rb == (lax.broadcasted_iota(i32, (RA + 8, 2 * RA), 1) & 1)
        for p in range(NPA):
            kvm_ref[p] = _pack(jnp.where(same, kv_ref[p], 0.0))

        def attend(c):
            top = lax.broadcasted_iota(i32, (8, TC), 0) < 4
            ot = []
            for p in range(NPA):
                ne = _dot(_unpack(kvm_ref[p]), _unpack(phiq_ref[c, p]))
                rc = 1.0 / (ne[RA:RA + 8] + 1e-6)
                sw = pltpu.roll(rc, 4, 0)
                ra, rb = jnp.where(top, rc, sw), jnp.where(top, sw, rc)
                ot.append(ne[0:RA] * jnp.concatenate([ra, ra, rc, rb, rb], axis=0))
            o = jnp.concatenate(ot, axis=0).T
            oa_ref[pl.ds(pl.multiple_of(c * (TC // 2), TC // 2), TC // 2), :] = _pack(o)

        if not first:
            for c in range(NCH):
                attend(c)
            return

        attend(0)
        with jax.named_scope("wait_w7"):
            cp_woa.wait()
            for n in range(3):
                cp_w(n, NTR - 1).wait()

        def body(c, carry):
            lhs = [_unpack(oa_ref[pl.ds(pl.multiple_of(c * (TC // 2) + r // 2, 64), 64), :])
                   for r in range(0, TC, 128)]
            attend(jnp.minimum(c + 1, NCH - 1))
            t = jnp.minimum(c, 5)
            transpose_w(t // 2, NPB - 2 + t % 2)
            for r in range(0, TC, 128):
                x_ref[pl.ds(pl.multiple_of(c * TC + r, 128), 128), :] += _dot(lhs[r // 128], wo_a[...])
            return carry

        lax.fori_loop(0, NCH, body, 0)

    def a_finish(jr, jw):
        y = _dot(_unpack(oa_ref[pl.ds(pl.multiple_of(jr * 32, 32), 32), :]), wo_a[...])
        x = x_ref[pl.ds(pl.multiple_of(jr * 64, 64), 64), :] + y
        x_ref[pl.ds(pl.multiple_of(jw * 64, 64), 64), :] = x
        xa_ref[...] = x

    def a_norm(first, j, i):
        if first:
            x = x_ref[pl.ds(pl.multiple_of(j * 64 + 8 * i, 8), 8), :]
        else:
            x = xa_ref[8 * i:8 * i + 8, :]
        xnb_ref[8 * i:8 * i + 8, :] = _ln(x)

    def b_finish(first, jr, jw, i):
        x = x_ref[pl.ds(pl.multiple_of(jr * 64 + 16 * i, 16), 16), :] + yb_ref[16 * i:16 * i + 16, :]
        if first:
            x_ref[pl.ds(pl.multiple_of(jw * 64 + 16 * i, 16), 16), :] = x
            xb_ref[16 * i:16 * i + 16, :] = x
            xna_ref[pl.ds(pl.multiple_of(jr * 32 + 8 * i, 8), 8), :] = _pack(_ln(xb_ref[16 * i:16 * i + 16, :]))
        else:
            xin_ref[pl.ds(pl.multiple_of(jr * 64 + 16 * i, 16), 16), :] = x.astype(bf16)

    wo32 = wo_ref.bitcast(u32)

    def b_step(h, is_a, side):
        st = {}
        nrow = 16 if is_a else 24

        def proj(p, which):
            c0 = p * PW
            y = _dot(h, _unpack(wb_ref[which, p]))
            if is_a:
                sv_ref[which, :, c0:c0 + PW] = y[L:L + 8]
                y = y[0:L]
            else:
                y = jnp.concatenate([y[0:8], sv_ref[which, :, c0:c0 + PW], y[8:32]], axis=0)
            if which == 0:
                st[(p, which)] = (jnp.concatenate([y[:, 0:128], y[:, 256:384]], axis=0).astype(bf16),
                                  y[:, 128:256].astype(bf16))
            else:
                st[(p, which)] = _split(y)

        def do_qk(p):
            st[(p, 'p')] = _probs(st.pop((p, 0)), st.pop((p, 1)))

        def do_pv(p):
            c0 = p * PW
            o = _pv(st.pop((p, 'p')), st.pop((p, 2)))
            if is_a:
                osv_ref[:, c0:c0 + PW] = o[32:L]
                o = o[0:32]
            else:
                o = jnp.concatenate([o, osv_ref[:, c0:c0 + PW]], axis=0)
            o_ref[0:nrow, c0:c0 + PW] = _pack(o)

        def do_o(n):
            k0 = st.get('k', 0)
            k1 = min(k0 + n, HD // 128)
            if k0 == k1:
                return
            st['k'] = k1
            w = jnp.concatenate([wo32[t, k0 * 64:k1 * 64, :] for t in range(D // 128)], axis=1)
            y = _dot(_unpack(o_ref[0:nrow, k0 * 128:k1 * 128]), _unpack(w))
            st['y'] = y if 'y' not in st else st['y'] + y

        o1, o2, o3, olag, f1, f2, f3 = SCH_A if is_a else SCH_B
        for s in range(NPB):
            on = s >= olag
            proj(s, 0)
            if on:
                do_o(o1)
            if s >= 1:
                do_qk(s - 1)
            proj(s, 1)
            if on:
                do_o(o2)
            if s >= 2:
                do_pv(s - 2)
            proj(s, 2)
            if on:
                do_o(o3)
            if s in side:
                side[s]()
            assert st.get('k', 0) <= 3 * max(s - 2, 0)
        do_o(f1)
        do_qk(NPB - 1)
        do_o(f2)
        do_pv(NPB - 2)
        do_o(f3)
        assert st.get('k', 0) <= 3 * (NPB - 2)
        do_pv(NPB - 1)
        do_o(3 * (NPB - 1) - st['k'])
        do_o(3)
        return st['y']

    def layer_b(first):
        mem_ref[...] = mem0[...].astype(f32)
        yb_ref[...] = jnp.zeros(yb_ref.shape, f32)
        if not first:
            a_finish(0, 0)
        for i in range(8):
            a_norm(first, 0, i)
        if first:
            with jax.named_scope("wait_wo"):
                for cp in cp_wo:
                    cp.wait()

        def body(j, carry):
            if not first:
                @pl.when(j >= 2)
                def _():
                    cp_out(j - 2, 1).start()

            jp = jnp.maximum(j - 1, 0)
            jw = jnp.where(j == 0, NB, jp)
            jn = jnp.minimum(j + 1, NB - 1)
            side = {2 + 3 * i: functools.partial(b_finish, first, jp, jw, i) for i in range(4)}
            y = b_step(jnp.concatenate([mem_ref[...], xnb_ref[0:L, :]], axis=0).astype(bf16), True, side)
            h2 = jnp.concatenate([y[0:8], xnb_ref[L:64, :]], axis=0).astype(bf16)
            if not first:
                a_finish(jn, j + 1)
            yb_ref[0:24, :] = y[8:32]
            side = {3 + i: functools.partial(a_norm, first, jn, i) for i in range(8)}
            y = b_step(h2, False, side)
            mem_ref[...] = y[0:8]
            yb_ref[32:64, :] = y[8:L]
            yb_ref[24:32, :] = y[L:L + 8]
            return carry

        with jax.named_scope("b_loop"):
            lax.fori_loop(0, NB, body, 0)
        for i in range(4):
            b_finish(first, NB - 1, NB - 1, i)

    for first in (True, False):
        kv_ref[...] = jnp.zeros(kv_ref.shape, f32)
        with jax.named_scope("a_p1"):
            a_phase1(first)
        with jax.named_scope("a_p2"):
            a_phase2(first)
        with jax.named_scope("layer_b"):
            layer_b(first)

    cp_out(NB - 2, 2).start()
    cp_out(0, NB).wait()


@jax.jit
def pallas_interleave_layers__linear_kernel_hedgehog__memory_aug_recurrent_mem_tr__prompt_kernel(
    A_x: jax.Array,
    A_wqkv: jax.Array,
    A_w_phi: jax.Array,
    A_wo: jax.Array,
    B_x: jax.Array,
    B_mem0: jax.Array,
    B_Wq: jax.Array,
    B_Wk: jax.Array,
    B_Wv: jax.Array,
    B_Wo: jax.Array,
    B_seg_len: jax.Array,
):
    del B_x, B_seg_len
    x = A_x.reshape(S, D)
    phi = A_w_phi.transpose(1, 2, 0)
    wqt = B_Wq.transpose(1, 2, 0).reshape(HD, D)
    wkt = B_Wk.transpose(1, 2, 0).reshape(HD, D)
    wvt = B_Wv.transpose(1, 2, 0).reshape(HD, D)
    wo = B_Wo.reshape(HD, D)
    hbm = pl.BlockSpec(memory_space=pl.ANY)
    out = pl.pallas_call(
        _kernel,
        out_shape=jax.ShapeDtypeStruct((S, D), bf16),
        in_specs=[hbm] * 9,
        out_specs=hbm,
        scratch_shapes=[
            pltpu.VMEM((S, D), bf16),
            pltpu.VMEM((3, D, D), bf16),
            pltpu.VMEM((DA, DA, HA), bf16),
            pltpu.VMEM((D, D), bf16),
            pltpu.VMEM((MEM, D), bf16),
            pltpu.VMEM((S + 64, D), f32),
            pltpu.VMEM((S // 2, D), u32),
            pltpu.VMEM((64, D), f32),
            pltpu.VMEM((64, D), f32),
            pltpu.VMEM((64, D), f32),
            pltpu.VMEM((64, D), f32),
            pltpu.VMEM((S // 2, D), u32),
            pltpu.VMEM((3, GA, 80, D), u32),
            pltpu.VMEM((2, GA, 160, 256), f32),
            pltpu.VMEM((NCH, NPA, RA, TC), u32),
            pltpu.VMEM((NPA, RA + 8, 2 * RA), f32),
            pltpu.VMEM((NPA, (RA + 8) // 2, 2 * RA), u32),
            pltpu.VMEM((3, HD + TRC, D), bf16),
            pltpu.VMEM((3, NPB + 2, D // 2, PW), u32),
            pltpu.VMEM((D // 128, HD, 128), bf16),
            pltpu.VMEM((MEM, D), f32),
            pltpu.VMEM((3, 8, HD), f32),
            pltpu.VMEM((8, HD), f32),
            pltpu.VMEM((24, HD), u32),
            pltpu.SemaphoreType.DMA((16 + 3 * NTR,)),
        ],
        compiler_params=pltpu.CompilerParams(vmem_limit_bytes=120 * 1024 * 1024),
    )(x, A_wqkv, phi, A_wo, B_mem0.reshape(MEM, D), wqt, wkt, wvt, wo)
    return out.reshape(1, S, D)
```

```python
import functools
import os

import jax
import jax.numpy as jnp
from jax import lax
import jax.experimental.pallas as pl
import jax.experimental.pallas.tpu as pltpu

f32, bf16, u32, i32 = jnp.float32, jnp.bfloat16, jnp.uint32, jnp.int32

S, D = 2048, 640
HA, DA = 32, 20
NPA = HA // 2
RA = 2 * DA
GA = 4
TC = 256
NCH = S // TC
XCH = 512
HB, DB, MEM, SEG = 32, 192, 8, 32
HD = HB * DB
L = MEM + SEG
NPB = HB // 2
PW = 2 * DB
SCALE = DB ** -0.5
TRC = 768
NTR = HD // TRC
NSEG = S // SEG
SPI = int(os.environ.get("SPI", "2"))
NB = NSEG // SPI
assert NTR == NCH

SCH = tuple(int(v) for v in os.environ.get("SCH", "1,0,1,3,1,4,6").split(","))
OUTER_BF16 = int(os.environ.get("OUTER_BF16", "1"))
KVLAG = int(os.environ.get("KVLAG", "12"))
P1U = int(os.environ.get("P1U", "2"))

_NN = (((1,), (0,)), ((), ()))
_NT = (((1,), (1,)), ((), ()))


def _dot(a, b):
    return lax.dot_general(a, b, _NN, preferred_element_type=f32)


def _dot_nt(a, b):
    return lax.dot_general(a, b, _NT, preferred_element_type=f32)


def _pack(x):
    return pltpu.bitcast(x.astype(bf16), u32)


def _unpack(x):
    return pltpu.bitcast(x, bf16)


def _lhs(x):
    return x.astype(bf16) if OUTER_BF16 else x


def _ln(x):
    m = jnp.mean(x, axis=-1, keepdims=True)
    xc = x - m
    r = lax.rsqrt(jnp.mean(xc * xc, axis=-1, keepdims=True) + 1e-5)
    return x * r - m * r


def _fold(op, p):
    r = p[0:8]
    for j in range(1, 5):
        r = op(r, p[8 * j:8 * j + 8])
    r = op(r, pltpu.roll(r, 2, 0))
    return op(r, pltpu.roll(r, 4, 0))


def _tile5(r):
    return jnp.concatenate([r] * 5, axis=0)


def _phi(p):
    ep = jnp.exp(p - _tile5(_fold(jnp.maximum, p)))
    en = jnp.exp(_tile5(_fold(jnp.minimum, p)) - p)
    ep = ep * _tile5(1.0 / _fold(jnp.add, ep))
    en = en * _tile5(1.0 / _fold(jnp.add, en))
    return jnp.concatenate([ep, en], axis=0).astype(bf16)


def _split(k):
    lo = lax.broadcasted_iota(i32, (L, 128), 1) < 64
    z = jnp.zeros((L, 128), f32)
    mid = k[:, 128:256]
    outer = jnp.concatenate([k[:, 0:128], k[:, 256:384]], axis=0).astype(bf16)
    mid = jnp.concatenate([jnp.where(lo, mid, z), jnp.where(lo, z, mid)], axis=0).astype(bf16)
    return outer, mid


def _probs(q, k):
    r = lax.broadcasted_iota(i32, (L, 2 * L), 0)
    c = lax.broadcasted_iota(i32, (L, 2 * L), 1)
    first = c < L
    so = _dot_nt(q[0], k[0])
    s = jnp.where(first, so[0:L], so[L:2 * L]) + _dot_nt(q[1], k[1])
    s = s * SCALE
    mask = (r < MEM) | (r >= jnp.where(first, c, c - L))
    s = jnp.where(mask, s, -1000000000.0)
    neg = jnp.full_like(s, -jnp.inf)
    ma = jnp.max(jnp.where(first, s, neg), axis=-1, keepdims=True)
    mb = jnp.max(jnp.where(first, neg, s), axis=-1, keepdims=True)
    e = jnp.exp(s - jnp.where(first, ma, mb))
    z = jnp.zeros_like(e)
    ea = jnp.where(first, e, z)
    eb = jnp.where(first, z, e)
    pa = ea * (1.0 / jnp.sum(ea, axis=-1, keepdims=True))
    pb = eb * (1.0 / jnp.sum(eb, axis=-1, keepdims=True))
    return _lhs(jnp.concatenate([pa, pb], axis=0)), pa + pb


def _pv(p, v):
    oo = _dot(p[0], v[0])
    return jnp.concatenate([oo[0:L], _dot(p[1], v[1]), oo[L:2 * L]], axis=1)


def _kernel(x_hbm, wqkv_hbm, phi_hbm, woa_hbm, mem0_hbm, wqt_hbm, wkt_hbm, wvt_hbm, wo_hbm, out_hbm,
            xin_ref, wqkv, phi_ref, wo_a, mem0, x_ref, xna_ref, xnb_ref, xa_ref, xb_ref, yb_ref, oa_ref,
            wat_ref, wop_ref, lhs_ref, phiq_ref, kv_ref, kvm_ref, stage_ref, wb_ref, wo_ref, mem_ref, o_ref,
            sems):
    cp_phi = pltpu.make_async_copy(phi_hbm, phi_ref, sems.at[0])
    cp_mem0 = pltpu.make_async_copy(mem0_hbm, mem0, sems.at[1])
    cp_woa = pltpu.make_async_copy(woa_hbm, wo_a, sems.at[2])
    cp_wo = [pltpu.make_async_copy(wo_hbm.at[:, pl.ds(128 * n, 128)], wo_ref.at[n], sems.at[7 + n])
             for n in range(D // 128)]
    big = (wqt_hbm, wkt_hbm, wvt_hbm)

    def cp_wqkv(n):
        return pltpu.make_async_copy(wqkv_hbm.at[:, pl.ds(pl.multiple_of(D * n, 128), D)], wqkv.at[n],
                                     sems.at[4 + n])

    def cp_x(j):
        rows = pl.ds(pl.multiple_of(j * XCH, XCH), XCH)
        return pltpu.make_async_copy(x_hbm.at[rows, :], xin_ref.at[rows, :], sems.at[12 + j])

    def cp_w(n, j):
        rows = pl.ds(pl.multiple_of(j * TRC, TRC), TRC)
        return pltpu.make_async_copy(big[n].at[rows, :], stage_ref.at[n, rows, :], sems.at[16 + n * NTR + j])

    def cp_out(j, nblk):
        rows = pl.ds(pl.multiple_of(j * SPI * SEG, SEG), SPI * SEG * nblk)
        return pltpu.make_async_copy(xin_ref.at[rows, :], out_hbm.at[rows, :], sems.at[3])

    cp_phi.start()
    for j in range(S // XCH):
        cp_x(j).start()
    for n in range(3):
        cp_wqkv(n).start()
    cp_mem0.start()
    for j in range(NTR):
        if j == NTR - 1:
            cp_woa.start()
        for n in range(3):
            cp_w(n, j).start()
    for cp in cp_wo:
        cp.start()

    def init_x(c, carry):
        with jax.named_scope("wait_x"):
            cp_x(c).wait()
        x = xin_ref[pl.ds(pl.multiple_of(c * XCH, XCH), XCH), :].astype(f32)
        x_ref[pl.ds(pl.multiple_of(c * XCH, XCH), XCH), :] = x
        xna_ref[pl.ds(pl.multiple_of(c * (XCH // 2), XCH // 2), XCH // 2), :] = _pack(_ln(x))
        return carry

    with jax.named_scope("wait_phi"):
        cp_phi.wait()
    ecol = lax.broadcasted_iota(i32, (HA, D), 1) - DA * lax.broadcasted_iota(i32, (HA, D), 0)
    tp = _dot(phi_ref[0], jnp.where(ecol == 0, 1.0, 0.0).astype(bf16))
    for d in range(1, DA):
        tp = tp + _dot(phi_ref[d], jnp.where(ecol == d, 1.0, 0.0).astype(bf16))
    rep = jnp.where((lax.broadcasted_iota(i32, (RA, DA), 0) >> 1) == lax.broadcasted_iota(i32, (RA, DA), 1),
                    1.0, 0.0).astype(bf16)
    urep = _dot(rep, tp.astype(bf16))
    for g in range(GA):
        col = lax.broadcasted_iota(i32, (RA, 256), 1) + 128 * g
        par = lax.broadcasted_iota(i32, (RA, 256), 0) & 1
        for pp in range(4):
            lo = (8 * g + 2 * pp + par) * DA
            blk = jnp.where((col >= lo) & (col < lo + DA), urep[:, 128 * g:128 * g + 256], 0.0)
            lhs_ref[0, g, RA * pp:RA * pp + RA, :] = blk
        lhs_ref[1, g] = jnp.where(lax.broadcasted_iota(i32, (160, 256), 1) + 128 * g
                                  == lax.broadcasted_iota(i32, (160, 256), 0) + 160 * g, 1.0, 0.0)

    with jax.named_scope("init_x"):
        lax.fori_loop(0, S // XCH, init_x, 0)

    def prep(n, carry):
        with jax.named_scope("wait_wqkv"):
            cp_wqkv(n).wait()
        for g in range(GA):
            wat_ref[n, g] = _pack(_dot_nt(lhs_ref[n // 2, g].astype(bf16), wqkv[n, :, 128 * g:128 * g + 256]))
        return carry

    with jax.named_scope("prep"):
        lax.fori_loop(0, 3, prep, 0)
        cp_mem0.wait()

    def transpose_w(n, p):
        t = stage_ref[n, pl.ds(pl.multiple_of(p * PW, PW), PW), :].T
        wb_ref[n, p] = pltpu.bitcast(t, u32)

    def a_phase1(first):
        def body(c, carry):
            if first:
                ct = jnp.where(c == 0, NTR, c - 1)

                @pl.when(c > 0)
                def _():
                    with jax.named_scope("wait_w"):
                        for n in range(3):
                            cp_w(n, c - 1).wait()

            xn = _unpack(xna_ref[pl.ds(pl.multiple_of(c * (TC // 2), TC // 2), TC // 2), :])
            ones = jnp.ones((8, TC), f32)
            pend = []

            def flush(n):
                while len(pend) > n:
                    p, vext, phik = pend.pop(0)
                    kv_ref[p] += _dot_nt(vext, phik)

            for g in range(GA):
                pq = _dot_nt(_unpack(wat_ref[0, g]), xn)
                flush(KVLAG)
                pk = _dot_nt(_unpack(wat_ref[1, g]), xn)
                vt = _dot_nt(_unpack(wat_ref[2, g]), xn)
                for pp in range(4):
                    p = 4 * g + pp
                    sl = slice(RA * pp, RA * pp + RA)
                    phiq_ref[c, p] = pltpu.bitcast(_phi(pq[sl]), u32)
                    vext = jnp.concatenate([vt[sl], ones], axis=0).astype(bf16)
                    pend.append((p, vext, _phi(pk[sl])))
                if first and g < 3:
                    transpose_w(g, 2 * ct)
                    transpose_w(g, 2 * ct + 1)
            flush(0)
            return carry

        lax.fori_loop(0, NCH, body, 0, unroll=1 if first else P1U)

    def a_phase2(first):
        r = lax.broadcasted_iota(i32, (RA + 8, 2 * RA), 0)
        rb = jnp.where(((r >= DA) & (r < RA)) | (r >= RA + 4), 1, 0)
        same = rb == (lax.broadcasted_iota(i32, (RA + 8, 2 * RA), 1) & 1)
        for p in range(NPA):
            kvm_ref[p] = _pack(jnp.where(same, kv_ref[p], 0.0))

        def attend(c):
            top = lax.broadcasted_iota(i32, (8, TC), 0) < 4
            ot = []
            for p in range(NPA):
                ne = _dot(_unpack(kvm_ref[p]), _unpack(phiq_ref[c, p]))
                rc = 1.0 / (ne[RA:RA + 8] + 1e-6)
                sw = pltpu.roll(rc, 4, 0)
                ra, rb = jnp.where(top, rc, sw), jnp.where(top, sw, rc)
                ot.append(ne[0:RA] * jnp.concatenate([ra, ra, rc, rb, rb], axis=0))
            o = jnp.concatenate(ot, axis=0).T
            oa_ref[pl.ds(pl.multiple_of(c * (TC // 2), TC // 2), TC // 2), :] = _pack(o)

        if not first:
            for c in range(NCH):
                attend(c)
            return

        attend(0)
        with jax.named_scope("wait_w7"):
            cp_woa.wait()
            for n in range(3):
                cp_w(n, NTR - 1).wait()

        def body(c, carry):
            lhs = [_unpack(oa_ref[pl.ds(pl.multiple_of(c * (TC // 2) + r // 2, 64), 64), :])
                   for r in range(0, TC, 128)]
            attend(jnp.minimum(c + 1, NCH - 1))
            t = jnp.minimum(c, 5)
            transpose_w(t // 2, NPB - 2 + t % 2)
            for r in range(0, TC, 128):
                x_ref[pl.ds(pl.multiple_of(c * TC + r, 128), 128), :] += _dot(lhs[r // 128], wo_a[...])
            return carry

        lax.fori_loop(0, NCH, body, 0)

    def seg_rows(sg, off=0, n=SEG):
        return pl.ds(pl.multiple_of(sg * SEG + off, 8), n)

    def a_finish(sr, sw):
        y = _dot(_unpack(oa_ref[pl.ds(pl.multiple_of(sr * (SEG // 2), SEG // 2), SEG // 2), :]),
                 _unpack(wop_ref[...]))
        x = x_ref[seg_rows(sr), :] + y
        x_ref[seg_rows(sw), :] = x
        xa_ref[...] = x

    def a_norm(first, sg, slot, i):
        x = x_ref[seg_rows(sg, 8 * i, 8), :] if first else xa_ref[8 * i:8 * i + 8, :]
        xnb_ref[slot, 8 * i:8 * i + 8, :] = _ln(x)

    def b_finish(first, sr, sw, slot, i):
        x = x_ref[seg_rows(sr, 16 * i, 16), :] + yb_ref[slot, 16 * i:16 * i + 16, :]
        if first:
            x_ref[seg_rows(sw, 16 * i, 16), :] = x
            xb_ref[16 * i:16 * i + 16, :] = x
            xna_ref[pl.ds(pl.multiple_of(sr * (SEG // 2) + 8 * i, 8), 8), :] = _pack(
                _ln(xb_ref[16 * i:16 * i + 16, :]))
        else:
            xin_ref[pl.ds(pl.multiple_of(sr * SEG + 16 * i, 16), 16), :] = x.astype(bf16)

    wo32 = wo_ref.bitcast(u32)

    def b_step(h, side):
        st = {}

        def proj(p, which):
            y = _dot(h, _unpack(wb_ref[which, p]))
            if which == 0:
                st[(p, which)] = (_lhs(jnp.concatenate([y[:, 0:128], y[:, 256:384]], axis=0)), y[:, 128:256])
            else:
                st[(p, which)] = _split(y)

        def do_qk(p):
            st[(p, 'p')] = _probs(st.pop((p, 0)), st.pop((p, 1)))

        def do_pv(p):
            o_ref[:, p * PW:(p + 1) * PW] = _pv(st.pop((p, 'p')), st.pop((p, 2)))

        def do_o(n):
            k0 = st.get('k', 0)
            k1 = min(k0 + n, HD // 128)
            if k0 == k1:
                return
            st['k'] = k1
            w = jnp.concatenate([wo32[t, k0 * 64:k1 * 64, :] for t in range(D // 128)], axis=1)
            y = _dot(o_ref[:, k0 * 128:k1 * 128], _unpack(w))
            st['y'] = y if 'y' not in st else st['y'] + y

        o1, o2, o3, olag, f1, f2, f3 = SCH
        for s in range(NPB):
            on = s >= olag
            proj(s, 0)
            if on:
                do_o(o1)
            if s >= 1:
                do_qk(s - 1)
            proj(s, 1)
            if on:
                do_o(o2)
            if s >= 2:
                do_pv(s - 2)
            proj(s, 2)
            if on:
                do_o(o3)
            if s in side:
                side[s]()
            assert st.get('k', 0) <= 3 * max(s - 2, 0)
        do_o(f1)
        do_qk(NPB - 1)
        do_o(f2)
        do_pv(NPB - 2)
        do_o(f3)
        assert st.get('k', 0) <= 3 * (NPB - 2)
        do_pv(NPB - 1)
        do_o(3 * (NPB - 1) - st['k'])
        do_o(3)
        return st['y']

    def layer_b(first):
        mem_ref[...] = mem0[...].astype(f32)
        yb_ref[1] = jnp.zeros((SEG, D), f32)
        if not first:
            a_finish(0, 0)
        for i in range(4):
            a_norm(first, 0, 0, i)
        if first:
            wop_ref[...] = pltpu.bitcast(wo_a[...], u32)
            with jax.named_scope("wait_wo"):
                for cp in cp_wo:
                    cp.wait()

        def body(j, carry):
            if not first:
                @pl.when(j >= 2)
                def _():
                    cp_out(j - 2, 1).start()

            mem = mem_ref[...]
            for t in range(SPI):
                sg = j * SPI + t
                sp = jnp.maximum(sg - 1, 0) if t == 0 else sg - 1
                sw = jnp.where(sg == 0, NSEG, sp) if t == 0 else sp
                sn = jnp.minimum(sg + 1, NSEG - 1) if t == SPI - 1 else sg + 1
                h = jnp.concatenate([mem, xnb_ref[t % 2]], axis=0)
                if not first:
                    a_finish(sn, sg + 1)
                side = {2 + 2 * i: functools.partial(b_finish, first, sp, sw, (t + 1) % 2, i) for i in range(2)}
                side.update({6 + 2 * i: functools.partial(a_norm, first, sn, (t + 1) % 2, i) for i in range(4)})
                y = b_step(h, side)
                mem = y[0:MEM]
                yb_ref[t % 2] = y[MEM:L]
            mem_ref[...] = mem
            return carry

        with jax.named_scope("b_loop"):
            lax.fori_loop(0, NB, body, 0)
        for i in range(2):
            b_finish(first, NSEG - 1, NSEG - 1, 1, i)

    for first in (True, False):
        kv_ref[...] = jnp.zeros(kv_ref.shape, f32)
        with jax.named_scope("a_p1"):
            a_phase1(first)
        with jax.named_scope("a_p2"):
            a_phase2(first)
        with jax.named_scope("layer_b"):
            layer_b(first)

    cp_out(NB - 2, 2).start()
    cp_out(0, NB).wait()


@jax.jit
def pallas_interleave_layers__linear_kernel_hedgehog__memory_aug_recurrent_mem_tr__prompt_kernel(
    A_x: jax.Array,
    A_wqkv: jax.Array,
    A_w_phi: jax.Array,
    A_wo: jax.Array,
    B_x: jax.Array,
    B_mem0: jax.Array,
    B_Wq: jax.Array,
    B_Wk: jax.Array,
    B_Wv: jax.Array,
    B_Wo: jax.Array,
    B_seg_len: jax.Array,
):
    del B_x, B_seg_len
    x = A_x.reshape(S, D)
    phi = A_w_phi.transpose(1, 2, 0)
    wqt = B_Wq.transpose(1, 2, 0).reshape(HD, D)
    wkt = B_Wk.transpose(1, 2, 0).reshape(HD, D)
    wvt = B_Wv.transpose(1, 2, 0).reshape(HD, D)
    wo = B_Wo.reshape(HD, D)
    hbm = pl.BlockSpec(memory_space=pl.ANY)
    out = pl.pallas_call(
        _kernel,
        out_shape=jax.ShapeDtypeStruct((S, D), bf16),
        in_specs=[hbm] * 9,
        out_specs=hbm,
        scratch_shapes=[
            pltpu.VMEM((S, D), bf16),
            pltpu.VMEM((3, D, D), bf16),
            pltpu.VMEM((DA, DA, HA), bf16),
            pltpu.VMEM((D, D), bf16),
            pltpu.VMEM((MEM, D), bf16),
            pltpu.VMEM((S + SEG, D), f32),
            pltpu.VMEM((S // 2, D), u32),
            pltpu.VMEM((2, SEG, D), f32),
            pltpu.VMEM((SEG, D), f32),
            pltpu.VMEM((SEG, D), f32),
            pltpu.VMEM((2, SEG, D), f32),
            pltpu.VMEM((S // 2, D), u32),
            pltpu.VMEM((3, GA, 80, D), u32),
            pltpu.VMEM((D // 2, D), u32),
            pltpu.VMEM((2, GA, 160, 256), f32),
            pltpu.VMEM((NCH, NPA, RA, TC), u32),
            pltpu.VMEM((NPA, RA + 8, 2 * RA), f32),
            pltpu.VMEM((NPA, (RA + 8) // 2, 2 * RA), u32),
            pltpu.VMEM((3, HD + TRC, D), bf16),
            pltpu.VMEM((3, NPB + 2, D // 2, PW), u32),
            pltpu.VMEM((D // 128, HD, 128), bf16),
            pltpu.VMEM((MEM, D), f32),
            pltpu.VMEM((L, HD), f32),
            pltpu.SemaphoreType.DMA((16 + 3 * NTR,)),
        ],
        compiler_params=pltpu.CompilerParams(vmem_limit_bytes=120 * 1024 * 1024),
    )(x, A_wqkv, phi, A_wo, B_mem0.reshape(MEM, D), wqt, wkt, wvt, wo)
    return out.reshape(1, S, D)
```

```python
import functools
import os

import jax
import jax.numpy as jnp
from jax import lax
import jax.experimental.pallas as pl
import jax.experimental.pallas.tpu as pltpu

f32, bf16, u32, i32 = jnp.float32, jnp.bfloat16, jnp.uint32, jnp.int32

S, D = 2048, 640
HA, DA = 32, 20
NPA = HA // 2
RA = 2 * DA
GA = 4
TC = 256
NCH = S // TC
XCH = 512
HB, DB, MEM, SEG = 32, 192, 8, 32
HD = HB * DB
L = MEM + SEG
NPB = HB // 2
PW = 2 * DB
SCALE = DB ** -0.5
TRC = 768
NTR = HD // TRC
NSEG = S // SEG
SPI = int(os.environ.get("SPI", "2"))
NB = NSEG // SPI
assert NTR == NCH

SCH = tuple(int(v) for v in os.environ.get("SCH", "1,0,1,4,2,4,7").split(","))
OUTER_BF16 = int(os.environ.get("OUTER_BF16", "1"))
KVLAG = int(os.environ.get("KVLAG", "12"))
P1U = int(os.environ.get("P1U", "2"))

_NN = (((1,), (0,)), ((), ()))
_NT = (((1,), (1,)), ((), ()))


def _dot(a, b):
    return lax.dot_general(a, b, _NN, preferred_element_type=f32)


def _dot_nt(a, b):
    return lax.dot_general(a, b, _NT, preferred_element_type=f32)


def _pack(x):
    return pltpu.bitcast(x.astype(bf16), u32)


def _unpack(x):
    return pltpu.bitcast(x, bf16)


def _lhs(x):
    return x.astype(bf16) if OUTER_BF16 else x


def _ln(x):
    m = jnp.mean(x, axis=-1, keepdims=True)
    xc = x - m
    r = lax.rsqrt(jnp.mean(xc * xc, axis=-1, keepdims=True) + 1e-5)
    return x * r - m * r


def _ln_chained(x, chain):
    m = jnp.mean(x, axis=-1, keepdims=True)
    xc = x - m
    r = lax.rsqrt(jnp.mean(xc * xc, axis=-1, keepdims=True) + 1e-5)
    chain.append(jnp.minimum(r, 0.0))
    return x * r - m * r


def _fold(op, p):
    r = p[0:8]
    for j in range(1, 5):
        r = op(r, p[8 * j:8 * j + 8])
    r = op(r, pltpu.roll(r, 2, 0))
    return op(r, pltpu.roll(r, 4, 0))


def _tile5(r):
    return jnp.concatenate([r] * 5, axis=0)


def _phi(p):
    ep = jnp.exp(p - _tile5(_fold(jnp.maximum, p)))
    en = jnp.exp(_tile5(_fold(jnp.minimum, p)) - p)
    ep = ep * _tile5(1.0 / _fold(jnp.add, ep))
    en = en * _tile5(1.0 / _fold(jnp.add, en))
    return jnp.concatenate([ep, en], axis=0).astype(bf16)


def _split(k):
    lo = lax.broadcasted_iota(i32, (L, 128), 1) < 64
    z = jnp.zeros((L, 128), f32)
    mid = k[:, 128:256]
    outer = jnp.concatenate([k[:, 0:128], k[:, 256:384]], axis=0).astype(bf16)
    mid = jnp.concatenate([jnp.where(lo, mid, z), jnp.where(lo, z, mid)], axis=0).astype(bf16)
    return outer, mid


def _probs(q, k, chain):
    r = lax.broadcasted_iota(i32, (L, 2 * L), 0)
    c = lax.broadcasted_iota(i32, (L, 2 * L), 1)
    first = c < L
    so = _dot_nt(q[0], k[0])
    s = jnp.where(first, so[0:L], so[L:2 * L]) + _dot_nt(q[1], k[1])
    s = s * SCALE
    if chain:
        s = jnp.concatenate([s[0:8] + chain.pop(0), s[8:L]], axis=0)
    mask = (r < MEM) | (r >= jnp.where(first, c, c - L))
    s = jnp.where(mask, s, -1000000000.0)
    neg = jnp.full_like(s, -jnp.inf)
    ma = jnp.max(jnp.where(first, s, neg), axis=-1, keepdims=True)
    mb = jnp.max(jnp.where(first, neg, s), axis=-1, keepdims=True)
    e = jnp.exp(s - jnp.where(first, ma, mb))
    z = jnp.zeros_like(e)
    ea = jnp.where(first, e, z)
    eb = jnp.where(first, z, e)
    pa = ea * (1.0 / jnp.sum(ea, axis=-1, keepdims=True))
    pb = eb * (1.0 / jnp.sum(eb, axis=-1, keepdims=True))
    return _lhs(jnp.concatenate([pa, pb], axis=0)), pa + pb


def _pv(p, v):
    oo = _dot(p[0], v[0])
    return jnp.concatenate([oo[0:L], _dot(p[1], v[1]), oo[L:2 * L]], axis=1)


def _kernel(x_hbm, wqkv_hbm, phi_hbm, woa_hbm, mem0_hbm, wqt_hbm, wkt_hbm, wvt_hbm, wo_hbm, out_hbm,
            xin_ref, wqkv, phi_ref, wo_a, mem0, x_ref, xna_ref, xnb_ref, xa_ref, xb_ref, yb_ref, oa_ref,
            wat_ref, wop_ref, lhs_ref, phiq_ref, kv_ref, kvm_ref, stage_ref, wb_ref, wo_ref, mem_ref, o_ref,
            sems):
    cp_phi = pltpu.make_async_copy(phi_hbm, phi_ref, sems.at[0])
    cp_mem0 = pltpu.make_async_copy(mem0_hbm, mem0, sems.at[1])
    cp_woa = pltpu.make_async_copy(woa_hbm, wo_a, sems.at[2])
    cp_wo = [pltpu.make_async_copy(wo_hbm.at[:, pl.ds(128 * n, 128)], wo_ref.at[n], sems.at[7 + n])
             for n in range(D // 128)]
    big = (wqt_hbm, wkt_hbm, wvt_hbm)

    def cp_wqkv(n):
        return pltpu.make_async_copy(wqkv_hbm.at[:, pl.ds(pl.multiple_of(D * n, 128), D)], wqkv.at[n],
                                     sems.at[4 + n])

    def cp_x(j):
        rows = pl.ds(pl.multiple_of(j * XCH, XCH), XCH)
        return pltpu.make_async_copy(x_hbm.at[rows, :], xin_ref.at[rows, :], sems.at[12 + j])

    def cp_w(n, j):
        rows = pl.ds(pl.multiple_of(j * TRC, TRC), TRC)
        return pltpu.make_async_copy(big[n].at[rows, :], stage_ref.at[n, rows, :], sems.at[16 + n * NTR + j])

    def cp_out(j, nblk):
        rows = pl.ds(pl.multiple_of(j * SPI * SEG, SEG), SPI * SEG * nblk)
        return pltpu.make_async_copy(xin_ref.at[rows, :], out_hbm.at[rows, :], sems.at[3])

    cp_phi.start()
    for j in range(S // XCH):
        cp_x(j).start()
    for n in range(3):
        cp_wqkv(n).start()
    cp_mem0.start()
    for j in range(NTR):
        if j == NTR - 1:
            cp_woa.start()
        for n in range(3):
            cp_w(n, j).start()
    for cp in cp_wo:
        cp.start()

    def init_x(c, carry):
        with jax.named_scope("wait_x"):
            cp_x(c).wait()
        x = xin_ref[pl.ds(pl.multiple_of(c * XCH, XCH), XCH), :].astype(f32)
        x_ref[pl.ds(pl.multiple_of(c * XCH, XCH), XCH), :] = x
        xna_ref[pl.ds(pl.multiple_of(c * (XCH // 2), XCH // 2), XCH // 2), :] = _pack(_ln(x))
        return carry

    with jax.named_scope("wait_phi"):
        cp_phi.wait()
    ecol = lax.broadcasted_iota(i32, (HA, D), 1) - DA * lax.broadcasted_iota(i32, (HA, D), 0)
    tp = _dot(phi_ref[0], jnp.where(ecol == 0, 1.0, 0.0).astype(bf16))
    for d in range(1, DA):
        tp = tp + _dot(phi_ref[d], jnp.where(ecol == d, 1.0, 0.0).astype(bf16))
    rep = jnp.where((lax.broadcasted_iota(i32, (RA, DA), 0) >> 1) == lax.broadcasted_iota(i32, (RA, DA), 1),
                    1.0, 0.0).astype(bf16)
    urep = _dot(rep, tp.astype(bf16))
    for g in range(GA):
        col = lax.broadcasted_iota(i32, (RA, 256), 1) + 128 * g
        par = lax.broadcasted_iota(i32, (RA, 256), 0) & 1
        for pp in range(4):
            lo = (8 * g + 2 * pp + par) * DA
            blk = jnp.where((col >= lo) & (col < lo + DA), urep[:, 128 * g:128 * g + 256], 0.0)
            lhs_ref[0, g, RA * pp:RA * pp + RA, :] = blk
        lhs_ref[1, g] = jnp.where(lax.broadcasted_iota(i32, (160, 256), 1) + 128 * g
                                  == lax.broadcasted_iota(i32, (160, 256), 0) + 160 * g, 1.0, 0.0)

    with jax.named_scope("init_x"):
        lax.fori_loop(0, S // XCH, init_x, 0)

    def prep(n, carry):
        with jax.named_scope("wait_wqkv"):
            cp_wqkv(n).wait()
        for g in range(GA):
            wat_ref[n, g] = _pack(_dot_nt(lhs_ref[n // 2, g].astype(bf16), wqkv[n, :, 128 * g:128 * g + 256]))
        return carry

    with jax.named_scope("prep"):
        lax.fori_loop(0, 3, prep, 0)
        cp_mem0.wait()

    def transpose_w(n, p):
        t = stage_ref[n, pl.ds(pl.multiple_of(p * PW, PW), PW), :].T
        wb_ref[n, p] = pltpu.bitcast(t, u32)

    def a_phase1(first):
        def body(c, carry):
            if first:
                ct = jnp.where(c == 0, NTR, c - 1)

                @pl.when(c > 0)
                def _():
                    with jax.named_scope("wait_w"):
                        for n in range(3):
                            cp_w(n, c - 1).wait()

            xn = _unpack(xna_ref[pl.ds(pl.multiple_of(c * (TC // 2), TC // 2), TC // 2), :])
            ones = jnp.ones((8, TC), f32)
            pend = []

            def flush(n):
                while len(pend) > n:
                    p, vext, phik = pend.pop(0)
                    kv_ref[p] += _dot_nt(vext, phik)

            for g in range(GA):
                pq = _dot_nt(_unpack(wat_ref[0, g]), xn)
                flush(KVLAG)
                pk = _dot_nt(_unpack(wat_ref[1, g]), xn)
                vt = _dot_nt(_unpack(wat_ref[2, g]), xn)
                for pp in range(4):
                    p = 4 * g + pp
                    sl = slice(RA * pp, RA * pp + RA)
                    phiq_ref[c, p] = pltpu.bitcast(_phi(pq[sl]), u32)
                    vext = jnp.concatenate([vt[sl], ones], axis=0).astype(bf16)
                    pend.append((p, vext, _phi(pk[sl])))
                if first and g < 3:
                    transpose_w(g, 2 * ct)
                    transpose_w(g, 2 * ct + 1)
            flush(0)
            return carry

        lax.fori_loop(0, NCH, body, 0, unroll=1 if first else P1U)

    def a_phase2(first):
        r = lax.broadcasted_iota(i32, (RA + 8, 2 * RA), 0)
        rb = jnp.where(((r >= DA) & (r < RA)) | (r >= RA + 4), 1, 0)
        same = rb == (lax.broadcasted_iota(i32, (RA + 8, 2 * RA), 1) & 1)
        for p in range(NPA):
            kvm_ref[p] = _pack(jnp.where(same, kv_ref[p], 0.0))

        def attend(c):
            top = lax.broadcasted_iota(i32, (8, TC), 0) < 4
            ot = []
            for p in range(NPA):
                ne = _dot(_unpack(kvm_ref[p]), _unpack(phiq_ref[c, p]))
                rc = 1.0 / (ne[RA:RA + 8] + 1e-6)
                sw = pltpu.roll(rc, 4, 0)
                ra, rb = jnp.where(top, rc, sw), jnp.where(top, sw, rc)
                ot.append(ne[0:RA] * jnp.concatenate([ra, ra, rc, rb, rb], axis=0))
            o = jnp.concatenate(ot, axis=0).T
            oa_ref[pl.ds(pl.multiple_of(c * (TC // 2), TC // 2), TC // 2), :] = _pack(o)

        if not first:
            for c in range(NCH):
                attend(c)
            return

        attend(0)
        with jax.named_scope("wait_w7"):
            cp_woa.wait()
            for n in range(3):
                cp_w(n, NTR - 1).wait()

        def body(c, carry):
            lhs = [_unpack(oa_ref[pl.ds(pl.multiple_of(c * (TC // 2) + r // 2, 64), 64), :])
                   for r in range(0, TC, 128)]
            attend(jnp.minimum(c + 1, NCH - 1))
            t = jnp.minimum(c, 5)
            transpose_w(t // 2, NPB - 2 + t % 2)
            for r in range(0, TC, 128):
                x_ref[pl.ds(pl.multiple_of(c * TC + r, 128), 128), :] += _dot(lhs[r // 128], wo_a[...])
            return carry

        lax.fori_loop(0, NCH, body, 0)

    def seg_rows(sg, off=0, n=SEG):
        return pl.ds(pl.multiple_of(sg * SEG + off, 8), n)

    def a_finish(sr, sw, n):
        cols = slice(128 * n, 128 * n + 128)
        y = _dot(_unpack(oa_ref[pl.ds(pl.multiple_of(sr * (SEG // 2), SEG // 2), SEG // 2), :]),
                 _unpack(wop_ref[:, cols]))
        x = x_ref[seg_rows(sr), cols] + y
        x_ref[seg_rows(sw), cols] = x
        xa_ref[:, cols] = x

    def a_norm(first, sg, slot, i, chain):
        x = x_ref[seg_rows(sg, 8 * i, 8), :] if first else xa_ref[8 * i:8 * i + 8, :]
        xnb_ref[slot, 8 * i:8 * i + 8, :] = _ln_chained(x, chain)

    def b_finish(first, sr, sw, slot, i, chain):
        x = x_ref[seg_rows(sr, 16 * i, 16), :] + yb_ref[slot, 16 * i:16 * i + 16, :]
        if first:
            x_ref[seg_rows(sw, 16 * i, 16), :] = x
            xb_ref[16 * i:16 * i + 16, :] = x
            xn = [_ln_chained(xb_ref[16 * i + k:16 * i + k + 8, :], chain) for k in (0, 8)]
            xna_ref[pl.ds(pl.multiple_of(sr * (SEG // 2) + 8 * i, 8), 8), :] = _pack(
                jnp.concatenate(xn, axis=0))
        else:
            xin_ref[pl.ds(pl.multiple_of(sr * SEG + 16 * i, 16), 16), :] = x.astype(bf16)

    wo32 = wo_ref.bitcast(u32)

    def b_step(h, side, chain):
        st = {}

        def proj(p, which):
            if p == 0 and which == 0:
                y = _dot(h[:, 0:128], _unpack(wb_ref[0, 0, 0:64, :]))
                for k in range(1, D // 128):
                    y = y + _dot(h[:, 128 * k:128 * k + 128], _unpack(wb_ref[0, 0, 64 * k:64 * k + 64, :]))
            else:
                y = _dot(h, _unpack(wb_ref[which, p]))
            y = jnp.concatenate([y[SEG:L], y[0:SEG]], axis=0)
            if which == 0:
                st[(p, which)] = (_lhs(jnp.concatenate([y[:, 0:128], y[:, 256:384]], axis=0)), y[:, 128:256])
            else:
                st[(p, which)] = _split(y)

        def do_qk(p):
            st[(p, 'p')] = _probs(st.pop((p, 0)), st.pop((p, 1)), chain)

        def do_pv(p):
            o_ref[:, p * PW:(p + 1) * PW] = _pv(st.pop((p, 'p')), st.pop((p, 2)))

        def do_o(n):
            k0 = st.get('k', 0)
            k1 = min(k0 + n, HD // 128)
            if k0 == k1:
                return
            st['k'] = k1
            w = jnp.concatenate([wo32[t, k0 * 64:k1 * 64, :] for t in range(D // 128)], axis=1)
            y = _dot(o_ref[:, k0 * 128:k1 * 128], _unpack(w))
            st['y'] = y if 'y' not in st else st['y'] + y

        o1, o2, o3, olag, f1, f2, f3 = SCH
        for s in range(NPB):
            on = s >= olag
            proj(s, 0)
            if on:
                do_o(o1)
            if s >= 1:
                do_qk(s - 1)
            proj(s, 1)
            if on:
                do_o(o2)
            if s >= 2:
                do_pv(s - 2)
            proj(s, 2)
            if on:
                do_o(o3)
            for job in side[s]:
                job()
            assert st.get('k', 0) <= 3 * max(s - 2, 0)
        do_o(f1)
        do_qk(NPB - 1)
        do_o(f2)
        do_pv(NPB - 2)
        do_o(f3)
        assert st.get('k', 0) <= 3 * (NPB - 2)
        do_pv(NPB - 1)
        do_o(3 * (NPB - 1) - st['k'])
        do_o(3)
        return st['y']

    def layer_b(first):
        mem_ref[...] = mem0[...].astype(f32)
        yb_ref[1] = jnp.zeros((SEG, D), f32)
        if not first:
            for n in range(D // 128):
                a_finish(0, 0, n)
        for i in range(4):
            a_norm(first, 0, 0, i, [])
        if first:
            wop_ref[...] = pltpu.bitcast(wo_a[...], u32)
            with jax.named_scope("wait_wo"):
                for cp in cp_wo:
                    cp.wait()

        def body(j, carry):
            if not first:
                @pl.when(j >= 2)
                def _():
                    cp_out(j - 2, 1).start()

            mem = mem_ref[...]
            for t in range(SPI):
                sg = j * SPI + t
                sp = jnp.maximum(sg - 1, 0) if t == 0 else sg - 1
                sw = jnp.where(sg == 0, NSEG, sp) if t == 0 else sp
                sn = jnp.minimum(sg + 1, NSEG - 1) if t == SPI - 1 else sg + 1
                h = jnp.concatenate([xnb_ref[t % 2], mem], axis=0)
                chain = []
                side = [[] for _ in range(NPB)]
                for i in range(2):
                    side[1 + 2 * i].append(functools.partial(b_finish, first, sp, sw, (t + 1) % 2, i, chain))
                if not first:
                    for n in range(D // 128):
                        side[n].append(functools.partial(a_finish, sn, sg + 1, n))
                for i in range(4):
                    side[6 + 2 * i].append(functools.partial(a_norm, first, sn, (t + 1) % 2, i, chain))
                y = b_step(h, side, chain)
                mem = y[0:MEM]
                yb_ref[t % 2] = y[MEM:L]
            mem_ref[...] = mem
            return carry

        with jax.named_scope("b_loop"):
            lax.fori_loop(0, NB, body, 0)
        for i in range(2):
            b_finish(first, NSEG - 1, NSEG - 1, 1, i, [])

    for first in (True, False):
        kv_ref[...] = jnp.zeros(kv_ref.shape, f32)
        with jax.named_scope("a_p1"):
            a_phase1(first)
        with jax.named_scope("a_p2"):
            a_phase2(first)
        with jax.named_scope("layer_b"):
            layer_b(first)

    cp_out(NB - 2, 2).start()
    cp_out(0, NB).wait()


@jax.jit
def pallas_interleave_layers__linear_kernel_hedgehog__memory_aug_recurrent_mem_tr__prompt_kernel(
    A_x: jax.Array,
    A_wqkv: jax.Array,
    A_w_phi: jax.Array,
    A_wo: jax.Array,
    B_x: jax.Array,
    B_mem0: jax.Array,
    B_Wq: jax.Array,
    B_Wk: jax.Array,
    B_Wv: jax.Array,
    B_Wo: jax.Array,
    B_seg_len: jax.Array,
):
    del B_x, B_seg_len
    x = A_x.reshape(S, D)
    phi = A_w_phi.transpose(1, 2, 0)
    wqt = B_Wq.transpose(1, 2, 0).reshape(HD, D)
    wkt = B_Wk.transpose(1, 2, 0).reshape(HD, D)
    wvt = B_Wv.transpose(1, 2, 0).reshape(HD, D)
    wo = B_Wo.reshape(HD, D)
    hbm = pl.BlockSpec(memory_space=pl.ANY)
    out = pl.pallas_call(
        _kernel,
        out_shape=jax.ShapeDtypeStruct((S, D), bf16),
        in_specs=[hbm] * 9,
        out_specs=hbm,
        scratch_shapes=[
            pltpu.VMEM((S, D), bf16),
            pltpu.VMEM((3, D, D), bf16),
            pltpu.VMEM((DA, DA, HA), bf16),
            pltpu.VMEM((D, D), bf16),
            pltpu.VMEM((MEM, D), bf16),
            pltpu.VMEM((S + SEG, D), f32),
            pltpu.VMEM((S // 2, D), u32),
            pltpu.VMEM((2, SEG, D), f32),
            pltpu.VMEM((SEG, D), f32),
            pltpu.VMEM((SEG, D), f32),
            pltpu.VMEM((2, SEG, D), f32),
            pltpu.VMEM((S // 2, D), u32),
            pltpu.VMEM((3, GA, 80, D), u32),
            pltpu.VMEM((D // 2, D), u32),
            pltpu.VMEM((2, GA, 160, 256), f32),
            pltpu.VMEM((NCH, NPA, RA, TC), u32),
            pltpu.VMEM((NPA, RA + 8, 2 * RA), f32),
            pltpu.VMEM((NPA, (RA + 8) // 2, 2 * RA), u32),
            pltpu.VMEM((3, HD + TRC, D), bf16),
            pltpu.VMEM((3, NPB + 2, D // 2, PW), u32),
            pltpu.VMEM((D // 128, HD, 128), bf16),
            pltpu.VMEM((MEM, D), f32),
            pltpu.VMEM((L, HD), f32),
            pltpu.SemaphoreType.DMA((16 + 3 * NTR,)),
        ],
        compiler_params=pltpu.CompilerParams(vmem_limit_bytes=120 * 1024 * 1024),
    )(x, A_wqkv, phi, A_wo, B_mem0.reshape(MEM, D), wqt, wkt, wvt, wo)
    return out.reshape(1, S, D)
```

```python
import functools
import os

import jax
import jax.numpy as jnp
from jax import lax
import jax.experimental.pallas as pl
import jax.experimental.pallas.tpu as pltpu

f32, bf16, u32, i32 = jnp.float32, jnp.bfloat16, jnp.uint32, jnp.int32

S, D = 2048, 640
HA, DA = 32, 20
NPA = HA // 2
RA = 2 * DA
GA = 4
TC = 256
NCH = S // TC
XCH = int(os.environ.get("XCH", "256"))
HB, DB, MEM, SEG = 32, 192, 8, 32
HD = HB * DB
L = MEM + SEG
NPB = HB // 2
PW = 2 * DB
SCALE = DB ** -0.5
TRC = 768
NTR = HD // TRC
NSEG = S // SEG
SPI = int(os.environ.get("SPI", "2"))
NB = NSEG // SPI
assert NTR == NCH

SCH = tuple(int(v) for v in os.environ.get("SCH", "1,0,1,4,2,4,7").split(","))
OUTER_BF16 = int(os.environ.get("OUTER_BF16", "1"))
WOMODE = int(os.environ.get("WOMODE", "2"))
KVLAG = int(os.environ.get("KVLAG", "12"))
P1U = int(os.environ.get("P1U", "4"))

_NN = (((1,), (0,)), ((), ()))
_NT = (((1,), (1,)), ((), ()))


def _dot(a, b):
    return lax.dot_general(a, b, _NN, preferred_element_type=f32)


def _dot_nt(a, b):
    return lax.dot_general(a, b, _NT, preferred_element_type=f32)


def _pack(x):
    return pltpu.bitcast(x.astype(bf16), u32)


def _unpack(x):
    return pltpu.bitcast(x, bf16)


def _lhs(x):
    return x.astype(bf16) if OUTER_BF16 else x


def _ln(x):
    m = jnp.mean(x, axis=-1, keepdims=True)
    xc = x - m
    r = lax.rsqrt(jnp.mean(xc * xc, axis=-1, keepdims=True) + 1e-5)
    return x * r - m * r


def _ln_chained(x, chain):
    m = jnp.mean(x, axis=-1, keepdims=True)
    xc = x - m
    r = lax.rsqrt(jnp.mean(xc * xc, axis=-1, keepdims=True) + 1e-5)
    chain.append(jnp.minimum(r, 0.0))
    return x * r - m * r


def _fold(op, p):
    r = p[0:8]
    for j in range(1, 5):
        r = op(r, p[8 * j:8 * j + 8])
    r = op(r, pltpu.roll(r, 2, 0))
    return op(r, pltpu.roll(r, 4, 0))


def _tile5(r):
    return jnp.concatenate([r] * 5, axis=0)


def _phi(p):
    ep = jnp.exp(p - _tile5(_fold(jnp.maximum, p)))
    en = jnp.exp(_tile5(_fold(jnp.minimum, p)) - p)
    ep = ep * _tile5(1.0 / _fold(jnp.add, ep))
    en = en * _tile5(1.0 / _fold(jnp.add, en))
    return jnp.concatenate([ep, en], axis=0).astype(bf16)


def _split(k):
    lo = lax.broadcasted_iota(i32, (L, 128), 1) < 64
    z = jnp.zeros((L, 128), f32)
    mid = k[:, 128:256]
    outer = jnp.concatenate([k[:, 0:128], k[:, 256:384]], axis=0).astype(bf16)
    mid = jnp.concatenate([jnp.where(lo, mid, z), jnp.where(lo, z, mid)], axis=0).astype(bf16)
    return outer, mid


def _probs(q, k, chain):
    r = lax.broadcasted_iota(i32, (L, 2 * L), 0)
    c = lax.broadcasted_iota(i32, (L, 2 * L), 1)
    first = c < L
    so = _dot_nt(q[0], k[0])
    s = jnp.where(first, so[0:L], so[L:2 * L]) + _dot_nt(q[1], k[1])
    s = s * SCALE
    if chain:
        s = jnp.concatenate([s[0:8] + chain.pop(0), s[8:L]], axis=0)
    mask = (r < MEM) | (r >= jnp.where(first, c, c - L))
    s = jnp.where(mask, s, -1000000000.0)
    neg = jnp.full_like(s, -jnp.inf)
    ma = jnp.max(jnp.where(first, s, neg), axis=-1, keepdims=True)
    mb = jnp.max(jnp.where(first, neg, s), axis=-1, keepdims=True)
    e = jnp.exp(s - jnp.where(first, ma, mb))
    z = jnp.zeros_like(e)
    ea = jnp.where(first, e, z)
    eb = jnp.where(first, z, e)
    pa = ea * (1.0 / jnp.sum(ea, axis=-1, keepdims=True))
    pb = eb * (1.0 / jnp.sum(eb, axis=-1, keepdims=True))
    return _lhs(jnp.concatenate([pa, pb], axis=0)), pa + pb


def _pv(p, v):
    oo = _dot(p[0], v[0])
    return jnp.concatenate([oo[0:L], _dot(p[1], v[1]), oo[L:2 * L]], axis=1)


def _kernel(x_hbm, wqkv_hbm, phi_hbm, woa_hbm, mem0_hbm, wqt_hbm, wkt_hbm, wvt_hbm, wo_hbm, out_hbm,
            xin_ref, wqkv, phi_ref, wo_a, mem0, x_ref, xna_ref, xnb_ref, xa_ref, xb_ref, yb_ref, oa_ref,
            wat_ref, wop_ref, lhs_ref, phiq_ref, kv_ref, kvm_ref, stage_ref, wb_ref, wo_ref, mem_ref, o_ref,
            sems):
    cp_phi = pltpu.make_async_copy(phi_hbm, phi_ref, sems.at[0])
    cp_mem0 = pltpu.make_async_copy(mem0_hbm, mem0, sems.at[1])
    cp_woa = pltpu.make_async_copy(woa_hbm, wo_a, sems.at[2])
    if WOMODE < 2:
        cp_wo = [pltpu.make_async_copy(wo_hbm.at[:, pl.ds(128 * n, 128)], wo_ref.at[n], sems.at[7 + n])
                 for n in range(D // 128)]
    else:
        cp_wo = [pltpu.make_async_copy(wo_hbm, wo_ref, sems.at[7])]
    big = (wqt_hbm, wkt_hbm, wvt_hbm)

    def cp_wqkv(n):
        return pltpu.make_async_copy(wqkv_hbm.at[:, pl.ds(pl.multiple_of(D * n, 128), D)], wqkv.at[n],
                                     sems.at[4 + n])

    def cp_x(j):
        rows = pl.ds(pl.multiple_of(j * XCH, XCH), XCH)
        return pltpu.make_async_copy(x_hbm.at[rows, :], xin_ref.at[rows, :], sems.at[12 + j])

    def cp_w(n, j):
        rows = pl.ds(pl.multiple_of(j * TRC, TRC), TRC)
        return pltpu.make_async_copy(big[n].at[rows, :], stage_ref.at[n, rows, :], sems.at[20 + n * NTR + j])

    def cp_rows(sg, nseg):
        rows = pl.ds(pl.multiple_of(sg * SEG, SEG), SEG * nseg)
        return pltpu.make_async_copy(xin_ref.at[rows, :], out_hbm.at[rows, :], sems.at[3])

    cp_phi.start()
    for n in range(3):
        cp_wqkv(n).start()
    for j in range(S // XCH):
        cp_x(j).start()
    cp_mem0.start()
    for j in range(NTR):
        if j == NTR - 1:
            cp_woa.start()
        for n in range(3):
            cp_w(n, j).start()
    for cp in cp_wo:
        cp.start()

    def init_x(c, carry):
        with jax.named_scope("wait_x"):
            cp_x(c).wait()
        x = xin_ref[pl.ds(pl.multiple_of(c * XCH, XCH), XCH), :].astype(f32)
        x_ref[pl.ds(pl.multiple_of(c * XCH, XCH), XCH), :] = x
        xna_ref[pl.ds(pl.multiple_of(c * (XCH // 2), XCH // 2), XCH // 2), :] = _pack(_ln(x))
        return carry

    with jax.named_scope("wait_phi"):
        cp_phi.wait()
    ecol = lax.broadcasted_iota(i32, (HA, D), 1) - DA * lax.broadcasted_iota(i32, (HA, D), 0)
    def scatter_phi(i, tp):
        for d in range(5):
            tp = tp + _dot(phi_ref[5 * i + d], jnp.where(ecol == 5 * i + d, 1.0, 0.0).astype(bf16))
        return tp

    tp = lax.fori_loop(0, DA // 5, scatter_phi, jnp.zeros((DA, D), f32))
    rep = jnp.where((lax.broadcasted_iota(i32, (RA, DA), 0) >> 1) == lax.broadcasted_iota(i32, (RA, DA), 1),
                    1.0, 0.0).astype(bf16)
    urep = _dot(rep, tp.astype(bf16))
    for g in range(GA):
        col = lax.broadcasted_iota(i32, (RA, 256), 1) + 128 * g
        par = lax.broadcasted_iota(i32, (RA, 256), 0) & 1
        for pp in range(4):
            lo = (8 * g + 2 * pp + par) * DA
            blk = jnp.where((col >= lo) & (col < lo + DA), urep[:, 128 * g:128 * g + 256], 0.0)
            lhs_ref[0, g, RA * pp:RA * pp + RA, :] = blk
        lhs_ref[1, g] = jnp.where(lax.broadcasted_iota(i32, (160, 256), 1) + 128 * g
                                  == lax.broadcasted_iota(i32, (160, 256), 0) + 160 * g, 1.0, 0.0)

    def prep(n, carry):
        with jax.named_scope("wait_wqkv"):
            cp_wqkv(n).wait()
        for g in range(GA):
            wat_ref[n, g] = _pack(_dot_nt(lhs_ref[n // 2, g].astype(bf16), wqkv[n, :, 128 * g:128 * g + 256]))
        return carry

    with jax.named_scope("prep"):
        lax.fori_loop(0, 3, prep, 0)
    with jax.named_scope("init_x"):
        lax.fori_loop(0, S // XCH, init_x, 0)
        cp_mem0.wait()

    def transpose_w(n, p):
        t = stage_ref[n, pl.ds(pl.multiple_of(p * PW, PW), PW), :].T
        wb_ref[n, p] = pltpu.bitcast(t, u32)

    def a_phase1(first):
        def body(c, carry):
            if first:
                ct = jnp.where(c == 0, NTR, c - 1)

                @pl.when(c > 0)
                def _():
                    with jax.named_scope("wait_w"):
                        for n in range(3):
                            cp_w(n, c - 1).wait()

            xn = _unpack(xna_ref[pl.ds(pl.multiple_of(c * (TC // 2), TC // 2), TC // 2), :])
            ones = jnp.ones((8, TC), f32)
            pend = []

            def flush(n):
                while len(pend) > n:
                    p, vext, phik = pend.pop(0)
                    kv_ref[p] += _dot_nt(vext, phik)

            for g in range(GA):
                pq = _dot_nt(_unpack(wat_ref[0, g]), xn)
                flush(KVLAG)
                pk = _dot_nt(_unpack(wat_ref[1, g]), xn)
                vt = _dot_nt(_unpack(wat_ref[2, g]), xn)
                for pp in range(4):
                    p = 4 * g + pp
                    sl = slice(RA * pp, RA * pp + RA)
                    phiq_ref[c, p] = pltpu.bitcast(_phi(pq[sl]), u32)
                    vext = jnp.concatenate([vt[sl], ones], axis=0).astype(bf16)
                    pend.append((p, vext, _phi(pk[sl])))
                if first and g < 3:
                    transpose_w(g, 2 * ct)
                    transpose_w(g, 2 * ct + 1)
            flush(0)
            return carry

        lax.fori_loop(0, NCH, body, 0, unroll=1 if first else P1U)

    def seg_rows(sg, off=0, n=SEG):
        return pl.ds(pl.multiple_of(sg * SEG + off, 8), n)

    def a_finish(sr, sw, n):
        cols = slice(128 * n, 128 * n + 128)
        y = _dot(_unpack(oa_ref[pl.ds(pl.multiple_of(sr * (SEG // 2), SEG // 2), SEG // 2), :]),
                 _unpack(wop_ref[:, cols]))
        x = x_ref[seg_rows(sr), cols] + y
        x_ref[seg_rows(sw), cols] = x
        xa_ref[:, cols] = x

    def a_norm(first, sg, slot, i, chain):
        x = x_ref[seg_rows(sg, 8 * i, 8), :] if first else xa_ref[8 * i:8 * i + 8, :]
        xnb_ref[slot, 8 * i:8 * i + 8, :] = _ln_chained(x, chain)

    def a_phase2(first):
        r = lax.broadcasted_iota(i32, (RA + 8, 2 * RA), 0)
        rb = jnp.where(((r >= DA) & (r < RA)) | (r >= RA + 4), 1, 0)
        same = rb == (lax.broadcasted_iota(i32, (RA + 8, 2 * RA), 1) & 1)
        for p in range(NPA):
            kvm_ref[p] = _pack(jnp.where(same, kv_ref[p], 0.0))

        def attend(c):
            top = lax.broadcasted_iota(i32, (8, TC), 0) < 4
            ot = []
            for p in range(NPA):
                ne = _dot(_unpack(kvm_ref[p]), _unpack(phiq_ref[c, p]))
                rc = 1.0 / (ne[RA:RA + 8] + 1e-6)
                sw = pltpu.roll(rc, 4, 0)
                ra, rb = jnp.where(top, rc, sw), jnp.where(top, sw, rc)
                ot.append(ne[0:RA] * jnp.concatenate([ra, ra, rc, rb, rb], axis=0))
            o = jnp.concatenate(ot, axis=0).T
            oa_ref[pl.ds(pl.multiple_of(c * (TC // 2), TC // 2), TC // 2), :] = _pack(o)

        if not first:
            wop_ref[...] = pltpu.bitcast(wo_a[...], u32)
            for c in range(NCH):
                attend(c)
                if c == 2:
                    for n in range(D // 128):
                        a_finish(0, 0, n)
                    for i in range(4):
                        a_norm(False, 0, 0, i, [])
            return

        attend(0)
        cp_woa.wait()

        def body(c, carry):
            @pl.when(c == 2)
            def _():
                for n in range(3):
                    cp_w(n, NTR - 1).wait()

            lhs = [_unpack(oa_ref[pl.ds(pl.multiple_of(c * (TC // 2) + r // 2, 64), 64), :])
                   for r in range(0, TC, 128)]
            attend(jnp.minimum(c + 1, NCH - 1))
            t = jnp.maximum(c - 2, 0)
            transpose_w(t // 2, jnp.where(c < 2, NPB, NPB - 2 + t % 2))
            for r in range(0, TC, 128):
                x_ref[pl.ds(pl.multiple_of(c * TC + r, 128), 128), :] += _dot(lhs[r // 128], wo_a[...])
            return carry

        lax.fori_loop(0, NCH, body, 0)

    def b_finish(first, sr, sw, slot, i, chain):
        x = x_ref[seg_rows(sr, 16 * i, 16), :] + yb_ref[slot, 16 * i:16 * i + 16, :]
        if first:
            x_ref[seg_rows(sw, 16 * i, 16), :] = x
            xb_ref[16 * i:16 * i + 16, :] = x
            xn = [_ln_chained(xb_ref[16 * i + k:16 * i + k + 8, :], chain) for k in (0, 8)]
            xna_ref[pl.ds(pl.multiple_of(sr * (SEG // 2) + 8 * i, 8), 8), :] = _pack(
                jnp.concatenate(xn, axis=0))
        else:
            xin_ref[pl.ds(pl.multiple_of(sr * SEG + 16 * i, 16), 16), :] = x.astype(bf16)

    wo32 = wo_ref.bitcast(u32) if WOMODE == 0 else None

    def b_step(h, side, chain):
        st = {}

        def proj(p, which):
            if p == 0 and which == 0:
                y = _dot(h[:, 0:128], _unpack(wb_ref[0, 0, 0:64, :]))
                for k in range(1, D // 128):
                    y = y + _dot(h[:, 128 * k:128 * k + 128], _unpack(wb_ref[0, 0, 64 * k:64 * k + 64, :]))
            else:
                y = _dot(h, _unpack(wb_ref[which, p]))
            y = jnp.concatenate([y[SEG:L], y[0:SEG]], axis=0)
            if which == 0:
                st[(p, which)] = (_lhs(jnp.concatenate([y[:, 0:128], y[:, 256:384]], axis=0)), y[:, 128:256])
            else:
                st[(p, which)] = _split(y)

        def do_qk(p):
            st[(p, 'p')] = _probs(st.pop((p, 0)), st.pop((p, 1)), chain)

        def do_pv(p):
            o_ref[:, p * PW:(p + 1) * PW] = _pv(st.pop((p, 'p')), st.pop((p, 2)))

        def do_o(n):
            k0 = st.get('k', 0)
            k1 = min(k0 + n, HD // 128)
            if k0 == k1:
                return
            st['k'] = k1
            if WOMODE == 0:
                w = _unpack(jnp.concatenate([wo32[t, k0 * 64:k1 * 64, :] for t in range(D // 128)], axis=1))
            elif WOMODE == 1:
                w = jnp.concatenate([wo_ref[t, k0 * 128:k1 * 128, :] for t in range(D // 128)], axis=1)
            else:
                w = wo_ref[k0 * 128:k1 * 128, :]
            y = _dot(o_ref[:, k0 * 128:k1 * 128], w)
            st['y'] = y if 'y' not in st else st['y'] + y

        o1, o2, o3, olag, f1, f2, f3 = SCH
        for s in range(NPB):
            on = s >= olag
            proj(s, 0)
            if on:
                do_o(o1)
            if s >= 1:
                do_qk(s - 1)
            proj(s, 1)
            if on:
                do_o(o2)
            if s >= 2:
                do_pv(s - 2)
            proj(s, 2)
            if on:
                do_o(o3)
            for job in side[s]:
                job()
            assert st.get('k', 0) <= 3 * max(s - 2, 0)
        do_o(f1)
        do_qk(NPB - 1)
        do_o(f2)
        do_pv(NPB - 2)
        do_o(f3)
        assert st.get('k', 0) <= 3 * (NPB - 2)
        do_pv(NPB - 1)
        do_o(3 * (NPB - 1) - st['k'])
        do_o(3)
        return st['y']

    def layer_b(first):
        mem_ref[...] = mem0[...].astype(f32)
        yb_ref[1] = jnp.zeros((SEG, D), f32)
        if first:
            for i in range(4):
                a_norm(first, 0, 0, i, [])
            with jax.named_scope("wait_wo"):
                for cp in cp_wo:
                    cp.wait()

        def body(j, carry):
            if not first:
                @pl.when(j >= 2)
                def _():
                    cp_rows((j - 2) * SPI, SPI).start()

            mem = mem_ref[...]
            for t in range(SPI):
                sg = j * SPI + t
                sp = jnp.maximum(sg - 1, 0) if t == 0 else sg - 1
                sw = jnp.where(sg == 0, NSEG, sp) if t == 0 else sp
                sn = jnp.minimum(sg + 1, NSEG - 1) if t == SPI - 1 else sg + 1
                h = jnp.concatenate([xnb_ref[t % 2], mem], axis=0)
                chain = []
                side = [[] for _ in range(NPB)]
                for i in range(2):
                    side[1 + 2 * i].append(functools.partial(b_finish, first, sp, sw, (t + 1) % 2, i, chain))
                if not first:
                    for n in range(D // 128):
                        side[n].append(functools.partial(a_finish, sn, sg + 1, n))
                for i in range(4):
                    side[6 + 2 * i].append(functools.partial(a_norm, first, sn, (t + 1) % 2, i, chain))
                y = b_step(h, side, chain)
                mem = y[0:MEM]
                yb_ref[t % 2] = y[MEM:L]
            mem_ref[...] = mem
            return carry

        with jax.named_scope("b_loop"):
            lax.fori_loop(0, NB, body, 0)
        if not first:
            cp_rows(NSEG - 2 * SPI, 2 * SPI - 1).start()
        for i in range(2):
            b_finish(first, NSEG - 1, NSEG - 1, 1, i, [])

    for first in (True, False):
        kv_ref[...] = jnp.zeros(kv_ref.shape, f32)
        with jax.named_scope("a_p1"):
            a_phase1(first)
        with jax.named_scope("a_p2"):
            a_phase2(first)
        with jax.named_scope("layer_b"):
            layer_b(first)

    cp_rows(NSEG - 1, 1).start()
    cp_rows(0, NSEG).wait()


@jax.jit
def pallas_interleave_layers__linear_kernel_hedgehog__memory_aug_recurrent_mem_tr__prompt_kernel(
    A_x: jax.Array,
    A_wqkv: jax.Array,
    A_w_phi: jax.Array,
    A_wo: jax.Array,
    B_x: jax.Array,
    B_mem0: jax.Array,
    B_Wq: jax.Array,
    B_Wk: jax.Array,
    B_Wv: jax.Array,
    B_Wo: jax.Array,
    B_seg_len: jax.Array,
):
    del B_x, B_seg_len
    x = A_x.reshape(S, D)
    phi = A_w_phi.transpose(1, 2, 0)
    wqt = B_Wq.transpose(1, 2, 0).reshape(HD, D)
    wkt = B_Wk.transpose(1, 2, 0).reshape(HD, D)
    wvt = B_Wv.transpose(1, 2, 0).reshape(HD, D)
    wo = B_Wo.reshape(HD, D)
    hbm = pl.BlockSpec(memory_space=pl.ANY)
    out = pl.pallas_call(
        _kernel,
        out_shape=jax.ShapeDtypeStruct((S, D), bf16),
        in_specs=[hbm] * 9,
        out_specs=hbm,
        scratch_shapes=[
            pltpu.VMEM((S, D), bf16),
            pltpu.VMEM((3, D, D), bf16),
            pltpu.VMEM((DA, DA, HA), bf16),
            pltpu.VMEM((D, D), bf16),
            pltpu.VMEM((MEM, D), bf16),
            pltpu.VMEM((S + SEG, D), f32),
            pltpu.VMEM((S // 2, D), u32),
            pltpu.VMEM((2, SEG, D), f32),
            pltpu.VMEM((SEG, D), f32),
            pltpu.VMEM((SEG, D), f32),
            pltpu.VMEM((2, SEG, D), f32),
            pltpu.VMEM((S // 2, D), u32),
            pltpu.VMEM((3, GA, 80, D), u32),
            pltpu.VMEM((D // 2, D), u32),
            pltpu.VMEM((2, GA, 160, 256), f32),
            pltpu.VMEM((NCH, NPA, RA, TC), u32),
            pltpu.VMEM((NPA, RA + 8, 2 * RA), f32),
            pltpu.VMEM((NPA, (RA + 8) // 2, 2 * RA), u32),
            pltpu.VMEM((3, HD + TRC, D), bf16),
            pltpu.VMEM((3, NPB + 2, D // 2, PW), u32),
            pltpu.VMEM((D // 128, HD, 128) if WOMODE < 2 else (HD, D), bf16),
            pltpu.VMEM((MEM, D), f32),
            pltpu.VMEM((L, HD), f32),
            pltpu.SemaphoreType.DMA((20 + 3 * NTR,)),
        ],
        compiler_params=pltpu.CompilerParams(vmem_limit_bytes=120 * 1024 * 1024),
    )(x, A_wqkv, phi, A_wo, B_mem0.reshape(MEM, D), wqt, wkt, wvt, wo)
    return out.reshape(1, S, D)
```

```python
import functools
import os

import jax
import jax.numpy as jnp
from jax import lax
import jax.experimental.pallas as pl
import jax.experimental.pallas.tpu as pltpu

f32, bf16, u32, i32 = jnp.float32, jnp.bfloat16, jnp.uint32, jnp.int32

S, D = 2048, 640
HA, DA = 32, 20
NPA = HA // 2
RA = 2 * DA
GA = 4
TC = 256
NCH = S // TC
XCH = int(os.environ.get("XCH", "256"))
HB, DB, MEM, SEG = 32, 192, 8, 32
HD = HB * DB
L = MEM + SEG
LM = L - 8
VBLK = (0, 192, 64, 256, 128, 320)
NPB = HB // 2
PW = 2 * DB
SCALE = DB ** -0.5
TRC = 768
NTR = HD // TRC
NSEG = S // SEG
SPI = int(os.environ.get("SPI", "2"))
NB = NSEG // SPI
assert NTR == NCH

SCH = tuple(int(v) for v in os.environ.get("SCH", "1,0,1,4,2,4,7").split(","))
TIE = int(os.environ.get("TIE", "1"))
APPROX = int(os.environ.get("APPROX", "0"))
KVLAG = int(os.environ.get("KVLAG", "12"))
P1U = int(os.environ.get("P1U", "4"))

_NN = (((1,), (0,)), ((), ()))
_NT = (((1,), (1,)), ((), ()))


def _dot(a, b):
    return lax.dot_general(a, b, _NN, preferred_element_type=f32)


def _dot_nt(a, b):
    return lax.dot_general(a, b, _NT, preferred_element_type=f32)


def _pack(x):
    return pltpu.bitcast(x.astype(bf16), u32)


def _unpack(x):
    return pltpu.bitcast(x, bf16)


def _ln(x):
    m = jnp.mean(x, axis=-1, keepdims=True)
    xc = x - m
    r = lax.rsqrt(jnp.mean(xc * xc, axis=-1, keepdims=True) + 1e-5)
    return x * r - m * r


def _ln_chained(x, chain):
    m = jnp.mean(x, axis=-1, keepdims=True)
    xc = x - m
    r = lax.rsqrt(jnp.mean(xc * xc, axis=-1, keepdims=True) + 1e-5)
    chain.append(jnp.minimum(r, 0.0))
    return x * r - m * r


def _fold(op, p):
    r = p[0:8]
    for j in range(1, 5):
        r = op(r, p[8 * j:8 * j + 8])
    r = op(r, pltpu.roll(r, 2, 0))
    return op(r, pltpu.roll(r, 4, 0))


def _tile5(r):
    return jnp.concatenate([r] * 5, axis=0)


def _phi(p):
    ep = jnp.exp(p - _tile5(_fold(jnp.maximum, p)))
    en = jnp.exp(_tile5(_fold(jnp.minimum, p)) - p)
    ep = ep * _tile5(1.0 / _fold(jnp.add, ep))
    en = en * _tile5(1.0 / _fold(jnp.add, en))
    return jnp.concatenate([ep, en], axis=0).astype(bf16)


def _split(k):
    lo = lax.broadcasted_iota(i32, (L, 128), 1) < 64
    z = jnp.zeros((L, 128), f32)
    mid = k[:, 128:256]
    outer = jnp.concatenate([k[:, 0:128], k[:, 256:384]], axis=0).astype(bf16)
    mid = jnp.concatenate([jnp.where(lo, mid, z), jnp.where(lo, z, mid)], axis=0).astype(bf16)
    return outer, mid


def _recip(x):
    return pl.reciprocal(x, approx=True) if APPROX else 1.0 / x


def _probs(q, k, zeros):
    r = lax.broadcasted_iota(i32, (LM, 2 * L), 0)
    c = lax.broadcasted_iota(i32, (LM, 2 * L), 1)
    first = c < L
    so = _dot_nt(q[0], k[0])
    s = jnp.where(first, so[0:LM], so[LM:2 * LM]) + _dot_nt(q[1], k[1])
    s = s * SCALE
    if zeros:
        s = jnp.concatenate([functools.reduce(jnp.add, zeros, s[0:8]), s[8:LM]], axis=0)
    mask = (r < MEM) | (r + 8 >= jnp.where(first, c, c - L))
    s = jnp.where(mask, s, -1000000000.0)
    neg = jnp.full_like(s, -jnp.inf)
    ma = jnp.max(jnp.where(first, s, neg), axis=-1, keepdims=True)
    mb = jnp.max(jnp.where(first, neg, s), axis=-1, keepdims=True)
    e = jnp.exp(s - jnp.where(first, ma, mb))
    z = jnp.zeros_like(e)
    sa = jnp.sum(jnp.where(first, e, z), axis=-1, keepdims=True)
    sb = jnp.sum(jnp.where(first, z, e), axis=-1, keepdims=True)
    return e * _recip(jnp.where(first, sa, sb))


def _kernel(x_hbm, wqkv_hbm, phi_hbm, woa_hbm, mem0_hbm, wqt_hbm, wkt_hbm, wvt_hbm, wo_hbm, out_hbm,
            xin_ref, wqkv, phi_ref, wo_a, mem0, x_ref, xna_ref, xnb_ref, xa_ref, xb_ref, yb_ref, oa_ref,
            wat_ref, wop_ref, lhs_ref, phiq_ref, kv_ref, kvm_ref, stage_ref, wb_ref, wo_ref, mem_ref, o_ref,
            sems):
    cp_phi = pltpu.make_async_copy(phi_hbm, phi_ref, sems.at[0])
    cp_mem0 = pltpu.make_async_copy(mem0_hbm, mem0, sems.at[1])
    cp_woa = pltpu.make_async_copy(woa_hbm, wo_a, sems.at[2])
    big = (wqt_hbm, wkt_hbm, wvt_hbm, wo_hbm)

    def cp_wqkv(n):
        return pltpu.make_async_copy(wqkv_hbm.at[:, pl.ds(pl.multiple_of(D * n, 128), D)], wqkv.at[n],
                                     sems.at[4 + n])

    def cp_x(j):
        rows = pl.ds(pl.multiple_of(j * XCH, XCH), XCH)
        return pltpu.make_async_copy(x_hbm.at[rows, :], xin_ref.at[rows, :], sems.at[12 + j])

    def cp_w(n, j):
        rows = pl.ds(pl.multiple_of(j * TRC, TRC), TRC)
        return pltpu.make_async_copy(big[n].at[rows, :], stage_ref.at[n, rows, :], sems.at[20 + n * NTR + j])

    def cp_rows(sg, nseg):
        rows = pl.ds(pl.multiple_of(sg * SEG, SEG), SEG * nseg)
        return pltpu.make_async_copy(xin_ref.at[rows, :], out_hbm.at[rows, :], sems.at[3])

    cp_phi.start()
    for n in range(3):
        cp_wqkv(n).start()
    for j in range(S // XCH):
        cp_x(j).start()
    cp_mem0.start()
    for j in range(NTR):
        if j == NTR - 1:
            cp_woa.start()
        for n in range(3):
            cp_w(n, j).start()
    for j in range(NTR):
        cp_w(3, j).start()

    def init_x(c, carry):
        with jax.named_scope("wait_x"):
            cp_x(c).wait()
        x = xin_ref[pl.ds(pl.multiple_of(c * XCH, XCH), XCH), :].astype(f32)
        x_ref[pl.ds(pl.multiple_of(c * XCH, XCH), XCH), :] = x
        xna_ref[pl.ds(pl.multiple_of(c * (XCH // 2), XCH // 2), XCH // 2), :] = _pack(_ln(x))
        return carry

    with jax.named_scope("wait_phi"):
        cp_phi.wait()
    ecol = lax.broadcasted_iota(i32, (HA, D), 1) - DA * lax.broadcasted_iota(i32, (HA, D), 0)
    def scatter_phi(i, tp):
        for d in range(5):
            tp = tp + _dot(phi_ref[5 * i + d], jnp.where(ecol == 5 * i + d, 1.0, 0.0).astype(bf16))
        return tp

    tp = lax.fori_loop(0, DA // 5, scatter_phi, jnp.zeros((DA, D), f32))
    rep = jnp.where((lax.broadcasted_iota(i32, (RA, DA), 0) >> 1) == lax.broadcasted_iota(i32, (RA, DA), 1),
                    1.0, 0.0).astype(bf16)
    urep = _dot(rep, tp.astype(bf16))
    for g in range(GA):
        col = lax.broadcasted_iota(i32, (RA, 256), 1) + 128 * g
        par = lax.broadcasted_iota(i32, (RA, 256), 0) & 1
        for pp in range(4):
            lo = (8 * g + 2 * pp + par) * DA
            blk = jnp.where((col >= lo) & (col < lo + DA), urep[:, 128 * g:128 * g + 256], 0.0)
            lhs_ref[0, g, RA * pp:RA * pp + RA, :] = blk
        lhs_ref[1, g] = jnp.where(lax.broadcasted_iota(i32, (160, 256), 1) + 128 * g
                                  == lax.broadcasted_iota(i32, (160, 256), 0) + 160 * g, 1.0, 0.0)

    def prep(n, carry):
        with jax.named_scope("wait_wqkv"):
            cp_wqkv(n).wait()
        for g in range(GA):
            wat_ref[n, g] = _pack(_dot_nt(lhs_ref[n // 2, g].astype(bf16), wqkv[n, :, 128 * g:128 * g + 256]))
        return carry

    with jax.named_scope("prep"):
        lax.fori_loop(0, 3, prep, 0)
    with jax.named_scope("init_x"):
        lax.fori_loop(0, S // XCH, init_x, 0)
        cp_mem0.wait()

    def transpose_w(n, p):
        blocks = []
        for i in range(6):
            off = jnp.where(n == 2, VBLK[i], 64 * i)
            blocks.append(stage_ref[n, pl.ds(pl.multiple_of(p * PW + off, 64), 64), :])
        wb_ref[n, p] = pltpu.bitcast(jnp.concatenate(blocks, axis=0).T, u32)

    def pack_wo(j):
        for i in range(12):
            src = pl.ds(pl.multiple_of(j * TRC + (i // 6) * PW + VBLK[i % 6], 64), 64)
            wo_ref[pl.ds(pl.multiple_of(j * (TRC // 2) + 32 * i, 32), 32), :] = pltpu.bitcast(
                stage_ref[3, src, :], u32)

    def a_phase1(first):
        def body(c, carry):
            if first:
                ct = jnp.where(c == 0, NTR, c - 1)

                @pl.when(c > 0)
                def _():
                    with jax.named_scope("wait_w"):
                        for n in range(3):
                            cp_w(n, c - 1).wait()

            xn = _unpack(xna_ref[pl.ds(pl.multiple_of(c * (TC // 2), TC // 2), TC // 2), :])
            ones = jnp.ones((8, TC), f32)
            pend = []

            def flush(n):
                while len(pend) > n:
                    p, vext, phik = pend.pop(0)
                    kv_ref[p] += _dot_nt(vext, phik)

            for g in range(GA):
                pq = _dot_nt(_unpack(wat_ref[0, g]), xn)
                flush(KVLAG)
                pk = _dot_nt(_unpack(wat_ref[1, g]), xn)
                vt = _dot_nt(_unpack(wat_ref[2, g]), xn)
                for pp in range(4):
                    p = 4 * g + pp
                    sl = slice(RA * pp, RA * pp + RA)
                    phiq_ref[c, p] = pltpu.bitcast(_phi(pq[sl]), u32)
                    vext = jnp.concatenate([vt[sl], ones], axis=0).astype(bf16)
                    pend.append((p, vext, _phi(pk[sl])))
                if first and g < 3:
                    transpose_w(g, 2 * ct)
                    transpose_w(g, 2 * ct + 1)
            flush(0)
            return carry

        lax.fori_loop(0, NCH, body, 0, unroll=1 if first else P1U)

    def seg_rows(sg, off=0, n=SEG):
        return pl.ds(pl.multiple_of(sg * SEG + off, 8), n)

    def a_finish(sr, sw, n):
        cols = slice(128 * n, 128 * n + 128)
        y = _dot(_unpack(oa_ref[pl.ds(pl.multiple_of(sr * (SEG // 2), SEG // 2), SEG // 2), :]),
                 _unpack(wop_ref[:, cols]))
        x = x_ref[seg_rows(sr), cols] + y
        x_ref[seg_rows(sw), cols] = x
        xa_ref[:, cols] = x

    def a_norm(first, sg, slot, i, chain):
        x = x_ref[seg_rows(sg, 8 * i, 8), :] if first else xa_ref[8 * i:8 * i + 8, :]
        xnb_ref[slot, 8 * i:8 * i + 8, :] = _ln_chained(x, chain)

    def a_phase2(first):
        r = lax.broadcasted_iota(i32, (RA + 8, 2 * RA), 0)
        rb = jnp.where(((r >= DA) & (r < RA)) | (r >= RA + 4), 1, 0)
        same = rb == (lax.broadcasted_iota(i32, (RA + 8, 2 * RA), 1) & 1)
        for p in range(NPA):
            kvm_ref[p] = _pack(jnp.where(same, kv_ref[p], 0.0))

        def attend(c):
            top = lax.broadcasted_iota(i32, (8, TC), 0) < 4
            ot = []
            for p in range(NPA):
                ne = _dot(_unpack(kvm_ref[p]), _unpack(phiq_ref[c, p]))
                rc = 1.0 / (ne[RA:RA + 8] + 1e-6)
                sw = pltpu.roll(rc, 4, 0)
                ra, rb = jnp.where(top, rc, sw), jnp.where(top, sw, rc)
                ot.append(ne[0:RA] * jnp.concatenate([ra, ra, rc, rb, rb], axis=0))
            o = jnp.concatenate(ot, axis=0).T
            oa_ref[pl.ds(pl.multiple_of(c * (TC // 2), TC // 2), TC // 2), :] = _pack(o)

        if not first:
            wop_ref[...] = pltpu.bitcast(wo_a[...], u32)
            for c in range(NCH):
                attend(c)
                if c == 2:
                    for n in range(D // 128):
                        a_finish(0, 0, n)
                    for i in range(4):
                        a_norm(False, 0, 0, i, [])
            return

        attend(0)
        cp_woa.wait()

        def body(c, carry):
            @pl.when(c == 2)
            def _():
                for n in range(3):
                    cp_w(n, NTR - 1).wait()

            @pl.when(c >= 2)
            def _():
                cp_w(3, c - 2).wait()

            lhs = [_unpack(oa_ref[pl.ds(pl.multiple_of(c * (TC // 2) + r // 2, 64), 64), :])
                   for r in range(0, TC, 128)]
            attend(jnp.minimum(c + 1, NCH - 1))
            t = jnp.maximum(c - 2, 0)
            transpose_w(t // 2, jnp.where(c < 2, NPB, NPB - 2 + t % 2))
            pack_wo(jnp.where(c < 2, NTR, t))
            for r in range(0, TC, 128):
                x_ref[pl.ds(pl.multiple_of(c * TC + r, 128), 128), :] += _dot(lhs[r // 128], wo_a[...])
            return carry

        lax.fori_loop(0, NCH, body, 0)

    def b_finish(first, sr, sw, slot, i, chain):
        x = x_ref[seg_rows(sr, 16 * i, 16), :] + yb_ref[slot, 16 * i:16 * i + 16, :]
        if first:
            x_ref[seg_rows(sw, 16 * i, 16), :] = x
            xb_ref[16 * i:16 * i + 16, :] = x
            xn = [_ln_chained(xb_ref[16 * i + k:16 * i + k + 8, :], chain) for k in (0, 8)]
            xna_ref[pl.ds(pl.multiple_of(sr * (SEG // 2) + 8 * i, 8), 8), :] = _pack(
                jnp.concatenate(xn, axis=0))
        else:
            xin_ref[pl.ds(pl.multiple_of(sr * SEG + 16 * i, 16), 16), :] = x.astype(bf16)

    def b_step(h, side, chain):
        st = {}

        def proj(p, which):
            if p == 0 and which == 0:
                y = _dot(h[:, 0:128], _unpack(wb_ref[0, 0, 0:64, :]))
                for k in range(1, D // 128):
                    y = y + _dot(h[:, 128 * k:128 * k + 128], _unpack(wb_ref[0, 0, 64 * k:64 * k + 64, :]))
            else:
                y = _dot(h, _unpack(wb_ref[which, p]))
            if which == 0:
                st[(p, 'qv')] = y[0:8] * SCALE
                y = jnp.concatenate([y[SEG:L], y[8:SEG]], axis=0)
                st[(p, 0)] = (jnp.concatenate([y[:, 0:128], y[:, 256:384]], axis=0).astype(bf16), y[:, 128:256])
                return
            y = jnp.concatenate([y[SEG:L], y[0:SEG]], axis=0)
            st[(p, 'kv', which)] = y[0:16]
            if which == 1:
                st[(p, 1)] = _split(y)
            else:
                lo = (lax.broadcasted_iota(i32, (L, PW), 1) & 64) == 0
                st[(p, 2)] = jnp.concatenate([jnp.where(lo, y, 0.0), jnp.where(lo, 0.0, y)], axis=0).astype(bf16)

        def do_qk(p):
            zeros = chain[:1] + st.pop('tie', [])
            del chain[:1]
            st[(p, 'p')] = _probs(st.pop((p, 0)), st.pop((p, 1)), zeros)

        def do_pv(p):
            cols = slice(p * PW, (p + 1) * PW)
            o = _dot(st.pop((p, 'p')), st.pop((p, 2)))
            o_ref[0:MEM, cols] = o[0:MEM]
            o_ref[2 * MEM:L, cols] = o[MEM:LM]
            lo = lax.broadcasted_iota(i32, (8, 128), 1) < 64
            row = lax.broadcasted_iota(i32, (8, 128), 0)
            q = st.pop((p, 'qv'))
            qa, qb = jnp.where(lo, q[:, 128:256], 0.0), jnp.where(lo, 0.0, q[:, 128:256])

            kv = (st.pop((p, 'kv', 1)), st.pop((p, 'kv', 2)))

            def key_row(which, k, t):
                return kv[which][k:k + 1, 128 * t:128 * t + 128]

            sc = []
            for k in range(16):
                km = key_row(0, k, 1)
                xa = jnp.sum(q[:, 0:128] * key_row(0, k, 0) + qa * km, axis=-1, keepdims=True)
                xb = jnp.sum(q[:, 256:384] * key_row(0, k, 2) + qb * km, axis=-1, keepdims=True)
                x = jnp.where(lo, xa, xb)
                sc.append(jnp.where(row >= k - MEM, x, -1000000000.0) if k > MEM else x)
            m = functools.reduce(jnp.maximum, sc)
            ev = [jnp.exp(x - m) for x in sc]
            rr = _recip(functools.reduce(jnp.add, ev))
            ov = [functools.reduce(jnp.add, [ev[k] * key_row(1, k, t) for k in range(16)]) * rr
                  for t in range(3)]
            o_ref[MEM:2 * MEM, cols] = jnp.concatenate(ov, axis=1)
            if TIE:
                z = jnp.minimum(functools.reduce(jnp.maximum, [jnp.abs(x) for x in ov]), 0.0)
                st['tie'] = [z[:, 0:2 * L]]

        def do_o(n):
            k0 = st.get('k', 0)
            k1 = min(k0 + n, HD // 128)
            if k0 == k1:
                return
            st['k'] = k1
            y = _dot(o_ref[:, k0 * 128:k1 * 128], _unpack(wo_ref[k0 * 64:k1 * 64, :]))
            st['y'] = y if 'y' not in st else st['y'] + y

        o1, o2, o3, olag, f1, f2, f3 = SCH
        for s in range(NPB):
            on = s >= olag
            proj(s, 0)
            if on:
                do_o(o1)
            if s >= 1:
                do_qk(s - 1)
            proj(s, 1)
            if on:
                do_o(o2)
            if s >= 2:
                do_pv(s - 2)
            proj(s, 2)
            if on:
                do_o(o3)
            for job in side[s]:
                job()
            assert st.get('k', 0) <= 3 * max(s - 2, 0)
        do_o(f1)
        do_qk(NPB - 1)
        do_o(f2)
        do_pv(NPB - 2)
        do_o(f3)
        assert st.get('k', 0) <= 3 * (NPB - 2)
        do_pv(NPB - 1)
        do_o(3 * (NPB - 1) - st['k'])
        do_o(3)
        return st['y']

    def layer_b(first):
        mem_ref[...] = mem0[...].astype(f32)
        yb_ref[1] = jnp.zeros((SEG, D), f32)
        if first:
            for i in range(4):
                a_norm(first, 0, 0, i, [])
            with jax.named_scope("wait_wo"):
                for j in range(NTR - 2, NTR):
                    cp_w(3, j).wait()
                    pack_wo(j)

        def body(j, carry):
            if not first:
                @pl.when(j >= 2)
                def _():
                    cp_rows((j - 2) * SPI, SPI).start()

            mem = mem_ref[...]
            for t in range(SPI):
                sg = j * SPI + t
                sp = jnp.maximum(sg - 1, 0) if t == 0 else sg - 1
                sw = jnp.where(sg == 0, NSEG, sp) if t == 0 else sp
                sn = jnp.minimum(sg + 1, NSEG - 1) if t == SPI - 1 else sg + 1
                h = jnp.concatenate([xnb_ref[t % 2], mem], axis=0)
                chain = []
                side = [[] for _ in range(NPB)]
                for i in range(2):
                    side[1 + 2 * i].append(functools.partial(b_finish, first, sp, sw, (t + 1) % 2, i, chain))
                if not first:
                    for n in range(D // 128):
                        side[n].append(functools.partial(a_finish, sn, sg + 1, n))
                for i in range(4):
                    side[6 + 2 * i].append(functools.partial(a_norm, first, sn, (t + 1) % 2, i, chain))
                y = b_step(h, side, chain)
                mem = y[0:MEM]
                yb_ref[t % 2] = y[MEM:L]
            mem_ref[...] = mem
            return carry

        with jax.named_scope("b_loop"):
            lax.fori_loop(0, NB, body, 0)
        if not first:
            cp_rows(NSEG - 2 * SPI, 2 * SPI - 1).start()
        for i in range(2):
            b_finish(first, NSEG - 1, NSEG - 1, 1, i, [])

    for first in (True, False):
        kv_ref[...] = jnp.zeros(kv_ref.shape, f32)
        with jax.named_scope("a_p1"):
            a_phase1(first)
        with jax.named_scope("a_p2"):
            a_phase2(first)
        with jax.named_scope("layer_b"):
            layer_b(first)

    cp_rows(NSEG - 1, 1).start()
    cp_rows(0, NSEG).wait()


@jax.jit
def pallas_interleave_layers__linear_kernel_hedgehog__memory_aug_recurrent_mem_tr__prompt_kernel(
    A_x: jax.Array,
    A_wqkv: jax.Array,
    A_w_phi: jax.Array,
    A_wo: jax.Array,
    B_x: jax.Array,
    B_mem0: jax.Array,
    B_Wq: jax.Array,
    B_Wk: jax.Array,
    B_Wv: jax.Array,
    B_Wo: jax.Array,
    B_seg_len: jax.Array,
):
    del B_x, B_seg_len
    x = A_x.reshape(S, D)
    phi = A_w_phi.transpose(1, 2, 0)
    wqt = B_Wq.transpose(1, 2, 0).reshape(HD, D)
    wkt = B_Wk.transpose(1, 2, 0).reshape(HD, D)
    wvt = B_Wv.transpose(1, 2, 0).reshape(HD, D)
    wo = B_Wo.reshape(HD, D)
    hbm = pl.BlockSpec(memory_space=pl.ANY)
    out = pl.pallas_call(
        _kernel,
        out_shape=jax.ShapeDtypeStruct((S, D), bf16),
        in_specs=[hbm] * 9,
        out_specs=hbm,
        scratch_shapes=[
            pltpu.VMEM((S, D), bf16),
            pltpu.VMEM((3, D, D), bf16),
            pltpu.VMEM((DA, DA, HA), bf16),
            pltpu.VMEM((D, D), bf16),
            pltpu.VMEM((MEM, D), bf16),
            pltpu.VMEM((S + SEG, D), f32),
            pltpu.VMEM((S // 2, D), u32),
            pltpu.VMEM((2, SEG, D), f32),
            pltpu.VMEM((SEG, D), f32),
            pltpu.VMEM((SEG, D), f32),
            pltpu.VMEM((2, SEG, D), f32),
            pltpu.VMEM((S // 2, D), u32),
            pltpu.VMEM((3, GA, 80, D), u32),
            pltpu.VMEM((D // 2, D), u32),
            pltpu.VMEM((2, GA, 160, 256), f32),
            pltpu.VMEM((NCH, NPA, RA, TC), u32),
            pltpu.VMEM((NPA, RA + 8, 2 * RA), f32),
            pltpu.VMEM((NPA, (RA + 8) // 2, 2 * RA), u32),
            pltpu.VMEM((4, HD + TRC, D), bf16),
            pltpu.VMEM((3, NPB + 2, D // 2, PW), u32),
            pltpu.VMEM(((HD + TRC) // 2, D), u32),
            pltpu.VMEM((MEM, D), f32),
            pltpu.VMEM((L, HD), f32),
            pltpu.SemaphoreType.DMA((20 + 4 * NTR,)),
        ],
        compiler_params=pltpu.CompilerParams(vmem_limit_bytes=120 * 1024 * 1024),
    )(x, A_wqkv, phi, A_wo, B_mem0.reshape(MEM, D), wqt, wkt, wvt, wo)
    return out.reshape(1, S, D)
```

```python
import functools
import os

import jax
import jax.numpy as jnp
from jax import lax
import jax.experimental.pallas as pl
import jax.experimental.pallas.tpu as pltpu

f32, bf16, u32, i32 = jnp.float32, jnp.bfloat16, jnp.uint32, jnp.int32

S, D = 2048, 640
HA, DA = 32, 20
NPA = HA // 2
RA = 2 * DA
GA = 4
TC = 256
NCH = S // TC
XCH = int(os.environ.get("XCH", "256"))
HB, DB, MEM, SEG = 32, 192, 8, 32
HD = HB * DB
L = MEM + SEG
LM = L - 8
VBLK = (0, 192, 64, 256, 128, 320)
NPB = HB // 2
PW = 2 * DB
SCALE = DB ** -0.5 * 1.4426950408889634
TRC = 768
NTR = HD // TRC
NSEG = S // SEG
SPI = int(os.environ.get("SPI", "2"))
NB = NSEG // SPI
assert NTR == NCH

SCH = tuple(int(v) for v in os.environ.get("SCH", "1,0,1,4,2,4,7").split(","))
VLAG = int(os.environ.get("VLAG", "1"))
VPOS = int(os.environ.get("VPOS", "1"))
KVLAG = int(os.environ.get("KVLAG", "12"))
P1U = int(os.environ.get("P1U", "4"))

_NN = (((1,), (0,)), ((), ()))
_NT = (((1,), (1,)), ((), ()))


def _dot(a, b):
    return lax.dot_general(a, b, _NN, preferred_element_type=f32)


def _dot_nt(a, b):
    return lax.dot_general(a, b, _NT, preferred_element_type=f32)


def _pack(x):
    return pltpu.bitcast(x.astype(bf16), u32)


def _unpack(x):
    return pltpu.bitcast(x, bf16)


def _ln(x):
    m = jnp.mean(x, axis=-1, keepdims=True)
    xc = x - m
    r = lax.rsqrt(jnp.mean(xc * xc, axis=-1, keepdims=True) + 1e-5)
    return x * r - m * r


def _ln_chained(x, chain):
    m = jnp.mean(x, axis=-1, keepdims=True)
    xc = x - m
    r = lax.rsqrt(jnp.mean(xc * xc, axis=-1, keepdims=True) + 1e-5)
    chain.append(jnp.minimum(r, 0.0))
    return x * r - m * r


def _fold(op, p):
    r = p[0:8]
    for j in range(1, 5):
        r = op(r, p[8 * j:8 * j + 8])
    r = op(r, pltpu.roll(r, 2, 0))
    return op(r, pltpu.roll(r, 4, 0))


def _tile5(r):
    return jnp.concatenate([r] * 5, axis=0)


def _phi(p):
    ep = jnp.exp(p - _tile5(_fold(jnp.maximum, p)))
    en = jnp.exp(_tile5(_fold(jnp.minimum, p)) - p)
    ep = ep * _tile5(1.0 / _fold(jnp.add, ep))
    en = en * _tile5(1.0 / _fold(jnp.add, en))
    return jnp.concatenate([ep, en], axis=0).astype(bf16)


def _split(k):
    lo = lax.broadcasted_iota(i32, (L, 128), 1) < 64
    z = jnp.zeros((L, 128), f32)
    mid = k[:, 128:256]
    outer = jnp.concatenate([k[:, 0:128], k[:, 256:384]], axis=0).astype(bf16)
    mid = jnp.concatenate([jnp.where(lo, mid, z), jnp.where(lo, z, mid)], axis=0).astype(bf16)
    return outer, mid


def _zero(x):
    return jnp.minimum(jnp.abs(x), 0.0)


def _probs(q, k, zeros):
    r = lax.broadcasted_iota(i32, (LM, 2 * L), 0)
    c = lax.broadcasted_iota(i32, (LM, 2 * L), 1)
    first = c < L
    so = _dot_nt(q[0], k[0])
    s = jnp.where(first, so[0:LM], so[LM:2 * LM]) + _dot_nt(q[1], k[1])
    s = s * SCALE
    if zeros:
        s = jnp.concatenate([functools.reduce(jnp.add, zeros, s[0:8]), s[8:LM]], axis=0)
    mask = (r < MEM) | (r + 8 >= jnp.where(first, c, c - L))
    s = jnp.where(mask, s, -1000000000.0)
    neg = jnp.full_like(s, -jnp.inf)
    ma = jnp.max(jnp.where(first, s, neg), axis=-1, keepdims=True)
    mb = jnp.max(jnp.where(first, neg, s), axis=-1, keepdims=True)
    e = jnp.exp2(s - jnp.where(first, ma, mb))
    z = jnp.zeros_like(e)
    sa = jnp.sum(jnp.where(first, e, z), axis=-1, keepdims=True)
    sb = jnp.sum(jnp.where(first, z, e), axis=-1, keepdims=True)
    return e * (1.0 / jnp.where(first, sa, sb))


def _kernel(x_hbm, wqkv_hbm, phi_hbm, woa_hbm, mem0_hbm, wqt_hbm, wkt_hbm, wvt_hbm, wo_hbm, out_hbm,
            xin_ref, wqkv, phi_ref, wo_a, mem0, x_ref, xna_ref, xnb_ref, xa_ref, xb_ref, yb_ref, oa_ref,
            wat_ref, wop_ref, lhs_ref, phiq_ref, kv_ref, kvm_ref, stage_ref, wb_ref, wo_ref, mem_ref, o_ref,
            sems):
    cp_phi = pltpu.make_async_copy(phi_hbm, phi_ref, sems.at[0])
    cp_mem0 = pltpu.make_async_copy(mem0_hbm, mem0, sems.at[1])
    cp_woa = pltpu.make_async_copy(woa_hbm, wo_a, sems.at[2])
    big = (wqt_hbm, wkt_hbm, wvt_hbm, wo_hbm)

    def cp_wqkv(n):
        return pltpu.make_async_copy(wqkv_hbm.at[:, pl.ds(pl.multiple_of(D * n, 128), D)], wqkv.at[n],
                                     sems.at[4 + n])

    def cp_x(j):
        rows = pl.ds(pl.multiple_of(j * XCH, XCH), XCH)
        return pltpu.make_async_copy(x_hbm.at[rows, :], xin_ref.at[rows, :], sems.at[12 + j])

    def cp_w(n, j):
        rows = pl.ds(pl.multiple_of(j * TRC, TRC), TRC)
        return pltpu.make_async_copy(big[n].at[rows, :], stage_ref.at[n, rows, :], sems.at[20 + n * NTR + j])

    def cp_rows(sg, nseg):
        rows = pl.ds(pl.multiple_of(sg * SEG, SEG), SEG * nseg)
        return pltpu.make_async_copy(xin_ref.at[rows, :], out_hbm.at[rows, :], sems.at[3])

    cp_phi.start()
    for n in range(3):
        cp_wqkv(n).start()
    for j in range(S // XCH):
        cp_x(j).start()
    cp_mem0.start()
    for j in range(NTR):
        if j == NTR - 1:
            cp_woa.start()
        for n in range(3):
            cp_w(n, j).start()
    for j in range(NTR):
        cp_w(3, j).start()

    def init_x(c, carry):
        with jax.named_scope("wait_x"):
            cp_x(c).wait()
        x = xin_ref[pl.ds(pl.multiple_of(c * XCH, XCH), XCH), :].astype(f32)
        x_ref[pl.ds(pl.multiple_of(c * XCH, XCH), XCH), :] = x
        xna_ref[pl.ds(pl.multiple_of(c * (XCH // 2), XCH // 2), XCH // 2), :] = _pack(_ln(x))
        return carry

    with jax.named_scope("wait_phi"):
        cp_phi.wait()
    ecol = lax.broadcasted_iota(i32, (HA, D), 1) - DA * lax.broadcasted_iota(i32, (HA, D), 0)
    def scatter_phi(i, tp):
        for d in range(5):
            tp = tp + _dot(phi_ref[5 * i + d], jnp.where(ecol == 5 * i + d, 1.0, 0.0).astype(bf16))
        return tp

    tp = lax.fori_loop(0, DA // 5, scatter_phi, jnp.zeros((DA, D), f32))
    rep = jnp.where((lax.broadcasted_iota(i32, (RA, DA), 0) >> 1) == lax.broadcasted_iota(i32, (RA, DA), 1),
                    1.0, 0.0).astype(bf16)
    urep = _dot(rep, tp.astype(bf16))
    for g in range(GA):
        col = lax.broadcasted_iota(i32, (RA, 256), 1) + 128 * g
        par = lax.broadcasted_iota(i32, (RA, 256), 0) & 1
        for pp in range(4):
            lo = (8 * g + 2 * pp + par) * DA
            blk = jnp.where((col >= lo) & (col < lo + DA), urep[:, 128 * g:128 * g + 256], 0.0)
            lhs_ref[0, g, RA * pp:RA * pp + RA, :] = blk
        lhs_ref[1, g] = jnp.where(lax.broadcasted_iota(i32, (160, 256), 1) + 128 * g
                                  == lax.broadcasted_iota(i32, (160, 256), 0) + 160 * g, 1.0, 0.0)

    def prep(n, carry):
        with jax.named_scope("wait_wqkv"):
            cp_wqkv(n).wait()
        for g in range(GA):
            wat_ref[n, g] = _pack(_dot_nt(lhs_ref[n // 2, g].astype(bf16), wqkv[n, :, 128 * g:128 * g + 256]))
        return carry

    with jax.named_scope("prep"):
        lax.fori_loop(0, 3, prep, 0)
    with jax.named_scope("init_x"):
        lax.fori_loop(0, S // XCH, init_x, 0)
        cp_mem0.wait()

    def transpose_w(n, p):
        blocks = []
        for i in range(6):
            off = jnp.where(n == 2, VBLK[i], 64 * i)
            blocks.append(stage_ref[n, pl.ds(pl.multiple_of(p * PW + off, 64), 64), :])
        wb_ref[n, p] = pltpu.bitcast(jnp.concatenate(blocks, axis=0).T, u32)

    def pack_wo(j):
        for i in range(12):
            src = pl.ds(pl.multiple_of(j * TRC + (i // 6) * PW + VBLK[i % 6], 64), 64)
            wo_ref[pl.ds(pl.multiple_of(j * (TRC // 2) + 32 * i, 32), 32), :] = pltpu.bitcast(
                stage_ref[3, src, :], u32)

    def a_phase1(first):
        def body(c, carry):
            if first:
                ct = jnp.where(c == 0, NTR, c - 1)

                @pl.when(c > 0)
                def _():
                    with jax.named_scope("wait_w"):
                        for n in range(3):
                            cp_w(n, c - 1).wait()

            xn = _unpack(xna_ref[pl.ds(pl.multiple_of(c * (TC // 2), TC // 2), TC // 2), :])
            ones = jnp.ones((8, TC), f32)
            pend = []

            def flush(n):
                while len(pend) > n:
                    p, vext, phik = pend.pop(0)
                    kv_ref[p] += _dot_nt(vext, phik)

            for g in range(GA):
                pq = _dot_nt(_unpack(wat_ref[0, g]), xn)
                flush(KVLAG)
                pk = _dot_nt(_unpack(wat_ref[1, g]), xn)
                vt = _dot_nt(_unpack(wat_ref[2, g]), xn)
                for pp in range(4):
                    p = 4 * g + pp
                    sl = slice(RA * pp, RA * pp + RA)
                    phiq_ref[c, p] = pltpu.bitcast(_phi(pq[sl]), u32)
                    vext = jnp.concatenate([vt[sl], ones], axis=0).astype(bf16)
                    pend.append((p, vext, _phi(pk[sl])))
                if first and g < 3:
                    transpose_w(g, 2 * ct)
                    transpose_w(g, 2 * ct + 1)
            flush(0)
            return carry

        lax.fori_loop(0, NCH, body, 0, unroll=1 if first else P1U)

    def seg_rows(sg, off=0, n=SEG):
        return pl.ds(pl.multiple_of(sg * SEG + off, 8), n)

    def a_finish(sr, sw, n):
        cols = slice(128 * n, 128 * n + 128)
        y = _dot(_unpack(oa_ref[pl.ds(pl.multiple_of(sr * (SEG // 2), SEG // 2), SEG // 2), :]),
                 _unpack(wop_ref[:, cols]))
        x = x_ref[seg_rows(sr), cols] + y
        x_ref[seg_rows(sw), cols] = x
        xa_ref[:, cols] = x

    def a_norm(first, sg, slot, i, chain):
        x = x_ref[seg_rows(sg, 8 * i, 8), :] if first else xa_ref[8 * i:8 * i + 8, :]
        xnb_ref[slot, 8 * i:8 * i + 8, :] = _ln_chained(x, chain)

    def a_phase2(first):
        r = lax.broadcasted_iota(i32, (RA + 8, 2 * RA), 0)
        rb = jnp.where(((r >= DA) & (r < RA)) | (r >= RA + 4), 1, 0)
        same = rb == (lax.broadcasted_iota(i32, (RA + 8, 2 * RA), 1) & 1)
        for p in range(NPA):
            kvm_ref[p] = _pack(jnp.where(same, kv_ref[p], 0.0))

        def attend(c):
            top = lax.broadcasted_iota(i32, (8, TC), 0) < 4
            ot = []
            for p in range(NPA):
                ne = _dot(_unpack(kvm_ref[p]), _unpack(phiq_ref[c, p]))
                rc = 1.0 / (ne[RA:RA + 8] + 1e-6)
                sw = pltpu.roll(rc, 4, 0)
                ra, rb = jnp.where(top, rc, sw), jnp.where(top, sw, rc)
                ot.append(ne[0:RA] * jnp.concatenate([ra, ra, rc, rb, rb], axis=0))
            o = jnp.concatenate(ot, axis=0).T
            oa_ref[pl.ds(pl.multiple_of(c * (TC // 2), TC // 2), TC // 2), :] = _pack(o)

        if not first:
            wop_ref[...] = pltpu.bitcast(wo_a[...], u32)
            for c in range(NCH):
                attend(c)
                if c == 2:
                    for n in range(D // 128):
                        a_finish(0, 0, n)
                    for i in range(4):
                        a_norm(False, 0, 0, i, [])
            return

        attend(0)
        cp_woa.wait()

        def body(c, carry):
            @pl.when(c == 2)
            def _():
                for n in range(3):
                    cp_w(n, NTR - 1).wait()

            @pl.when(c >= 2)
            def _():
                cp_w(3, c - 2).wait()

            lhs = [_unpack(oa_ref[pl.ds(pl.multiple_of(c * (TC // 2) + r // 2, 64), 64), :])
                   for r in range(0, TC, 128)]
            attend(jnp.minimum(c + 1, NCH - 1))
            t = jnp.maximum(c - 2, 0)
            transpose_w(t // 2, jnp.where(c < 2, NPB, NPB - 2 + t % 2))
            pack_wo(jnp.where(c < 2, NTR, t))
            for r in range(0, TC, 128):
                x_ref[pl.ds(pl.multiple_of(c * TC + r, 128), 128), :] += _dot(lhs[r // 128], wo_a[...])
            return carry

        lax.fori_loop(0, NCH, body, 0)

    def b_finish(first, sr, sw, slot, i, chain):
        x = x_ref[seg_rows(sr, 16 * i, 16), :] + yb_ref[slot, 16 * i:16 * i + 16, :]
        if first:
            x_ref[seg_rows(sw, 16 * i, 16), :] = x
            xb_ref[16 * i:16 * i + 16, :] = x
            xn = [_ln_chained(xb_ref[16 * i + k:16 * i + k + 8, :], chain) for k in (0, 8)]
            xna_ref[pl.ds(pl.multiple_of(sr * (SEG // 2) + 8 * i, 8), 8), :] = _pack(
                jnp.concatenate(xn, axis=0))
        else:
            xin_ref[pl.ds(pl.multiple_of(sr * SEG + 16 * i, 16), 16), :] = x.astype(bf16)

    def b_step(h, side, chain):
        st = {}

        def proj(p, which):
            if p == 0 and which == 0:
                y = _dot(h[:, 0:128], _unpack(wb_ref[0, 0, 0:64, :]))
                for k in range(1, D // 128):
                    y = y + _dot(h[:, 128 * k:128 * k + 128], _unpack(wb_ref[0, 0, 64 * k:64 * k + 64, :]))
            else:
                y = _dot(h, _unpack(wb_ref[which, p]))
            if which == 0:
                st[(p, 'qv')] = y[0:8] * SCALE
                y = jnp.concatenate([y[SEG:L], y[8:SEG]], axis=0)
                st[(p, 0)] = (jnp.concatenate([y[:, 0:128], y[:, 256:384]], axis=0).astype(bf16), y[:, 128:256])
                return
            y = jnp.concatenate([y[SEG:L], y[0:SEG]], axis=0)
            st[(p, 'kv', which)] = y[0:16]
            if which == 1:
                st[(p, 1)] = _split(y)
            else:
                lo = (lax.broadcasted_iota(i32, (L, PW), 1) & 64) == 0
                st[(p, 2)] = jnp.concatenate([jnp.where(lo, y, 0.0), jnp.where(lo, 0.0, y)], axis=0).astype(bf16)

        def do_qk(p):
            zeros = chain[:1] + st.pop('tie', [])
            del chain[:1]
            st[(p, 'p')] = _probs(st.pop((p, 0)), st.pop((p, 1)), zeros)

        def do_pv(p):
            cols = slice(p * PW, (p + 1) * PW)
            o = _dot(st.pop((p, 'p')), st.pop((p, 2)))
            o_ref[0:MEM, cols] = o[0:MEM]
            o_ref[2 * MEM:L, cols] = o[MEM:LM]

        def do_vpu(p):
            cols = slice(p * PW, (p + 1) * PW)
            lo = lax.broadcasted_iota(i32, (8, 128), 1) < 64
            row = lax.broadcasted_iota(i32, (8, 128), 0)
            q = st.pop((p, 'qv'))
            qa, qb = jnp.where(lo, q[:, 128:256], 0.0), jnp.where(lo, 0.0, q[:, 128:256])

            kk, vv = st.pop((p, 'kv', 1)), st.pop((p, 'kv', 2))
            sc = []
            for k in range(16):
                km = jnp.broadcast_to(kk[k:k + 1, 128:256], (8, 128))
                xa = jnp.sum(q[:, 0:128] * kk[k:k + 1, 0:128] + qa * km, axis=-1, keepdims=True)
                xb = jnp.sum(q[:, 256:384] * kk[k:k + 1, 256:384] + qb * km, axis=-1, keepdims=True)
                x = jnp.where(lo, xa, xb)
                sc.append(jnp.where(row >= k - MEM, x, -1000000000.0) if k > MEM else x)
            m = functools.reduce(jnp.maximum, sc)
            ev = [jnp.exp2(x - m) for x in sc]
            rr = 1.0 / functools.reduce(jnp.add, ev)
            z = _zero(m)
            ov = []
            for t in range(3):
                v = [vv[8 * b:8 * b + 8, 128 * t:128 * t + 128] + z for b in range(2)]
                ov.append(functools.reduce(
                    jnp.add, [ev[k] * v[k // 8][k % 8:k % 8 + 1] for k in range(16)]) * rr)
                z = _zero(ov[-1])
            o_ref[MEM:2 * MEM, cols] = jnp.concatenate(ov, axis=1)
            st['tie'] = [z[:, 0:2 * L]]

        def do_o(n):
            k0 = st.get('k', 0)
            k1 = min(k0 + n, HD // 128)
            if k0 == k1:
                return
            st['k'] = k1
            y = _dot(o_ref[:, k0 * 128:k1 * 128], _unpack(wo_ref[k0 * 64:k1 * 64, :]))
            st['y'] = y if 'y' not in st else st['y'] + y

        o1, o2, o3, olag, f1, f2, f3 = SCH
        for s in range(NPB):
            on = s >= olag
            proj(s, 0)
            if on:
                do_o(o1)
            if s >= 1:
                do_qk(s - 1)
            if s >= VLAG and VPOS == 0:
                do_vpu(s - VLAG)
            proj(s, 1)
            if on:
                do_o(o2)
            if s >= 2:
                do_pv(s - 2)
            if s >= VLAG and VPOS == 1:
                do_vpu(s - VLAG)
            proj(s, 2)
            if on:
                do_o(o3)
            for job in side[s]:
                job()
            assert st.get('k', 0) <= 3 * max(s - 2, 0)
        do_o(f1)
        do_qk(NPB - 1)
        for p in range(NPB - VLAG, NPB):
            do_vpu(p)
        do_o(f2)
        do_pv(NPB - 2)
        do_o(f3)
        assert st.get('k', 0) <= 3 * (NPB - 2)
        do_pv(NPB - 1)
        do_o(3 * (NPB - 1) - st['k'])
        do_o(3)
        return st['y']

    def layer_b(first):
        mem_ref[...] = mem0[...].astype(f32)
        yb_ref[1] = jnp.zeros((SEG, D), f32)
        if first:
            for i in range(4):
                a_norm(first, 0, 0, i, [])
            with jax.named_scope("wait_wo"):
                for j in range(NTR - 2, NTR):
                    cp_w(3, j).wait()
                    pack_wo(j)

        def body(j, carry):
            if not first:
                @pl.when(j >= 2)
                def _():
                    cp_rows((j - 2) * SPI, SPI).start()

            mem = mem_ref[...]
            for t in range(SPI):
                sg = j * SPI + t
                sp = jnp.maximum(sg - 1, 0) if t == 0 else sg - 1
                sw = jnp.where(sg == 0, NSEG, sp) if t == 0 else sp
                sn = jnp.minimum(sg + 1, NSEG - 1) if t == SPI - 1 else sg + 1
                h = jnp.concatenate([xnb_ref[t % 2], mem], axis=0)
                chain = []
                side = [[] for _ in range(NPB)]
                for i in range(2):
                    side[1 + 2 * i].append(functools.partial(b_finish, first, sp, sw, (t + 1) % 2, i, chain))
                if not first:
                    for n in range(D // 128):
                        side[n].append(functools.partial(a_finish, sn, sg + 1, n))
                for i in range(4):
                    side[6 + 2 * i].append(functools.partial(a_norm, first, sn, (t + 1) % 2, i, chain))
                y = b_step(h, side, chain)
                mem = y[0:MEM]
                yb_ref[t % 2] = y[MEM:L]
            mem_ref[...] = mem
            return carry

        with jax.named_scope("b_loop"):
            lax.fori_loop(0, NB, body, 0)
        if not first:
            cp_rows(NSEG - 2 * SPI, 2 * SPI - 1).start()
        for i in range(2):
            b_finish(first, NSEG - 1, NSEG - 1, 1, i, [])

    for first in (True, False):
        kv_ref[...] = jnp.zeros(kv_ref.shape, f32)
        with jax.named_scope("a_p1"):
            a_phase1(first)
        with jax.named_scope("a_p2"):
            a_phase2(first)
        with jax.named_scope("layer_b"):
            layer_b(first)

    cp_rows(NSEG - 1, 1).start()
    cp_rows(0, NSEG).wait()


@jax.jit
def pallas_interleave_layers__linear_kernel_hedgehog__memory_aug_recurrent_mem_tr__prompt_kernel(
    A_x: jax.Array,
    A_wqkv: jax.Array,
    A_w_phi: jax.Array,
    A_wo: jax.Array,
    B_x: jax.Array,
    B_mem0: jax.Array,
    B_Wq: jax.Array,
    B_Wk: jax.Array,
    B_Wv: jax.Array,
    B_Wo: jax.Array,
    B_seg_len: jax.Array,
):
    del B_x, B_seg_len
    x = A_x.reshape(S, D)
    phi = A_w_phi.transpose(1, 2, 0)
    wqt = B_Wq.transpose(1, 2, 0).reshape(HD, D)
    wkt = B_Wk.transpose(1, 2, 0).reshape(HD, D)
    wvt = B_Wv.transpose(1, 2, 0).reshape(HD, D)
    wo = B_Wo.reshape(HD, D)
    hbm = pl.BlockSpec(memory_space=pl.ANY)
    out = pl.pallas_call(
        _kernel,
        out_shape=jax.ShapeDtypeStruct((S, D), bf16),
        in_specs=[hbm] * 9,
        out_specs=hbm,
        scratch_shapes=[
            pltpu.VMEM((S, D), bf16),
            pltpu.VMEM((3, D, D), bf16),
            pltpu.VMEM((DA, DA, HA), bf16),
            pltpu.VMEM((D, D), bf16),
            pltpu.VMEM((MEM, D), bf16),
            pltpu.VMEM((S + SEG, D), f32),
            pltpu.VMEM((S // 2, D), u32),
            pltpu.VMEM((2, SEG, D), f32),
            pltpu.VMEM((SEG, D), f32),
            pltpu.VMEM((SEG, D), f32),
            pltpu.VMEM((2, SEG, D), f32),
            pltpu.VMEM((S // 2, D), u32),
            pltpu.VMEM((3, GA, 80, D), u32),
            pltpu.VMEM((D // 2, D), u32),
            pltpu.VMEM((2, GA, 160, 256), f32),
            pltpu.VMEM((NCH, NPA, RA, TC), u32),
            pltpu.VMEM((NPA, RA + 8, 2 * RA), f32),
            pltpu.VMEM((NPA, (RA + 8) // 2, 2 * RA), u32),
            pltpu.VMEM((4, HD + TRC, D), bf16),
            pltpu.VMEM((3, NPB + 2, D // 2, PW), u32),
            pltpu.VMEM(((HD + TRC) // 2, D), u32),
            pltpu.VMEM((MEM, D), f32),
            pltpu.VMEM((L, HD), f32),
            pltpu.SemaphoreType.DMA((20 + 4 * NTR,)),
        ],
        compiler_params=pltpu.CompilerParams(vmem_limit_bytes=120 * 1024 * 1024),
    )(x, A_wqkv, phi, A_wo, B_mem0.reshape(MEM, D), wqt, wkt, wvt, wo)
    return out.reshape(1, S, D)
```

```python
import functools
import os

import jax
import jax.numpy as jnp
from jax import lax
import jax.experimental.pallas as pl
import jax.experimental.pallas.tpu as pltpu

f32, bf16, u32, i32 = jnp.float32, jnp.bfloat16, jnp.uint32, jnp.int32

S, D = 2048, 640
HA, DA = 32, 20
NPA = HA // 2
RA = 2 * DA
GA = 4
TC = 256
NCH = S // TC
XCH = int(os.environ.get("XCH", "256"))
HB, DB, MEM, SEG = 32, 192, 8, 32
HD = HB * DB
L = MEM + SEG
LM = L - 8
VBLK = (0, 192, 64, 256, 128, 320)
NPB = HB // 2
PW = 2 * DB
SCALE = DB ** -0.5 * 1.4426950408889634
TRC = 768
NTR = HD // TRC
NSEG = S // SEG
SPI1 = int(os.environ.get("SPI1", "2"))
SPI2 = int(os.environ.get("SPI2", "4"))
assert NTR == NCH

SCH = tuple(int(v) for v in os.environ.get("SCH", "1,0,1,4,2,4,7").split(","))
VLAG = int(os.environ.get("VLAG", "1"))
VPOS = int(os.environ.get("VPOS", "1"))
KVLAG = int(os.environ.get("KVLAG", "12"))
P1U = int(os.environ.get("P1U", "2"))

_NN = (((1,), (0,)), ((), ()))
_NT = (((1,), (1,)), ((), ()))


def _dot(a, b):
    return lax.dot_general(a, b, _NN, preferred_element_type=f32)


def _dot_nt(a, b):
    return lax.dot_general(a, b, _NT, preferred_element_type=f32)


def _pack(x):
    return pltpu.bitcast(x.astype(bf16), u32)


def _unpack(x):
    return pltpu.bitcast(x, bf16)


def _ln(x):
    m = jnp.mean(x, axis=-1, keepdims=True)
    xc = x - m
    r = lax.rsqrt(jnp.mean(xc * xc, axis=-1, keepdims=True) + 1e-5)
    return x * r - m * r


def _ln_chained(x, chain):
    m = jnp.mean(x, axis=-1, keepdims=True)
    xc = x - m
    r = lax.rsqrt(jnp.mean(xc * xc, axis=-1, keepdims=True) + 1e-5)
    chain.append(jnp.minimum(r, 0.0))
    return x * r - m * r


def _fold(op, p):
    r = p[0:8]
    for j in range(1, 5):
        r = op(r, p[8 * j:8 * j + 8])
    r = op(r, pltpu.roll(r, 2, 0))
    return op(r, pltpu.roll(r, 4, 0))


def _tile5(r):
    return jnp.concatenate([r] * 5, axis=0)


def _phi(p):
    ep = jnp.exp(p - _tile5(_fold(jnp.maximum, p)))
    en = jnp.exp(_tile5(_fold(jnp.minimum, p)) - p)
    ep = ep * _tile5(1.0 / _fold(jnp.add, ep))
    en = en * _tile5(1.0 / _fold(jnp.add, en))
    return jnp.concatenate([ep, en], axis=0).astype(bf16)


def _split(k):
    lo = lax.broadcasted_iota(i32, (L, 128), 1) < 64
    z = jnp.zeros((L, 128), f32)
    mid = k[:, 128:256]
    outer = jnp.concatenate([k[:, 0:128], k[:, 256:384]], axis=0).astype(bf16)
    mid = jnp.concatenate([jnp.where(lo, mid, z), jnp.where(lo, z, mid)], axis=0).astype(bf16)
    return outer, mid


def _zero(x):
    return jnp.minimum(jnp.abs(x), 0.0)


def _probs(q, k, zeros):
    r = lax.broadcasted_iota(i32, (LM, 2 * L), 0)
    c = lax.broadcasted_iota(i32, (LM, 2 * L), 1)
    first = c < L
    so = _dot_nt(q[0], k[0])
    s = jnp.where(first, so[0:LM], so[LM:2 * LM]) + _dot_nt(q[1], k[1])
    s = s * SCALE
    if zeros:
        s = jnp.concatenate([functools.reduce(jnp.add, zeros, s[0:8]), s[8:LM]], axis=0)
    mask = (r < MEM) | (r + 8 >= jnp.where(first, c, c - L))
    s = jnp.where(mask, s, -1000000000.0)
    neg = jnp.full_like(s, -jnp.inf)
    ma = jnp.max(jnp.where(first, s, neg), axis=-1, keepdims=True)
    mb = jnp.max(jnp.where(first, neg, s), axis=-1, keepdims=True)
    e = jnp.exp2(s - jnp.where(first, ma, mb))
    z = jnp.zeros_like(e)
    sa = jnp.sum(jnp.where(first, e, z), axis=-1, keepdims=True)
    sb = jnp.sum(jnp.where(first, z, e), axis=-1, keepdims=True)
    return e * (1.0 / jnp.where(first, sa, sb))


def _kernel(x_hbm, wqkv_hbm, phi_hbm, woa_hbm, mem0_hbm, wqt_hbm, wkt_hbm, wvt_hbm, wo_hbm, out_hbm,
            xin_ref, wqkv, phi_ref, wo_a, mem0, x_ref, xna_ref, xnb_ref, xa_ref, xb_ref, yb_ref, oa_ref,
            wat_ref, wop_ref, lhs_ref, phiq_ref, kv_ref, kvm_ref, stage_ref, wb_ref, wo_ref, mem_ref, o_ref,
            sems):
    cp_phi = pltpu.make_async_copy(phi_hbm, phi_ref, sems.at[0])
    cp_mem0 = pltpu.make_async_copy(mem0_hbm, mem0, sems.at[1])
    cp_woa = pltpu.make_async_copy(woa_hbm, wo_a, sems.at[2])
    big = (wqt_hbm, wkt_hbm, wvt_hbm, wo_hbm)

    def cp_wqkv(n):
        return pltpu.make_async_copy(wqkv_hbm.at[:, pl.ds(pl.multiple_of(D * n, 128), D)], wqkv.at[n],
                                     sems.at[4 + n])

    def cp_x(j):
        rows = pl.ds(pl.multiple_of(j * XCH, XCH), XCH)
        return pltpu.make_async_copy(x_hbm.at[rows, :], xin_ref.at[rows, :], sems.at[12 + j])

    def cp_w(n, j):
        rows = pl.ds(pl.multiple_of(j * TRC, TRC), TRC)
        return pltpu.make_async_copy(big[n].at[rows, :], stage_ref.at[n, rows, :], sems.at[20 + n * NTR + j])

    def cp_rows(sg, nseg):
        rows = pl.ds(pl.multiple_of(sg * SEG, SEG), SEG * nseg)
        return pltpu.make_async_copy(xin_ref.at[rows, :], out_hbm.at[rows, :], sems.at[3])

    cp_phi.start()
    for n in range(3):
        cp_wqkv(n).start()
    for j in range(S // XCH):
        cp_x(j).start()
    cp_mem0.start()
    for j in range(NTR):
        if j == NTR - 1:
            cp_woa.start()
        for n in range(3):
            cp_w(n, j).start()
    for j in range(NTR):
        cp_w(3, j).start()

    def init_x(c, carry):
        with jax.named_scope("wait_x"):
            cp_x(c).wait()
        x = xin_ref[pl.ds(pl.multiple_of(c * XCH, XCH), XCH), :].astype(f32)
        x_ref[pl.ds(pl.multiple_of(c * XCH, XCH), XCH), :] = x
        xna_ref[pl.ds(pl.multiple_of(c * (XCH // 2), XCH // 2), XCH // 2), :] = _pack(_ln(x))
        return carry

    with jax.named_scope("wait_phi"):
        cp_phi.wait()
    ecol = lax.broadcasted_iota(i32, (HA, D), 1) - DA * lax.broadcasted_iota(i32, (HA, D), 0)
    def scatter_phi(i, tp):
        for d in range(5):
            tp = tp + _dot(phi_ref[5 * i + d], jnp.where(ecol == 5 * i + d, 1.0, 0.0).astype(bf16))
        return tp

    tp = lax.fori_loop(0, DA // 5, scatter_phi, jnp.zeros((DA, D), f32))
    rep = jnp.where((lax.broadcasted_iota(i32, (RA, DA), 0) >> 1) == lax.broadcasted_iota(i32, (RA, DA), 1),
                    1.0, 0.0).astype(bf16)
    urep = _dot(rep, tp.astype(bf16))
    for g in range(GA):
        col = lax.broadcasted_iota(i32, (RA, 256), 1) + 128 * g
        par = lax.broadcasted_iota(i32, (RA, 256), 0) & 1
        for pp in range(4):
            lo = (8 * g + 2 * pp + par) * DA
            blk = jnp.where((col >= lo) & (col < lo + DA), urep[:, 128 * g:128 * g + 256], 0.0)
            lhs_ref[0, g, RA * pp:RA * pp + RA, :] = blk
        lhs_ref[1, g] = jnp.where(lax.broadcasted_iota(i32, (160, 256), 1) + 128 * g
                                  == lax.broadcasted_iota(i32, (160, 256), 0) + 160 * g, 1.0, 0.0)

    def prep(n, carry):
        with jax.named_scope("wait_wqkv"):
            cp_wqkv(n).wait()
        for g in range(GA):
            wat_ref[n, g] = _pack(_dot_nt(lhs_ref[n // 2, g].astype(bf16), wqkv[n, :, 128 * g:128 * g + 256]))
        return carry

    with jax.named_scope("prep"):
        lax.fori_loop(0, 3, prep, 0)
    with jax.named_scope("init_x"):
        lax.fori_loop(0, S // XCH, init_x, 0)
        cp_mem0.wait()

    def transpose_w(n, p):
        blocks = []
        for i in range(6):
            off = jnp.where(n == 2, VBLK[i], 64 * i)
            blocks.append(stage_ref[n, pl.ds(pl.multiple_of(p * PW + off, 64), 64), :])
        wb_ref[n, p] = pltpu.bitcast(jnp.concatenate(blocks, axis=0).T, u32)

    def pack_wo(j):
        for i in range(12):
            src = pl.ds(pl.multiple_of(j * TRC + (i // 6) * PW + VBLK[i % 6], 64), 64)
            wo_ref[pl.ds(pl.multiple_of(j * (TRC // 2) + 32 * i, 32), 32), :] = pltpu.bitcast(
                stage_ref[3, src, :], u32)

    def a_phase1(first):
        def body(c, carry):
            if first:
                ct = jnp.where(c == 0, NTR, c - 1)

                @pl.when(c > 0)
                def _():
                    with jax.named_scope("wait_w"):
                        for n in range(3):
                            cp_w(n, c - 1).wait()

            xn = _unpack(xna_ref[pl.ds(pl.multiple_of(c * (TC // 2), TC // 2), TC // 2), :])
            ones = jnp.ones((8, TC), f32)
            pend = []

            def flush(n):
                while len(pend) > n:
                    p, vext, phik = pend.pop(0)
                    kv_ref[p] += _dot_nt(vext, phik)

            for g in range(GA):
                pq = _dot_nt(_unpack(wat_ref[0, g]), xn)
                flush(KVLAG)
                pk = _dot_nt(_unpack(wat_ref[1, g]), xn)
                vt = _dot_nt(_unpack(wat_ref[2, g]), xn)
                for pp in range(4):
                    p = 4 * g + pp
                    sl = slice(RA * pp, RA * pp + RA)
                    phiq_ref[c, p] = pltpu.bitcast(_phi(pq[sl]), u32)
                    vext = jnp.concatenate([vt[sl], ones], axis=0).astype(bf16)
                    pend.append((p, vext, _phi(pk[sl])))
                if first and g < 3:
                    transpose_w(g, 2 * ct)
                    transpose_w(g, 2 * ct + 1)
            flush(0)
            return carry

        lax.fori_loop(0, NCH, body, 0, unroll=1 if first else P1U)

    def seg_rows(sg, off=0, n=SEG):
        return pl.ds(pl.multiple_of(sg * SEG + off, 8), n)

    def a_finish(sr, sw, n):
        cols = slice(128 * n, 128 * n + 128)
        y = _dot(_unpack(oa_ref[pl.ds(pl.multiple_of(sr * (SEG // 2), SEG // 2), SEG // 2), :]),
                 _unpack(wop_ref[:, cols]))
        x = x_ref[seg_rows(sr), cols] + y
        x_ref[seg_rows(sw), cols] = x
        xa_ref[:, cols] = x

    def a_norm(first, sg, slot, i, chain):
        x = x_ref[seg_rows(sg, 8 * i, 8), :] if first else xa_ref[8 * i:8 * i + 8, :]
        xnb_ref[slot, 8 * i:8 * i + 8, :] = _ln_chained(x, chain)

    def a_phase2(first):
        if first:
            cp_woa.wait()
        r = lax.broadcasted_iota(i32, (RA + 8, 2 * RA), 0)
        rb = jnp.where(((r >= DA) & (r < RA)) | (r >= RA + 4), 1, 0)
        same = rb == (lax.broadcasted_iota(i32, (RA + 8, 2 * RA), 1) & 1)
        for p in range(NPA):
            kvm_ref[p] = _pack(jnp.where(same, kv_ref[p], 0.0))

        def attend(c):
            top = lax.broadcasted_iota(i32, (8, TC), 0) < 4
            ot = []
            for p in range(NPA):
                ne = _dot(_unpack(kvm_ref[p]), _unpack(phiq_ref[c, p]))
                rc = 1.0 / (ne[RA:RA + 8] + 1e-6)
                sw = pltpu.roll(rc, 4, 0)
                ra, rb = jnp.where(top, rc, sw), jnp.where(top, sw, rc)
                ot.append(ne[0:RA] * jnp.concatenate([ra, ra, rc, rb, rb], axis=0))
            o = jnp.concatenate(ot, axis=0).T
            oa_ref[pl.ds(pl.multiple_of(c * (TC // 2), TC // 2), TC // 2), :] = _pack(o)

        if not first:
            for c in range(NCH):
                attend(c)
                if c == 2:
                    for n in range(D // 128):
                        a_finish(0, 0, n)
                    for i in range(4):
                        a_norm(False, 0, 0, i, [])
            return

        wop_ref[...] = pltpu.bitcast(wo_a[...], u32)
        attend(0)

        def body(c, carry):
            @pl.when(c == 2)
            def _():
                for n in range(3):
                    cp_w(n, NTR - 1).wait()

            @pl.when(c >= 2)
            def _():
                cp_w(3, c - 2).wait()

            lhs = [_unpack(oa_ref[pl.ds(pl.multiple_of(c * (TC // 2) + r // 2, 64), 64), :])
                   for r in range(0, TC, 128)]
            attend(jnp.minimum(c + 1, NCH - 1))
            t = jnp.maximum(c - 2, 0)
            transpose_w(t // 2, jnp.where(c < 2, NPB, NPB - 2 + t % 2))
            pack_wo(jnp.where(c < 2, NTR, t))
            for r in range(0, TC, 128):
                x_ref[pl.ds(pl.multiple_of(c * TC + r, 128), 128), :] += _dot(lhs[r // 128], _unpack(wop_ref[...]))
            return carry

        lax.fori_loop(0, NCH, body, 0)

    def b_finish(first, sr, sw, slot, i, chain):
        x = x_ref[seg_rows(sr, 16 * i, 16), :] + yb_ref[slot, 16 * i:16 * i + 16, :]
        if first:
            x_ref[seg_rows(sw, 16 * i, 16), :] = x
            xb_ref[16 * i:16 * i + 16, :] = x
            xn = [_ln_chained(xb_ref[16 * i + k:16 * i + k + 8, :], chain) for k in (0, 8)]
            xna_ref[pl.ds(pl.multiple_of(sr * (SEG // 2) + 8 * i, 8), 8), :] = _pack(
                jnp.concatenate(xn, axis=0))
        else:
            xin_ref[pl.ds(pl.multiple_of(sr * SEG + 16 * i, 16), 16), :] = x.astype(bf16)

    def b_step(h, side, chain):
        st = {}

        def proj(p, which):
            if p == 0 and which == 0:
                y = _dot(h[:, 0:128], _unpack(wb_ref[0, 0, 0:64, :]))
                for k in range(1, D // 128):
                    y = y + _dot(h[:, 128 * k:128 * k + 128], _unpack(wb_ref[0, 0, 64 * k:64 * k + 64, :]))
            else:
                y = _dot(h, _unpack(wb_ref[which, p]))
            if which == 0:
                st[(p, 'qv')] = y[0:8] * SCALE
                y = jnp.concatenate([y[SEG:L], y[8:SEG]], axis=0)
                st[(p, 0)] = (jnp.concatenate([y[:, 0:128], y[:, 256:384]], axis=0).astype(bf16), y[:, 128:256])
                return
            y = jnp.concatenate([y[SEG:L], y[0:SEG]], axis=0)
            st[(p, 'kv', which)] = y[0:16]
            if which == 1:
                st[(p, 1)] = _split(y)
            else:
                lo = (lax.broadcasted_iota(i32, (L, PW), 1) & 64) == 0
                st[(p, 2)] = jnp.concatenate([jnp.where(lo, y, 0.0), jnp.where(lo, 0.0, y)], axis=0).astype(bf16)

        def do_qk(p):
            zeros = chain[:1] + st.pop('tie', [])
            del chain[:1]
            st[(p, 'p')] = _probs(st.pop((p, 0)), st.pop((p, 1)), zeros)

        def do_pv(p):
            cols = slice(p * PW, (p + 1) * PW)
            o = _dot(st.pop((p, 'p')), st.pop((p, 2)))
            o_ref[0:MEM, cols] = o[0:MEM]
            o_ref[2 * MEM:L, cols] = o[MEM:LM]

        def do_vpu(p):
            cols = slice(p * PW, (p + 1) * PW)
            lo = lax.broadcasted_iota(i32, (8, 128), 1) < 64
            row = lax.broadcasted_iota(i32, (8, 128), 0)
            q = st.pop((p, 'qv'))
            qa, qb = jnp.where(lo, q[:, 128:256], 0.0), jnp.where(lo, 0.0, q[:, 128:256])

            kk, vv = st.pop((p, 'kv', 1)), st.pop((p, 'kv', 2))
            sc = []
            for k in range(16):
                km = jnp.broadcast_to(kk[k:k + 1, 128:256], (8, 128))
                xa = jnp.sum(q[:, 0:128] * kk[k:k + 1, 0:128] + qa * km, axis=-1, keepdims=True)
                xb = jnp.sum(q[:, 256:384] * kk[k:k + 1, 256:384] + qb * km, axis=-1, keepdims=True)
                x = jnp.where(lo, xa, xb)
                sc.append(jnp.where(row >= k - MEM, x, -1000000000.0) if k > MEM else x)
            m = functools.reduce(jnp.maximum, sc)
            ev = [jnp.exp2(x - m) for x in sc]
            rr = 1.0 / functools.reduce(jnp.add, ev)
            z = _zero(m)
            ov = []
            for t in range(3):
                v = [vv[8 * b:8 * b + 8, 128 * t:128 * t + 128] + z for b in range(2)]
                ov.append(functools.reduce(
                    jnp.add, [ev[k] * v[k // 8][k % 8:k % 8 + 1] for k in range(16)]) * rr)
                z = _zero(ov[-1])
            o_ref[MEM:2 * MEM, cols] = jnp.concatenate(ov, axis=1)
            st['tie'] = [z[:, 0:2 * L]]

        def do_o(n):
            k0 = st.get('k', 0)
            k1 = min(k0 + n, HD // 128)
            if k0 == k1:
                return
            st['k'] = k1
            y = _dot(o_ref[:, k0 * 128:k1 * 128], _unpack(wo_ref[k0 * 64:k1 * 64, :]))
            st['y'] = y if 'y' not in st else st['y'] + y

        o1, o2, o3, olag, f1, f2, f3 = SCH
        for s in range(NPB):
            on = s >= olag
            proj(s, 0)
            if on:
                do_o(o1)
            if s >= 1:
                do_qk(s - 1)
            if s >= VLAG and VPOS == 0:
                do_vpu(s - VLAG)
            proj(s, 1)
            if on:
                do_o(o2)
            if s >= 2:
                do_pv(s - 2)
            if s >= VLAG and VPOS == 1:
                do_vpu(s - VLAG)
            proj(s, 2)
            if on:
                do_o(o3)
            for job in side[s]:
                job()
            assert st.get('k', 0) <= 3 * max(s - 2, 0)
        do_o(f1)
        do_qk(NPB - 1)
        for p in range(NPB - VLAG, NPB):
            do_vpu(p)
        do_o(f2)
        do_pv(NPB - 2)
        do_o(f3)
        assert st.get('k', 0) <= 3 * (NPB - 2)
        do_pv(NPB - 1)
        do_o(3 * (NPB - 1) - st['k'])
        do_o(3)
        return st['y']

    def layer_b(first):
        SPI = SPI1 if first else SPI2
        mem_ref[...] = mem0[...].astype(f32)
        yb_ref[1] = jnp.zeros((SEG, D), f32)
        if first:
            for i in range(4):
                a_norm(first, 0, 0, i, [])
            with jax.named_scope("wait_wo"):
                for j in range(NTR - 2, NTR):
                    cp_w(3, j).wait()
                    pack_wo(j)

        def body(j, carry):
            mem = mem_ref[...]
            for t in range(SPI):
                sg = j * SPI + t
                if not first and t % 2 == 0:
                    if t >= 4:
                        cp_rows(sg - 3, 2).start()
                    else:
                        @pl.when(sg >= 4)
                        def _():
                            cp_rows(sg - 3, 2).start()
                sp = jnp.maximum(sg - 1, 0) if t == 0 else sg - 1
                sw = jnp.where(sg == 0, NSEG, sp) if t == 0 else sp
                sn = jnp.minimum(sg + 1, NSEG - 1) if t == SPI - 1 else sg + 1
                h = jnp.concatenate([xnb_ref[t % 2], mem], axis=0)
                chain = []
                side = [[] for _ in range(NPB)]
                for i in range(2):
                    side[1 + 2 * i].append(functools.partial(b_finish, first, sp, sw, (t + 1) % 2, i, chain))
                if not first:
                    for n in range(D // 128):
                        side[n].append(functools.partial(a_finish, sn, sg + 1, n))
                for i in range(4):
                    side[6 + 2 * i].append(functools.partial(a_norm, first, sn, (t + 1) % 2, i, chain))
                y = b_step(h, side, chain)
                mem = y[0:MEM]
                yb_ref[t % 2] = y[MEM:L]
            mem_ref[...] = mem
            return carry

        with jax.named_scope("b_loop"):
            lax.fori_loop(0, NSEG // SPI, body, 0)
        if not first:
            cp_rows(0, 1).start()
            cp_rows(NSEG - 3, 2).start()
        for i in range(2):
            b_finish(first, NSEG - 1, NSEG - 1, 1, i, [])

    for first in (True, False):
        kv_ref[...] = jnp.zeros(kv_ref.shape, f32)
        with jax.named_scope("a_p1"):
            a_phase1(first)
        with jax.named_scope("a_p2"):
            a_phase2(first)
        with jax.named_scope("layer_b"):
            layer_b(first)

    cp_rows(NSEG - 1, 1).start()
    cp_rows(0, NSEG).wait()


@jax.jit
def pallas_interleave_layers__linear_kernel_hedgehog__memory_aug_recurrent_mem_tr__prompt_kernel(
    A_x: jax.Array,
    A_wqkv: jax.Array,
    A_w_phi: jax.Array,
    A_wo: jax.Array,
    B_x: jax.Array,
    B_mem0: jax.Array,
    B_Wq: jax.Array,
    B_Wk: jax.Array,
    B_Wv: jax.Array,
    B_Wo: jax.Array,
    B_seg_len: jax.Array,
):
    del B_x, B_seg_len
    x = A_x.reshape(S, D)
    phi = A_w_phi.transpose(1, 2, 0)
    wqt = B_Wq.transpose(1, 2, 0).reshape(HD, D)
    wkt = B_Wk.transpose(1, 2, 0).reshape(HD, D)
    wvt = B_Wv.transpose(1, 2, 0).reshape(HD, D)
    wo = B_Wo.reshape(HD, D)
    hbm = pl.BlockSpec(memory_space=pl.ANY)
    out = pl.pallas_call(
        _kernel,
        out_shape=jax.ShapeDtypeStruct((S, D), bf16),
        in_specs=[hbm] * 9,
        out_specs=hbm,
        scratch_shapes=[
            pltpu.VMEM((S, D), bf16),
            pltpu.VMEM((3, D, D), bf16),
            pltpu.VMEM((DA, DA, HA), bf16),
            pltpu.VMEM((D, D), bf16),
            pltpu.VMEM((MEM, D), bf16),
            pltpu.VMEM((S + SEG, D), f32),
            pltpu.VMEM((S // 2, D), u32),
            pltpu.VMEM((2, SEG, D), f32),
            pltpu.VMEM((SEG, D), f32),
            pltpu.VMEM((SEG, D), f32),
            pltpu.VMEM((2, SEG, D), f32),
            pltpu.VMEM((S // 2, D), u32),
            pltpu.VMEM((3, GA, 80, D), u32),
            pltpu.VMEM((D // 2, D), u32),
            pltpu.VMEM((2, GA, 160, 256), f32),
            pltpu.VMEM((NCH, NPA, RA, TC), u32),
            pltpu.VMEM((NPA, RA + 8, 2 * RA), f32),
            pltpu.VMEM((NPA, (RA + 8) // 2, 2 * RA), u32),
            pltpu.VMEM((4, HD + TRC, D), bf16),
            pltpu.VMEM((3, NPB + 2, D // 2, PW), u32),
            pltpu.VMEM(((HD + TRC) // 2, D), u32),
            pltpu.VMEM((MEM, D), f32),
            pltpu.VMEM((L, HD), f32),
            pltpu.SemaphoreType.DMA((20 + 4 * NTR,)),
        ],
        compiler_params=pltpu.CompilerParams(vmem_limit_bytes=120 * 1024 * 1024),
    )(x, A_wqkv, phi, A_wo, B_mem0.reshape(MEM, D), wqt, wkt, wvt, wo)
    return out.reshape(1, S, D)
```

```python
import functools
import os

import jax
import jax.numpy as jnp
from jax import lax
import jax.experimental.pallas as pl
import jax.experimental.pallas.tpu as pltpu

f32, bf16, u32, i32 = jnp.float32, jnp.bfloat16, jnp.uint32, jnp.int32

S, D = 2048, 640
HA, DA = 32, 20
NPA = HA // 2
RA = 2 * DA
GA = 4
TC = 256
NCH = S // TC
XCH = int(os.environ.get("XCH", "256"))
HB, DB, MEM, SEG = 32, 192, 8, 32
HD = HB * DB
L = MEM + SEG
LM = L - 8
VBLK = (0, 192, 64, 256, 128, 320)
NPB = HB // 2
PW = 2 * DB
SCALE = DB ** -0.5 * 1.4426950408889634
TRC = 768
NTR = HD // TRC
NSEG = S // SEG
SPI1 = int(os.environ.get("SPI1", "2"))
SPI2 = int(os.environ.get("SPI2", "4"))
assert NTR == NCH

SCH = tuple(int(v) for v in os.environ.get("SCH", "1,0,1,4,2,4,7").split(","))
VLAG = int(os.environ.get("VLAG", "1"))
VPOS = int(os.environ.get("VPOS", "1"))
KVLAG = int(os.environ.get("KVLAG", "12"))
P1U = int(os.environ.get("P1U", "2"))

_NN = (((1,), (0,)), ((), ()))
_NT = (((1,), (1,)), ((), ()))


def _dot(a, b):
    return lax.dot_general(a, b, _NN, preferred_element_type=f32)


def _dot_nt(a, b):
    return lax.dot_general(a, b, _NT, preferred_element_type=f32)


def _pack(x):
    return pltpu.bitcast(x.astype(bf16), u32)


def _unpack(x):
    return pltpu.bitcast(x, bf16)


def _ln(x):
    m = jnp.mean(x, axis=-1, keepdims=True)
    xc = x - m
    r = lax.rsqrt(jnp.mean(xc * xc, axis=-1, keepdims=True) + 1e-5)
    return x * r - m * r


def _ln_chained(x, chain):
    m = jnp.mean(x, axis=-1, keepdims=True)
    xc = x - m
    r = lax.rsqrt(jnp.mean(xc * xc, axis=-1, keepdims=True) + 1e-5)
    chain.append(jnp.minimum(r, 0.0))
    return x * r - m * r


def _fold(op, p):
    r = p[0:8]
    for j in range(1, 5):
        r = op(r, p[8 * j:8 * j + 8])
    r = op(r, pltpu.roll(r, 2, 0))
    return op(r, pltpu.roll(r, 4, 0))


def _tile5(r):
    return jnp.concatenate([r] * 5, axis=0)


def _phi(p):
    ep = jnp.exp(p - _tile5(_fold(jnp.maximum, p)))
    en = jnp.exp(_tile5(_fold(jnp.minimum, p)) - p)
    ep = ep * _tile5(1.0 / _fold(jnp.add, ep))
    en = en * _tile5(1.0 / _fold(jnp.add, en))
    return jnp.concatenate([ep, en], axis=0).astype(bf16)


def _split(k):
    lo = lax.broadcasted_iota(i32, (L, 128), 1) < 64
    z = jnp.zeros((L, 128), f32)
    mid = k[:, 128:256]
    outer = jnp.concatenate([k[:, 0:128], k[:, 256:384]], axis=0).astype(bf16)
    mid = jnp.concatenate([jnp.where(lo, mid, z), jnp.where(lo, z, mid)], axis=0).astype(bf16)
    return outer, mid


def _zero(x):
    return jnp.minimum(jnp.abs(x), 0.0)


def _probs(q, k, zeros):
    r = lax.broadcasted_iota(i32, (LM, 2 * L), 0)
    c = lax.broadcasted_iota(i32, (LM, 2 * L), 1)
    first = c < L
    so = _dot_nt(q[0], k[0])
    s = jnp.where(first, so[0:LM], so[LM:2 * LM]) + _dot_nt(q[1], k[1])
    s = s * SCALE
    if zeros:
        s = jnp.concatenate([functools.reduce(jnp.add, zeros, s[0:8]), s[8:LM]], axis=0)
    mask = (r < MEM) | (r + 8 >= jnp.where(first, c, c - L))
    s = jnp.where(mask, s, -1000000000.0)
    neg = jnp.full_like(s, -jnp.inf)
    ma = jnp.max(jnp.where(first, s, neg), axis=-1, keepdims=True)
    mb = jnp.max(jnp.where(first, neg, s), axis=-1, keepdims=True)
    e = jnp.exp2(s - jnp.where(first, ma, mb))
    z = jnp.zeros_like(e)
    sa = jnp.sum(jnp.where(first, e, z), axis=-1, keepdims=True)
    sb = jnp.sum(jnp.where(first, z, e), axis=-1, keepdims=True)
    return e * (1.0 / jnp.where(first, sa, sb))


def _kernel(x_hbm, wqkv_hbm, phi_hbm, woa_hbm, mem0_hbm, wqt_hbm, wkt_hbm, wvt_hbm, wo_hbm, out_hbm,
            xin_ref, wqkv, phi_ref, wo_a, mem0, x_ref, xna_ref, xnb_ref, xa_ref, xb_ref, yb_ref, oa_ref,
            wat_ref, wop_ref, lhs_ref, phiq_ref, kv_ref, kvm_ref, stage_ref, wb_ref, wo_ref, mem_ref, o_ref,
            sems):
    cp_phi = pltpu.make_async_copy(phi_hbm, phi_ref, sems.at[0])
    cp_mem0 = pltpu.make_async_copy(mem0_hbm, mem0, sems.at[1])
    cp_woa = pltpu.make_async_copy(woa_hbm, wo_a, sems.at[2])
    big = (wqt_hbm, wkt_hbm, wvt_hbm, wo_hbm)

    def cp_wqkv(n):
        return pltpu.make_async_copy(wqkv_hbm.at[:, pl.ds(pl.multiple_of(D * n, 128), D)], wqkv.at[n],
                                     sems.at[4 + n])

    def cp_x(j):
        rows = pl.ds(pl.multiple_of(j * XCH, XCH), XCH)
        return pltpu.make_async_copy(x_hbm.at[rows, :], xin_ref.at[rows, :], sems.at[12 + j])

    def cp_w(n, j):
        rows = pl.ds(pl.multiple_of(j * TRC, TRC), TRC)
        return pltpu.make_async_copy(big[n].at[rows, :], stage_ref.at[n, rows, :], sems.at[20 + n * NTR + j])

    def cp_rows(sg, nseg):
        rows = pl.ds(pl.multiple_of(sg * SEG, SEG), SEG * nseg)
        return pltpu.make_async_copy(xin_ref.at[rows, :], out_hbm.at[rows, :], sems.at[3])

    cp_phi.start()
    for n in range(3):
        cp_wqkv(n).start()
    for j in range(S // XCH):
        cp_x(j).start()
    cp_mem0.start()
    for j in range(NTR):
        if j == NTR - 1:
            cp_woa.start()
        for n in range(3):
            cp_w(n, j).start()
    for j in range(NTR):
        cp_w(3, j).start()

    def init_x(c, carry):
        with jax.named_scope("wait_x"):
            cp_x(c).wait()
        x = xin_ref[pl.ds(pl.multiple_of(c * XCH, XCH), XCH), :].astype(f32)
        x_ref[pl.ds(pl.multiple_of(c * XCH, XCH), XCH), :] = x
        xna_ref[pl.ds(pl.multiple_of(c * (XCH // 2), XCH // 2), XCH // 2), :] = _pack(_ln(x))
        return carry

    with jax.named_scope("wait_phi"):
        cp_phi.wait()
    ecol = lax.broadcasted_iota(i32, (HA, D), 1) - DA * lax.broadcasted_iota(i32, (HA, D), 0)
    def scatter_phi(i, tp):
        for d in range(5):
            tp = tp + _dot(phi_ref[5 * i + d], jnp.where(ecol == 5 * i + d, 1.0, 0.0).astype(bf16))
        return tp

    tp = lax.fori_loop(0, DA // 5, scatter_phi, jnp.zeros((DA, D), f32))
    rep = jnp.where((lax.broadcasted_iota(i32, (RA, DA), 0) >> 1) == lax.broadcasted_iota(i32, (RA, DA), 1),
                    1.0, 0.0).astype(bf16)
    urep = _dot(rep, tp.astype(bf16))
    for g in range(GA):
        col = lax.broadcasted_iota(i32, (RA, 256), 1) + 128 * g
        par = lax.broadcasted_iota(i32, (RA, 256), 0) & 1
        for pp in range(4):
            lo = (8 * g + 2 * pp + par) * DA
            blk = jnp.where((col >= lo) & (col < lo + DA), urep[:, 128 * g:128 * g + 256], 0.0)
            lhs_ref[0, g, RA * pp:RA * pp + RA, :] = blk
        lhs_ref[1, g] = jnp.where(lax.broadcasted_iota(i32, (160, 256), 1) + 128 * g
                                  == lax.broadcasted_iota(i32, (160, 256), 0) + 160 * g, 1.0, 0.0)

    def prep(n, carry):
        with jax.named_scope("wait_wqkv"):
            cp_wqkv(n).wait()
        for g in range(GA):
            wat_ref[n, g] = _pack(_dot_nt(lhs_ref[n // 2, g].astype(bf16), wqkv[n, :, 128 * g:128 * g + 256]))
        return carry

    with jax.named_scope("prep"):
        lax.fori_loop(0, 3, prep, 0)
    with jax.named_scope("init_x"):
        lax.fori_loop(0, S // XCH, init_x, 0)
        cp_mem0.wait()

    def transpose_w(n, p):
        blocks = []
        for i in range(6):
            off = jnp.where(n == 2, VBLK[i], 64 * i)
            blocks.append(stage_ref[n, pl.ds(pl.multiple_of(p * PW + off, 64), 64), :])
        wb_ref[n, p] = pltpu.bitcast(jnp.concatenate(blocks, axis=0).T, u32)

    def pack_wo(j):
        for i in range(12):
            src = pl.ds(pl.multiple_of(j * TRC + (i // 6) * PW + VBLK[i % 6], 64), 64)
            wo_ref[pl.ds(pl.multiple_of(j * (TRC // 2) + 32 * i, 32), 32), :] = pltpu.bitcast(
                stage_ref[3, src, :], u32)

    def a_phase1(first):
        def body(c, carry):
            if first:
                ct = [jnp.where(c < lag, NTR, c - lag) for lag in (1, 1, 2)]

                @pl.when(c >= 2)
                def _():
                    cp_w(2, c - 2).wait()

                @pl.when(c >= 1)
                def _():
                    with jax.named_scope("wait_w"):
                        cp_w(0, c - 1).wait()
                        cp_w(1, c - 1).wait()

            xn = _unpack(xna_ref[pl.ds(pl.multiple_of(c * (TC // 2), TC // 2), TC // 2), :])
            ones = jnp.ones((8, TC), f32)
            pend = []

            def flush(n):
                while len(pend) > n:
                    p, vext, phik = pend.pop(0)
                    kv_ref[p] += _dot_nt(vext, phik)

            for g in range(GA):
                pq = _dot_nt(_unpack(wat_ref[0, g]), xn)
                flush(KVLAG)
                pk = _dot_nt(_unpack(wat_ref[1, g]), xn)
                vt = _dot_nt(_unpack(wat_ref[2, g]), xn)
                for pp in range(4):
                    p = 4 * g + pp
                    sl = slice(RA * pp, RA * pp + RA)
                    phiq_ref[c, p] = pltpu.bitcast(_phi(pq[sl]), u32)
                    vext = jnp.concatenate([vt[sl], ones], axis=0).astype(bf16)
                    pend.append((p, vext, _phi(pk[sl])))
                if first and g < 3:
                    transpose_w(g, 2 * ct[g])
                    transpose_w(g, 2 * ct[g] + 1)
            flush(0)
            return carry

        lax.fori_loop(0, NCH, body, 0, unroll=1 if first else P1U)

    def seg_rows(sg, off=0, n=SEG):
        return pl.ds(pl.multiple_of(sg * SEG + off, 8), n)

    def a_finish(sr, sw, n):
        cols = slice(128 * n, 128 * n + 128)
        y = _dot(_unpack(oa_ref[pl.ds(pl.multiple_of(sr * (SEG // 2), SEG // 2), SEG // 2), :]),
                 _unpack(wop_ref[:, cols]))
        x = x_ref[seg_rows(sr), cols] + y
        x_ref[seg_rows(sw), cols] = x
        xa_ref[:, cols] = x

    def a_norm(first, sg, slot, i, chain):
        x = x_ref[seg_rows(sg, 8 * i, 8), :] if first else xa_ref[8 * i:8 * i + 8, :]
        xnb_ref[slot, 8 * i:8 * i + 8, :] = _ln_chained(x, chain)

    def a_phase2(first):
        if first:
            cp_w(2, NTR - 2).wait()
            cp_woa.wait()
        r = lax.broadcasted_iota(i32, (RA + 8, 2 * RA), 0)
        rb = jnp.where(((r >= DA) & (r < RA)) | (r >= RA + 4), 1, 0)
        same = rb == (lax.broadcasted_iota(i32, (RA + 8, 2 * RA), 1) & 1)
        for p in range(NPA):
            kvm_ref[p] = _pack(jnp.where(same, kv_ref[p], 0.0))

        def attend(c):
            top = lax.broadcasted_iota(i32, (8, TC), 0) < 4
            ot = []
            for p in range(NPA):
                ne = _dot(_unpack(kvm_ref[p]), _unpack(phiq_ref[c, p]))
                rc = 1.0 / (ne[RA:RA + 8] + 1e-6)
                sw = pltpu.roll(rc, 4, 0)
                ra, rb = jnp.where(top, rc, sw), jnp.where(top, sw, rc)
                ot.append(ne[0:RA] * jnp.concatenate([ra, ra, rc, rb, rb], axis=0))
            o = jnp.concatenate(ot, axis=0).T
            oa_ref[pl.ds(pl.multiple_of(c * (TC // 2), TC // 2), TC // 2), :] = _pack(o)

        if not first:
            for c in range(NCH):
                attend(c)
                if c == 2:
                    for n in range(D // 128):
                        a_finish(0, 0, n)
                    for i in range(4):
                        a_norm(False, 0, 0, i, [])
            return

        wop_ref[...] = pltpu.bitcast(wo_a[...], u32)
        attend(0)

        def body(c, carry):
            @pl.when(c == 2)
            def _():
                for n in range(3):
                    cp_w(n, NTR - 1).wait()

            @pl.when(c >= 2)
            def _():
                cp_w(3, c - 2).wait()

            lhs = [_unpack(oa_ref[pl.ds(pl.multiple_of(c * (TC // 2) + r // 2, 64), 64), :])
                   for r in range(0, TC, 128)]
            attend(jnp.minimum(c + 1, NCH - 1))
            t = jnp.maximum(c - 2, 0)
            transpose_w(jnp.where(c < 2, 2, t // 2), jnp.where(c < 2, NPB - 4, NPB - 2) + c % 2)
            pack_wo(jnp.where(c < 2, NTR, t))
            for r in range(0, TC, 128):
                x_ref[pl.ds(pl.multiple_of(c * TC + r, 128), 128), :] += _dot(lhs[r // 128], _unpack(wop_ref[...]))
            return carry

        lax.fori_loop(0, NCH, body, 0)

    def b_finish(first, sr, sw, slot, i, chain):
        x = x_ref[seg_rows(sr, 16 * i, 16), :] + yb_ref[slot, 16 * i:16 * i + 16, :]
        if first:
            x_ref[seg_rows(sw, 16 * i, 16), :] = x
            xb_ref[16 * i:16 * i + 16, :] = x
            xn = [_ln_chained(xb_ref[16 * i + k:16 * i + k + 8, :], chain) for k in (0, 8)]
            xna_ref[pl.ds(pl.multiple_of(sr * (SEG // 2) + 8 * i, 8), 8), :] = _pack(
                jnp.concatenate(xn, axis=0))
        else:
            xin_ref[pl.ds(pl.multiple_of(sr * SEG + 16 * i, 16), 16), :] = x.astype(bf16)

    def b_step(h, side, chain):
        st = {}

        def proj(p, which):
            if p == 0 and which == 0:
                y = _dot(h[:, 0:128], _unpack(wb_ref[0, 0, 0:64, :]))
                for k in range(1, D // 128):
                    y = y + _dot(h[:, 128 * k:128 * k + 128], _unpack(wb_ref[0, 0, 64 * k:64 * k + 64, :]))
            else:
                y = _dot(h, _unpack(wb_ref[which, p]))
            if which == 0:
                st[(p, 'qv')] = y[0:8] * SCALE
                y = jnp.concatenate([y[SEG:L], y[8:SEG]], axis=0)
                st[(p, 0)] = (jnp.concatenate([y[:, 0:128], y[:, 256:384]], axis=0).astype(bf16), y[:, 128:256])
                return
            y = jnp.concatenate([y[SEG:L], y[0:SEG]], axis=0)
            st[(p, 'kv', which)] = y[0:16]
            if which == 1:
                st[(p, 1)] = _split(y)
            else:
                lo = (lax.broadcasted_iota(i32, (L, PW), 1) & 64) == 0
                st[(p, 2)] = jnp.concatenate([jnp.where(lo, y, 0.0), jnp.where(lo, 0.0, y)], axis=0).astype(bf16)

        def do_qk(p):
            zeros = chain[:1] + st.pop('tie', [])
            del chain[:1]
            st[(p, 'p')] = _probs(st.pop((p, 0)), st.pop((p, 1)), zeros)

        def do_pv(p):
            cols = slice(p * PW, (p + 1) * PW)
            o = _dot(st.pop((p, 'p')), st.pop((p, 2)))
            o_ref[0:MEM, cols] = o[0:MEM]
            o_ref[2 * MEM:L, cols] = o[MEM:LM]

        def do_vpu(p):
            cols = slice(p * PW, (p + 1) * PW)
            lo = lax.broadcasted_iota(i32, (8, 128), 1) < 64
            row = lax.broadcasted_iota(i32, (8, 128), 0)
            q = st.pop((p, 'qv'))
            qa, qb = jnp.where(lo, q[:, 128:256], 0.0), jnp.where(lo, 0.0, q[:, 128:256])

            kk, vv = st.pop((p, 'kv', 1)), st.pop((p, 'kv', 2))
            sc = []
            for k in range(16):
                km = jnp.broadcast_to(kk[k:k + 1, 128:256], (8, 128))
                xa = jnp.sum(q[:, 0:128] * kk[k:k + 1, 0:128] + qa * km, axis=-1, keepdims=True)
                xb = jnp.sum(q[:, 256:384] * kk[k:k + 1, 256:384] + qb * km, axis=-1, keepdims=True)
                x = jnp.where(lo, xa, xb)
                sc.append(jnp.where(row >= k - MEM, x, -1000000000.0) if k > MEM else x)
            m = functools.reduce(jnp.maximum, sc)
            ev = [jnp.exp2(x - m) for x in sc]
            rr = 1.0 / functools.reduce(jnp.add, ev)
            z = _zero(m)
            ov = []
            for t in range(3):
                v = [vv[8 * b:8 * b + 8, 128 * t:128 * t + 128] + z for b in range(2)]
                ov.append(functools.reduce(
                    jnp.add, [ev[k] * v[k // 8][k % 8:k % 8 + 1] for k in range(16)]) * rr)
                z = _zero(ov[-1])
            o_ref[MEM:2 * MEM, cols] = jnp.concatenate(ov, axis=1)
            st['tie'] = [z[:, 0:2 * L]]

        def do_o(n):
            k0 = st.get('k', 0)
            k1 = min(k0 + n, HD // 128)
            if k0 == k1:
                return
            st['k'] = k1
            y = _dot(o_ref[:, k0 * 128:k1 * 128], _unpack(wo_ref[k0 * 64:k1 * 64, :]))
            st['y'] = y if 'y' not in st else st['y'] + y

        o1, o2, o3, olag, f1, f2, f3 = SCH
        for s in range(NPB):
            on = s >= olag
            proj(s, 0)
            if on:
                do_o(o1)
            if s >= 1:
                do_qk(s - 1)
            if s >= VLAG and VPOS == 0:
                do_vpu(s - VLAG)
            proj(s, 1)
            if on:
                do_o(o2)
            if s >= 2:
                do_pv(s - 2)
            if s >= VLAG and VPOS == 1:
                do_vpu(s - VLAG)
            proj(s, 2)
            if on:
                do_o(o3)
            for job in side[s]:
                job()
            assert st.get('k', 0) <= 3 * max(s - 2, 0)
        do_o(f1)
        do_qk(NPB - 1)
        for p in range(NPB - VLAG, NPB):
            do_vpu(p)
        do_o(f2)
        do_pv(NPB - 2)
        do_o(f3)
        assert st.get('k', 0) <= 3 * (NPB - 2)
        do_pv(NPB - 1)
        do_o(3 * (NPB - 1) - st['k'])
        do_o(3)
        return st['y']

    def layer_b(first):
        SPI = SPI1 if first else SPI2
        mem_ref[...] = mem0[...].astype(f32)
        yb_ref[1] = jnp.zeros((SEG, D), f32)
        if first:
            for i in range(4):
                a_norm(first, 0, 0, i, [])
            with jax.named_scope("wait_wo"):
                for j in range(NTR - 2, NTR):
                    cp_w(3, j).wait()
                    pack_wo(j)

        def body(j, carry):
            mem = mem_ref[...]
            for t in range(SPI):
                sg = j * SPI + t
                if not first and t % 2 == 0:
                    if t >= 4:
                        cp_rows(sg - 3, 2).start()
                    else:
                        @pl.when(sg >= 4)
                        def _():
                            cp_rows(sg - 3, 2).start()
                sp = jnp.maximum(sg - 1, 0) if t == 0 else sg - 1
                sw = jnp.where(sg == 0, NSEG, sp) if t == 0 else sp
                sn = jnp.minimum(sg + 1, NSEG - 1) if t == SPI - 1 else sg + 1
                h = jnp.concatenate([xnb_ref[t % 2], mem], axis=0)
                chain = []
                side = [[] for _ in range(NPB)]
                for i in range(2):
                    side[1 + 2 * i].append(functools.partial(b_finish, first, sp, sw, (t + 1) % 2, i, chain))
                if not first:
                    for n in range(D // 128):
                        side[n].append(functools.partial(a_finish, sn, sg + 1, n))
                for i in range(4):
                    side[6 + 2 * i].append(functools.partial(a_norm, first, sn, (t + 1) % 2, i, chain))
                y = b_step(h, side, chain)
                mem = y[0:MEM]
                yb_ref[t % 2] = y[MEM:L]
            mem_ref[...] = mem
            return carry

        with jax.named_scope("b_loop"):
            lax.fori_loop(0, NSEG // SPI, body, 0)
        if not first:
            cp_rows(0, 1).start()
            cp_rows(NSEG - 3, 2).start()
        for i in range(2):
            b_finish(first, NSEG - 1, NSEG - 1, 1, i, [])

    for first in (True, False):
        kv_ref[...] = jnp.zeros(kv_ref.shape, f32)
        with jax.named_scope("a_p1"):
            a_phase1(first)
        with jax.named_scope("a_p2"):
            a_phase2(first)
        with jax.named_scope("layer_b"):
            layer_b(first)

    cp_rows(NSEG - 1, 1).start()
    cp_rows(0, NSEG).wait()


@jax.jit
def pallas_interleave_layers__linear_kernel_hedgehog__memory_aug_recurrent_mem_tr__prompt_kernel(
    A_x: jax.Array,
    A_wqkv: jax.Array,
    A_w_phi: jax.Array,
    A_wo: jax.Array,
    B_x: jax.Array,
    B_mem0: jax.Array,
    B_Wq: jax.Array,
    B_Wk: jax.Array,
    B_Wv: jax.Array,
    B_Wo: jax.Array,
    B_seg_len: jax.Array,
):
    del B_x, B_seg_len
    x = A_x.reshape(S, D)
    phi = A_w_phi.transpose(1, 2, 0)
    wqt = B_Wq.transpose(1, 2, 0).reshape(HD, D)
    wkt = B_Wk.transpose(1, 2, 0).reshape(HD, D)
    wvt = B_Wv.transpose(1, 2, 0).reshape(HD, D)
    wo = B_Wo.reshape(HD, D)
    hbm = pl.BlockSpec(memory_space=pl.ANY)
    out = pl.pallas_call(
        _kernel,
        out_shape=jax.ShapeDtypeStruct((S, D), bf16),
        in_specs=[hbm] * 9,
        out_specs=hbm,
        scratch_shapes=[
            pltpu.VMEM((S, D), bf16),
            pltpu.VMEM((3, D, D), bf16),
            pltpu.VMEM((DA, DA, HA), bf16),
            pltpu.VMEM((D, D), bf16),
            pltpu.VMEM((MEM, D), bf16),
            pltpu.VMEM((S + SEG, D), f32),
            pltpu.VMEM((S // 2, D), u32),
            pltpu.VMEM((2, SEG, D), f32),
            pltpu.VMEM((SEG, D), f32),
            pltpu.VMEM((SEG, D), f32),
            pltpu.VMEM((2, SEG, D), f32),
            pltpu.VMEM((S // 2, D), u32),
            pltpu.VMEM((3, GA, 80, D), u32),
            pltpu.VMEM((D // 2, D), u32),
            pltpu.VMEM((2, GA, 160, 256), f32),
            pltpu.VMEM((NCH, NPA, RA, TC), u32),
            pltpu.VMEM((NPA, RA + 8, 2 * RA), f32),
            pltpu.VMEM((NPA, (RA + 8) // 2, 2 * RA), u32),
            pltpu.VMEM((4, HD + TRC, D), bf16),
            pltpu.VMEM((3, NPB + 2, D // 2, PW), u32),
            pltpu.VMEM(((HD + TRC) // 2, D), u32),
            pltpu.VMEM((MEM, D), f32),
            pltpu.VMEM((L, HD), f32),
            pltpu.SemaphoreType.DMA((20 + 4 * NTR,)),
        ],
        compiler_params=pltpu.CompilerParams(vmem_limit_bytes=120 * 1024 * 1024),
    )(x, A_wqkv, phi, A_wo, B_mem0.reshape(MEM, D), wqt, wkt, wvt, wo)
    return out.reshape(1, S, D)
```

```python
import functools

import jax
import jax.numpy as jnp
from jax import lax
import jax.experimental.pallas as pl
import jax.experimental.pallas.tpu as pltpu

f32, bf16, u32, i32 = jnp.float32, jnp.bfloat16, jnp.uint32, jnp.int32

S, D = 2048, 640
HA, DA = 32, 20
NPA = HA // 2
RA = 2 * DA
GA = 4
TC = 256
NCH = S // TC
XCH = 256
HB, DB, MEM, SEG = 32, 192, 8, 32
HD = HB * DB
L = MEM + SEG
LM = L - 8
VBLK = (0, 192, 64, 256, 128, 320)
NPB = HB // 2
PW = 2 * DB
SCALE = DB ** -0.5 * 1.4426950408889634
TRC = 768
NTR = HD // TRC
NSEG = S // SEG
SPI1, SPI2 = 2, 4
assert NTR == NCH

_NN = (((1,), (0,)), ((), ()))
_NT = (((1,), (1,)), ((), ()))


def _dot(a, b):
    return lax.dot_general(a, b, _NN, preferred_element_type=f32)


def _dot_nt(a, b):
    return lax.dot_general(a, b, _NT, preferred_element_type=f32)


def _pack(x):
    return pltpu.bitcast(x.astype(bf16), u32)


def _unpack(x):
    return pltpu.bitcast(x, bf16)


def _ln(x):
    m = jnp.mean(x, axis=-1, keepdims=True)
    xc = x - m
    r = lax.rsqrt(jnp.mean(xc * xc, axis=-1, keepdims=True) + 1e-5)
    return x * r - m * r


def _ln_chained(x, chain):
    m = jnp.mean(x, axis=-1, keepdims=True)
    xc = x - m
    r = lax.rsqrt(jnp.mean(xc * xc, axis=-1, keepdims=True) + 1e-5)
    chain.append(jnp.minimum(r, 0.0))
    return x * r - m * r


def _fold(op, p):
    r = p[0:8]
    for j in range(1, 5):
        r = op(r, p[8 * j:8 * j + 8])
    r = op(r, pltpu.roll(r, 2, 0))
    return op(r, pltpu.roll(r, 4, 0))


def _tile5(r):
    return jnp.concatenate([r] * 5, axis=0)


def _phi(p):
    ep = jnp.exp(p - _tile5(_fold(jnp.maximum, p)))
    en = jnp.exp(_tile5(_fold(jnp.minimum, p)) - p)
    ep = ep * _tile5(1.0 / _fold(jnp.add, ep))
    en = en * _tile5(1.0 / _fold(jnp.add, en))
    return jnp.concatenate([ep, en], axis=0).astype(bf16)


def _split(k):
    lo = lax.broadcasted_iota(i32, (L, 128), 1) < 64
    z = jnp.zeros((L, 128), f32)
    mid = k[:, 128:256]
    outer = jnp.concatenate([k[:, 0:128], k[:, 256:384]], axis=0).astype(bf16)
    mid = jnp.concatenate([jnp.where(lo, mid, z), jnp.where(lo, z, mid)], axis=0).astype(bf16)
    return outer, mid


def _zero(x):
    return jnp.minimum(jnp.abs(x), 0.0)


def _probs(q, k, zeros):
    r = lax.broadcasted_iota(i32, (LM, 2 * L), 0)
    c = lax.broadcasted_iota(i32, (LM, 2 * L), 1)
    first = c < L
    so = _dot_nt(q[0], k[0])
    s = jnp.where(first, so[0:LM], so[LM:2 * LM]) + _dot_nt(q[1], k[1])
    s = s * SCALE
    if zeros:
        s = jnp.concatenate([functools.reduce(jnp.add, zeros, s[0:8]), s[8:LM]], axis=0)
    mask = (r < MEM) | (r + 8 >= jnp.where(first, c, c - L))
    s = jnp.where(mask, s, -1000000000.0)
    neg = jnp.full_like(s, -jnp.inf)
    ma = jnp.max(jnp.where(first, s, neg), axis=-1, keepdims=True)
    mb = jnp.max(jnp.where(first, neg, s), axis=-1, keepdims=True)
    e = jnp.exp2(s - jnp.where(first, ma, mb))
    z = jnp.zeros_like(e)
    sa = jnp.sum(jnp.where(first, e, z), axis=-1, keepdims=True)
    sb = jnp.sum(jnp.where(first, z, e), axis=-1, keepdims=True)
    return e * (1.0 / jnp.where(first, sa, sb))


def _kernel(x_hbm, wqkv_hbm, phi_hbm, woa_hbm, mem0_hbm, wqt_hbm, wkt_hbm, wvt_hbm, wo_hbm, out_hbm,
            xin_ref, wqkv, phi_ref, wo_a, mem0, x_ref, xna_ref, xnb_ref, xa_ref, xb_ref, yb_ref, oa_ref,
            wat_ref, wop_ref, lhs_ref, phiq_ref, kv_ref, kvm_ref, stage_ref, wb_ref, wo_ref, mem_ref, o_ref,
            sems):
    cp_phi = pltpu.make_async_copy(phi_hbm, phi_ref, sems.at[0])
    cp_mem0 = pltpu.make_async_copy(mem0_hbm, mem0, sems.at[1])
    cp_woa = pltpu.make_async_copy(woa_hbm, wo_a, sems.at[2])
    big = (wqt_hbm, wkt_hbm, wvt_hbm, wo_hbm)

    def cp_wqkv(n):
        return pltpu.make_async_copy(wqkv_hbm.at[:, pl.ds(pl.multiple_of(D * n, 128), D)], wqkv.at[n],
                                     sems.at[4 + n])

    def cp_x(j):
        rows = pl.ds(pl.multiple_of(j * XCH, XCH), XCH)
        return pltpu.make_async_copy(x_hbm.at[rows, :], xin_ref.at[rows, :], sems.at[12 + j])

    def cp_w(n, j):
        rows = pl.ds(pl.multiple_of(j * TRC, TRC), TRC)
        return pltpu.make_async_copy(big[n].at[rows, :], stage_ref.at[n, rows, :], sems.at[20 + n * NTR + j])

    def cp_rows(sg, nseg):
        rows = pl.ds(pl.multiple_of(sg * SEG, SEG), SEG * nseg)
        return pltpu.make_async_copy(xin_ref.at[rows, :], out_hbm.at[rows, :], sems.at[3])

    cp_phi.start()
    for n in range(3):
        cp_wqkv(n).start()
    for j in range(S // XCH):
        cp_x(j).start()
    cp_mem0.start()
    for j in range(NTR):
        if j == NTR - 1:
            cp_woa.start()
        for n in range(3):
            cp_w(n, j).start()
    for j in range(NTR):
        cp_w(3, j).start()

    def init_x(c, carry):
        with jax.named_scope("wait_x"):
            cp_x(c).wait()
        x = xin_ref[pl.ds(pl.multiple_of(c * XCH, XCH), XCH), :].astype(f32)
        x_ref[pl.ds(pl.multiple_of(c * XCH, XCH), XCH), :] = x
        xna_ref[pl.ds(pl.multiple_of(c * (XCH // 2), XCH // 2), XCH // 2), :] = _pack(_ln(x))
        return carry

    with jax.named_scope("wait_phi"):
        cp_phi.wait()
    ecol = lax.broadcasted_iota(i32, (HA, D), 1) - DA * lax.broadcasted_iota(i32, (HA, D), 0)

    def scatter_phi(i, tp):
        for d in range(5):
            tp = tp + _dot(phi_ref[5 * i + d], jnp.where(ecol == 5 * i + d, 1.0, 0.0).astype(bf16))
        return tp

    tp = lax.fori_loop(0, DA // 5, scatter_phi, jnp.zeros((DA, D), f32))
    rep = jnp.where((lax.broadcasted_iota(i32, (RA, DA), 0) >> 1) == lax.broadcasted_iota(i32, (RA, DA), 1),
                    1.0, 0.0).astype(bf16)
    urep = _dot(rep, tp.astype(bf16))
    for g in range(GA):
        col = lax.broadcasted_iota(i32, (RA, 256), 1) + 128 * g
        par = lax.broadcasted_iota(i32, (RA, 256), 0) & 1
        for pp in range(4):
            lo = (8 * g + 2 * pp + par) * DA
            blk = jnp.where((col >= lo) & (col < lo + DA), urep[:, 128 * g:128 * g + 256], 0.0)
            lhs_ref[0, g, RA * pp:RA * pp + RA, :] = blk
        lhs_ref[1, g] = jnp.where(lax.broadcasted_iota(i32, (160, 256), 1) + 128 * g
                                  == lax.broadcasted_iota(i32, (160, 256), 0) + 160 * g, 1.0, 0.0)

    def prep(n, carry):
        with jax.named_scope("wait_wqkv"):
            cp_wqkv(n).wait()
        for g in range(GA):
            wat_ref[n, g] = _pack(_dot_nt(lhs_ref[n // 2, g].astype(bf16), wqkv[n, :, 128 * g:128 * g + 256]))
        return carry

    with jax.named_scope("prep"):
        lax.fori_loop(0, 3, prep, 0)
    with jax.named_scope("init_x"):
        lax.fori_loop(0, S // XCH, init_x, 0)
        cp_mem0.wait()

    def transpose_w(n, p):
        blocks = []
        for i in range(6):
            off = jnp.where(n == 2, VBLK[i], 64 * i)
            blocks.append(stage_ref[n, pl.ds(pl.multiple_of(p * PW + off, 64), 64), :])
        wb_ref[n, p] = pltpu.bitcast(jnp.concatenate(blocks, axis=0).T, u32)

    def pack_wo(j):
        for i in range(12):
            src = pl.ds(pl.multiple_of(j * TRC + (i // 6) * PW + VBLK[i % 6], 64), 64)
            wo_ref[pl.ds(pl.multiple_of(j * (TRC // 2) + 32 * i, 32), 32), :] = pltpu.bitcast(
                stage_ref[3, src, :], u32)

    def a_phase1(first):
        def body(c, carry):
            if first:
                ct = [jnp.where(c < lag, NTR, c - lag) for lag in (1, 1, 2)]

                @pl.when(c >= 2)
                def _():
                    cp_w(2, c - 2).wait()

                @pl.when(c >= 1)
                def _():
                    with jax.named_scope("wait_w"):
                        cp_w(0, c - 1).wait()
                        cp_w(1, c - 1).wait()

            xn = _unpack(xna_ref[pl.ds(pl.multiple_of(c * (TC // 2), TC // 2), TC // 2), :])
            ones = jnp.ones((8, TC), f32)
            pend = []
            for g in range(GA):
                pq = _dot_nt(_unpack(wat_ref[0, g]), xn)
                pk = _dot_nt(_unpack(wat_ref[1, g]), xn)
                vt = _dot_nt(_unpack(wat_ref[2, g]), xn)
                for pp in range(4):
                    p = 4 * g + pp
                    sl = slice(RA * pp, RA * pp + RA)
                    phiq_ref[c, p] = pltpu.bitcast(_phi(pq[sl]), u32)
                    vext = jnp.concatenate([vt[sl], ones], axis=0).astype(bf16)
                    pend.append((p, vext, _phi(pk[sl])))
                if first and g < 3:
                    transpose_w(g, 2 * ct[g])
                    transpose_w(g, 2 * ct[g] + 1)
            for p, vext, phik in pend:
                kv_ref[p] += _dot_nt(vext, phik)
            return carry

        lax.fori_loop(0, NCH, body, 0, unroll=1 if first else 2)

    def seg_rows(sg, off=0, n=SEG):
        return pl.ds(pl.multiple_of(sg * SEG + off, 8), n)

    def a_finish(sr, sw, n):
        cols = slice(128 * n, 128 * n + 128)
        y = _dot(_unpack(oa_ref[pl.ds(pl.multiple_of(sr * (SEG // 2), SEG // 2), SEG // 2), :]),
                 _unpack(wop_ref[:, cols]))
        x = x_ref[seg_rows(sr), cols] + y
        x_ref[seg_rows(sw), cols] = x
        xa_ref[:, cols] = x

    def a_norm(first, sg, slot, i, chain):
        x = x_ref[seg_rows(sg, 8 * i, 8), :] if first else xa_ref[8 * i:8 * i + 8, :]
        xnb_ref[slot, 8 * i:8 * i + 8, :] = _ln_chained(x, chain)

    def a_phase2(first):
        if first:
            cp_w(2, NTR - 2).wait()
            cp_woa.wait()
        r = lax.broadcasted_iota(i32, (RA + 8, 2 * RA), 0)
        rb = jnp.where(((r >= DA) & (r < RA)) | (r >= RA + 4), 1, 0)
        same = rb == (lax.broadcasted_iota(i32, (RA + 8, 2 * RA), 1) & 1)
        for p in range(NPA):
            kvm_ref[p] = _pack(jnp.where(same, kv_ref[p], 0.0))

        def attend(c):
            top = lax.broadcasted_iota(i32, (8, TC), 0) < 4
            ot = []
            for p in range(NPA):
                ne = _dot(_unpack(kvm_ref[p]), _unpack(phiq_ref[c, p]))
                rc = 1.0 / (ne[RA:RA + 8] + 1e-6)
                sw = pltpu.roll(rc, 4, 0)
                ra, rb = jnp.where(top, rc, sw), jnp.where(top, sw, rc)
                ot.append(ne[0:RA] * jnp.concatenate([ra, ra, rc, rb, rb], axis=0))
            o = jnp.concatenate(ot, axis=0).T
            oa_ref[pl.ds(pl.multiple_of(c * (TC // 2), TC // 2), TC // 2), :] = _pack(o)

        if not first:
            for c in range(NCH):
                attend(c)
                if c == 2:
                    for n in range(D // 128):
                        a_finish(0, 0, n)
                    for i in range(4):
                        a_norm(False, 0, 0, i, [])
            return

        wop_ref[...] = pltpu.bitcast(wo_a[...], u32)
        attend(0)

        def body(c, carry):
            @pl.when(c == 2)
            def _():
                for n in range(3):
                    cp_w(n, NTR - 1).wait()

            @pl.when(c >= 2)
            def _():
                cp_w(3, c - 2).wait()

            lhs = [_unpack(oa_ref[pl.ds(pl.multiple_of(c * (TC // 2) + r // 2, 64), 64), :])
                   for r in range(0, TC, 128)]
            attend(jnp.minimum(c + 1, NCH - 1))
            t = jnp.maximum(c - 2, 0)
            transpose_w(jnp.where(c < 2, 2, t // 2), jnp.where(c < 2, NPB - 4, NPB - 2) + c % 2)
            pack_wo(jnp.where(c < 2, NTR, t))
            for r in range(0, TC, 128):
                x_ref[pl.ds(pl.multiple_of(c * TC + r, 128), 128), :] += _dot(lhs[r // 128], _unpack(wop_ref[...]))
            return carry

        lax.fori_loop(0, NCH, body, 0)

    def b_finish(first, sr, sw, slot, i, chain):
        x = x_ref[seg_rows(sr, 16 * i, 16), :] + yb_ref[slot, 16 * i:16 * i + 16, :]
        if first:
            x_ref[seg_rows(sw, 16 * i, 16), :] = x
            xb_ref[16 * i:16 * i + 16, :] = x
            xn = [_ln_chained(xb_ref[16 * i + k:16 * i + k + 8, :], chain) for k in (0, 8)]
            xna_ref[pl.ds(pl.multiple_of(sr * (SEG // 2) + 8 * i, 8), 8), :] = _pack(
                jnp.concatenate(xn, axis=0))
        else:
            xin_ref[pl.ds(pl.multiple_of(sr * SEG + 16 * i, 16), 16), :] = x.astype(bf16)

    def b_step(h, side, chain):
        st = {}

        def proj(p, which):
            if p == 0 and which == 0:
                y = _dot(h[:, 0:128], _unpack(wb_ref[0, 0, 0:64, :]))
                for k in range(1, D // 128):
                    y = y + _dot(h[:, 128 * k:128 * k + 128], _unpack(wb_ref[0, 0, 64 * k:64 * k + 64, :]))
            else:
                y = _dot(h, _unpack(wb_ref[which, p]))
            if which == 0:
                st[(p, 'qv')] = y[0:8] * SCALE
                y = jnp.concatenate([y[SEG:L], y[8:SEG]], axis=0)
                st[(p, 0)] = (jnp.concatenate([y[:, 0:128], y[:, 256:384]], axis=0).astype(bf16), y[:, 128:256])
                return
            y = jnp.concatenate([y[SEG:L], y[0:SEG]], axis=0)
            st[(p, 'kv', which)] = y[0:16]
            if which == 1:
                st[(p, 1)] = _split(y)
            else:
                lo = (lax.broadcasted_iota(i32, (L, PW), 1) & 64) == 0
                st[(p, 2)] = jnp.concatenate([jnp.where(lo, y, 0.0), jnp.where(lo, 0.0, y)], axis=0).astype(bf16)

        def do_qk(p):
            zeros = chain[:1] + st.pop('tie', [])
            del chain[:1]
            st[(p, 'p')] = _probs(st.pop((p, 0)), st.pop((p, 1)), zeros)

        def do_pv(p):
            cols = slice(p * PW, (p + 1) * PW)
            o = _dot(st.pop((p, 'p')), st.pop((p, 2)))
            o_ref[0:MEM, cols] = o[0:MEM]
            o_ref[2 * MEM:L, cols] = o[MEM:LM]

        def do_vpu(p):
            cols = slice(p * PW, (p + 1) * PW)
            lo = lax.broadcasted_iota(i32, (8, 128), 1) < 64
            row = lax.broadcasted_iota(i32, (8, 128), 0)
            q = st.pop((p, 'qv'))
            qa, qb = jnp.where(lo, q[:, 128:256], 0.0), jnp.where(lo, 0.0, q[:, 128:256])

            kk, vv = st.pop((p, 'kv', 1)), st.pop((p, 'kv', 2))
            sc = []
            for k in range(16):
                km = jnp.broadcast_to(kk[k:k + 1, 128:256], (8, 128))
                xa = jnp.sum(q[:, 0:128] * kk[k:k + 1, 0:128] + qa * km, axis=-1, keepdims=True)
                xb = jnp.sum(q[:, 256:384] * kk[k:k + 1, 256:384] + qb * km, axis=-1, keepdims=True)
                x = jnp.where(lo, xa, xb)
                sc.append(jnp.where(row >= k - MEM, x, -1000000000.0) if k > MEM else x)
            m = functools.reduce(jnp.maximum, sc)
            ev = [jnp.exp2(x - m) for x in sc]
            rr = 1.0 / functools.reduce(jnp.add, ev)
            z = _zero(m)
            ov = []
            for t in range(3):
                v = [vv[8 * b:8 * b + 8, 128 * t:128 * t + 128] + z for b in range(2)]
                ov.append(functools.reduce(
                    jnp.add, [ev[k] * v[k // 8][k % 8:k % 8 + 1] for k in range(16)]) * rr)
                z = _zero(ov[-1])
            o_ref[MEM:2 * MEM, cols] = jnp.concatenate(ov, axis=1)
            st['tie'] = [z[:, 0:2 * L]]

        def do_o(n):
            k0 = st.get('k', 0)
            k1 = st['k'] = k0 + n
            y = _dot(o_ref[:, k0 * 128:k1 * 128], _unpack(wo_ref[k0 * 64:k1 * 64, :]))
            st['y'] = y if 'y' not in st else st['y'] + y

        for s in range(NPB):
            proj(s, 0)
            if s >= 4:
                do_o(1)
            if s >= 1:
                do_qk(s - 1)
            proj(s, 1)
            if s >= 2:
                do_pv(s - 2)
            if s >= 1:
                do_vpu(s - 1)
            proj(s, 2)
            if s >= 4:
                do_o(1)
            for job in side[s]:
                job()
            assert st.get('k', 0) <= 3 * max(s - 2, 0)
        do_o(2)
        do_qk(NPB - 1)
        do_vpu(NPB - 1)
        do_o(4)
        do_pv(NPB - 2)
        do_o(7)
        assert st['k'] <= 3 * (NPB - 2)
        do_pv(NPB - 1)
        do_o(3 * (NPB - 1) - st['k'])
        do_o(3)
        return st['y']

    def layer_b(first):
        SPI = SPI1 if first else SPI2
        mem_ref[...] = mem0[...].astype(f32)
        yb_ref[1] = jnp.zeros((SEG, D), f32)
        if first:
            for i in range(4):
                a_norm(first, 0, 0, i, [])
            with jax.named_scope("wait_wo"):
                for j in range(NTR - 2, NTR):
                    cp_w(3, j).wait()
                    pack_wo(j)

        def body(j, carry):
            mem = mem_ref[...]
            for t in range(SPI):
                sg = j * SPI + t
                if not first and t % 2 == 0:
                    @pl.when(sg >= 4)
                    def _():
                        cp_rows(sg - 3, 2).start()

                sp = jnp.maximum(sg - 1, 0) if t == 0 else sg - 1
                sw = jnp.where(sg == 0, NSEG, sp) if t == 0 else sp
                sn = jnp.minimum(sg + 1, NSEG - 1) if t == SPI - 1 else sg + 1
                h = jnp.concatenate([xnb_ref[t % 2], mem], axis=0)
                chain = []
                side = [[] for _ in range(NPB)]
                for i in range(2):
                    side[1 + 2 * i].append(functools.partial(b_finish, first, sp, sw, (t + 1) % 2, i, chain))
                if not first:
                    for n in range(D // 128):
                        side[n].append(functools.partial(a_finish, sn, sg + 1, n))
                for i in range(4):
                    side[6 + 2 * i].append(functools.partial(a_norm, first, sn, (t + 1) % 2, i, chain))
                y = b_step(h, side, chain)
                mem = y[0:MEM]
                yb_ref[t % 2] = y[MEM:L]
            mem_ref[...] = mem
            return carry

        with jax.named_scope("b_loop"):
            lax.fori_loop(0, NSEG // SPI, body, 0)
        if not first:
            cp_rows(0, 1).start()
            cp_rows(NSEG - 3, 2).start()
        for i in range(2):
            b_finish(first, NSEG - 1, NSEG - 1, 1, i, [])

    for first in (True, False):
        kv_ref[...] = jnp.zeros(kv_ref.shape, f32)
        with jax.named_scope("a_p1"):
            a_phase1(first)
        with jax.named_scope("a_p2"):
            a_phase2(first)
        with jax.named_scope("layer_b"):
            layer_b(first)

    cp_rows(NSEG - 1, 1).start()
    cp_rows(0, NSEG).wait()


@jax.jit
def pallas_interleave_layers__linear_kernel_hedgehog__memory_aug_recurrent_mem_tr__prompt_kernel(
    A_x: jax.Array,
    A_wqkv: jax.Array,
    A_w_phi: jax.Array,
    A_wo: jax.Array,
    B_x: jax.Array,
    B_mem0: jax.Array,
    B_Wq: jax.Array,
    B_Wk: jax.Array,
    B_Wv: jax.Array,
    B_Wo: jax.Array,
    B_seg_len: jax.Array,
):
    del B_x, B_seg_len
    x = A_x.reshape(S, D)
    phi = A_w_phi.transpose(1, 2, 0)
    wqt = B_Wq.transpose(1, 2, 0).reshape(HD, D)
    wkt = B_Wk.transpose(1, 2, 0).reshape(HD, D)
    wvt = B_Wv.transpose(1, 2, 0).reshape(HD, D)
    wo = B_Wo.reshape(HD, D)
    hbm = pl.BlockSpec(memory_space=pl.ANY)
    out = pl.pallas_call(
        _kernel,
        out_shape=jax.ShapeDtypeStruct((S, D), bf16),
        in_specs=[hbm] * 9,
        out_specs=hbm,
        scratch_shapes=[
            pltpu.VMEM((S, D), bf16),
            pltpu.VMEM((3, D, D), bf16),
            pltpu.VMEM((DA, DA, HA), bf16),
            pltpu.VMEM((D, D), bf16),
            pltpu.VMEM((MEM, D), bf16),
            pltpu.VMEM((S + SEG, D), f32),
            pltpu.VMEM((S // 2, D), u32),
            pltpu.VMEM((2, SEG, D), f32),
            pltpu.VMEM((SEG, D), f32),
            pltpu.VMEM((SEG, D), f32),
            pltpu.VMEM((2, SEG, D), f32),
            pltpu.VMEM((S // 2, D), u32),
            pltpu.VMEM((3, GA, 80, D), u32),
            pltpu.VMEM((D // 2, D), u32),
            pltpu.VMEM((2, GA, 160, 256), f32),
            pltpu.VMEM((NCH, NPA, RA, TC), u32),
            pltpu.VMEM((NPA, RA + 8, 2 * RA), f32),
            pltpu.VMEM((NPA, (RA + 8) // 2, 2 * RA), u32),
            pltpu.VMEM((4, HD + TRC, D), bf16),
            pltpu.VMEM((3, NPB + 2, D // 2, PW), u32),
            pltpu.VMEM(((HD + TRC) // 2, D), u32),
            pltpu.VMEM((MEM, D), f32),
            pltpu.VMEM((L, HD), f32),
            pltpu.SemaphoreType.DMA((20 + 4 * NTR,)),
        ],
        compiler_params=pltpu.CompilerParams(vmem_limit_bytes=120 * 1024 * 1024),
    )(x, A_wqkv, phi, A_wo, B_mem0.reshape(MEM, D), wqt, wkt, wvt, wo)
    return out.reshape(1, S, D)
```

```python
import functools

import jax
import jax.numpy as jnp
from jax import lax
import jax.experimental.pallas as pl
import jax.experimental.pallas.tpu as pltpu

f32, bf16, u32, i32 = jnp.float32, jnp.bfloat16, jnp.uint32, jnp.int32

S, D = 2048, 640
HA, DA = 32, 20
NPA = HA // 2
RA = 2 * DA
GA = 4
TC = 256
NCH = S // TC
XCH = 256
HB, DB, MEM, SEG = 32, 192, 8, 32
HD = HB * DB
L = MEM + SEG
LM = L - 8
VBLK = (0, 192, 64, 256, 128, 320)
NPB = HB // 2
PW = 2 * DB
SCALE = DB ** -0.5 * 1.4426950408889634
TRC = 768
NTR = HD // TRC
NSEG = S // SEG
SPI1, SPI2 = 2, 4
assert NTR == NCH

_NN = (((1,), (0,)), ((), ()))
_NT = (((1,), (1,)), ((), ()))


def _dot(a, b):
    return lax.dot_general(a, b, _NN, preferred_element_type=f32)


def _dot_nt(a, b):
    return lax.dot_general(a, b, _NT, preferred_element_type=f32)


def _pack(x):
    return pltpu.bitcast(x.astype(bf16), u32)


def _unpack(x):
    return pltpu.bitcast(x, bf16)


def _ln(x):
    m = jnp.mean(x, axis=-1, keepdims=True)
    xc = x - m
    r = lax.rsqrt(jnp.mean(xc * xc, axis=-1, keepdims=True) + 1e-5)
    return x * r - m * r


def _ln_chained(x, chain):
    m = jnp.mean(x, axis=-1, keepdims=True)
    xc = x - m
    r = lax.rsqrt(jnp.mean(xc * xc, axis=-1, keepdims=True) + 1e-5)
    chain.append(jnp.minimum(r, 0.0))
    return x * r - m * r


def _fold(op, p):
    r = p[0:8]
    for j in range(1, 5):
        r = op(r, p[8 * j:8 * j + 8])
    r = op(r, pltpu.roll(r, 2, 0))
    return op(r, pltpu.roll(r, 4, 0))


def _tile5(r):
    return jnp.concatenate([r] * 5, axis=0)


def _phi(p):
    ep = jnp.exp(p - _tile5(_fold(jnp.maximum, p)))
    en = jnp.exp(_tile5(_fold(jnp.minimum, p)) - p)
    ep = ep * _tile5(1.0 / _fold(jnp.add, ep))
    en = en * _tile5(1.0 / _fold(jnp.add, en))
    return jnp.concatenate([ep, en], axis=0).astype(bf16)


def _split(k):
    lo = lax.broadcasted_iota(i32, (L, 128), 1) < 64
    z = jnp.zeros((L, 128), f32)
    mid = k[:, 128:256]
    outer = jnp.concatenate([k[:, 0:128], k[:, 256:384]], axis=0).astype(bf16)
    mid = jnp.concatenate([jnp.where(lo, mid, z), jnp.where(lo, z, mid)], axis=0).astype(bf16)
    return outer, mid


def _zero(x):
    return jnp.minimum(jnp.abs(x), 0.0)


def _probs(q, k, zeros):
    r = lax.broadcasted_iota(i32, (LM, 2 * L), 0)
    c = lax.broadcasted_iota(i32, (LM, 2 * L), 1)
    first = c < L
    so = _dot_nt(q[0], k[0])
    s = jnp.where(first, so[0:LM], so[LM:2 * LM]) + _dot_nt(q[1], k[1])
    s = s * SCALE
    if zeros:
        s = jnp.concatenate([functools.reduce(jnp.add, zeros, s[0:8]), s[8:LM]], axis=0)
    mask = (r < MEM) | (r + 8 >= jnp.where(first, c, c - L))
    s = jnp.where(mask, s, -1000000000.0)
    neg = jnp.full_like(s, -jnp.inf)
    ma = jnp.max(jnp.where(first, s, neg), axis=-1, keepdims=True)
    mb = jnp.max(jnp.where(first, neg, s), axis=-1, keepdims=True)
    e = jnp.exp2(s - jnp.where(first, ma, mb))
    z = jnp.zeros_like(e)
    sa = jnp.sum(jnp.where(first, e, z), axis=-1, keepdims=True)
    sb = jnp.sum(jnp.where(first, z, e), axis=-1, keepdims=True)
    return e * (1.0 / jnp.where(first, sa, sb))


def _kernel(x_hbm, wqkv_hbm, phi_hbm, woa_hbm, mem0_hbm, wqt_hbm, wkt_hbm, wvt_hbm, wo_hbm, out_hbm,
            xin_ref, wqkv, phi_ref, wo_a, mem0, x_ref, xna_ref, xnb_ref, xa_ref, xb_ref, yb_ref, oa_ref,
            wat_ref, wop_ref, lhs_ref, phiq_ref, kv_ref, kvm_ref, stage_ref, wb_ref, wo_ref, mem_ref, o_ref,
            sems):
    cp_phi = pltpu.make_async_copy(phi_hbm, phi_ref, sems.at[0])
    cp_mem0 = pltpu.make_async_copy(mem0_hbm, mem0, sems.at[1])
    cp_woa = pltpu.make_async_copy(woa_hbm, wo_a, sems.at[2])
    big = (wqt_hbm, wkt_hbm, wvt_hbm, wo_hbm)

    def cp_wqkv(n):
        return pltpu.make_async_copy(wqkv_hbm.at[:, pl.ds(pl.multiple_of(D * n, 128), D)], wqkv.at[n],
                                     sems.at[4 + n])

    def cp_x(j):
        rows = pl.ds(pl.multiple_of(j * XCH, XCH), XCH)
        return pltpu.make_async_copy(x_hbm.at[rows, :], xin_ref.at[rows, :], sems.at[12 + j])

    def cp_w(n, j):
        rows = pl.ds(pl.multiple_of(j * TRC, TRC), TRC)
        return pltpu.make_async_copy(big[n].at[rows, :], stage_ref.at[n, rows, :], sems.at[20 + n * NTR + j])

    def cp_rows(sg, nseg):
        rows = pl.ds(pl.multiple_of(sg * SEG, SEG), SEG * nseg)
        return pltpu.make_async_copy(xin_ref.at[rows, :], out_hbm.at[rows, :], sems.at[3])

    cp_phi.start()
    for n in range(3):
        cp_wqkv(n).start()
    for j in range(S // XCH):
        cp_x(j).start()
    cp_mem0.start()
    for j in range(NTR):
        if j == NTR - 1:
            cp_woa.start()
        for n in range(3):
            cp_w(n, j).start()
    for j in range(NTR):
        cp_w(3, j).start()

    def init_x(c, carry):
        with jax.named_scope("wait_x"):
            cp_x(c).wait()
        x = xin_ref[pl.ds(pl.multiple_of(c * XCH, XCH), XCH), :].astype(f32)
        x_ref[pl.ds(pl.multiple_of(c * XCH, XCH), XCH), :] = x
        xna_ref[pl.ds(pl.multiple_of(c * (XCH // 2), XCH // 2), XCH // 2), :] = _pack(_ln(x))
        return carry

    stage_ref[:, HD:HD + 64, :] = jnp.zeros((4, 64, D), bf16)

    with jax.named_scope("wait_phi"):
        cp_phi.wait()
    ecol = lax.broadcasted_iota(i32, (HA, D), 1) - DA * lax.broadcasted_iota(i32, (HA, D), 0)

    def scatter_phi(i, tp):
        for d in range(5):
            tp = tp + _dot(phi_ref[5 * i + d], jnp.where(ecol == 5 * i + d, 1.0, 0.0).astype(bf16))
        return tp

    tp = lax.fori_loop(0, DA // 5, scatter_phi, jnp.zeros((DA, D), f32))
    rep = jnp.where((lax.broadcasted_iota(i32, (RA, DA), 0) >> 1) == lax.broadcasted_iota(i32, (RA, DA), 1),
                    1.0, 0.0).astype(bf16)
    urep = _dot(rep, tp.astype(bf16))
    for g in range(GA):
        col = lax.broadcasted_iota(i32, (RA, 256), 1) + 128 * g
        par = lax.broadcasted_iota(i32, (RA, 256), 0) & 1
        for pp in range(4):
            lo = (8 * g + 2 * pp + par) * DA
            blk = jnp.where((col >= lo) & (col < lo + DA), urep[:, 128 * g:128 * g + 256], 0.0)
            lhs_ref[0, g, RA * pp:RA * pp + RA, :] = blk
        lhs_ref[1, g] = jnp.where(lax.broadcasted_iota(i32, (160, 256), 1) + 128 * g
                                  == lax.broadcasted_iota(i32, (160, 256), 0) + 160 * g, 1.0, 0.0)

    def prep(n, carry):
        with jax.named_scope("wait_wqkv"):
            cp_wqkv(n).wait()
        for g in range(GA):
            wat_ref[n, g] = _pack(_dot_nt(lhs_ref[n // 2, g].astype(bf16), wqkv[n, :, 128 * g:128 * g + 256]))
        return carry

    with jax.named_scope("prep"):
        lax.fori_loop(0, 3, prep, 0)
    with jax.named_scope("init_x"):
        lax.fori_loop(0, S // XCH, init_x, 0)
        cp_mem0.wait()

    def transpose_w(n, p):
        blocks = []
        for i in range(6):
            off = jnp.minimum(p * PW + jnp.where(n == 2, VBLK[i], 64 * i), HD)
            blocks.append(stage_ref[n, pl.ds(pl.multiple_of(off, 64), 64), :])
        wb_ref[n, p] = pltpu.bitcast(jnp.concatenate(blocks, axis=0).T, u32)

    def pack_wo(j):
        for i in range(12):
            src = pl.ds(pl.multiple_of(jnp.minimum(j * TRC + (i // 6) * PW + VBLK[i % 6], HD), 64), 64)
            wo_ref[pl.ds(pl.multiple_of(j * (TRC // 2) + 32 * i, 32), 32), :] = pltpu.bitcast(
                stage_ref[3, src, :], u32)

    def a_phase1(first):
        def body(c, carry):
            if first:
                ct = [jnp.where(c < lag, NTR, c - lag) for lag in (1, 1, 2)]

                @pl.when(c >= 2)
                def _():
                    cp_w(2, c - 2).wait()

                @pl.when(c >= 1)
                def _():
                    with jax.named_scope("wait_w"):
                        cp_w(0, c - 1).wait()
                        cp_w(1, c - 1).wait()

            xn = _unpack(xna_ref[pl.ds(pl.multiple_of(c * (TC // 2), TC // 2), TC // 2), :])
            ones = jnp.ones((8, TC), f32)
            pend = []
            for g in range(GA):
                pq = _dot_nt(_unpack(wat_ref[0, g]), xn)
                pk = _dot_nt(_unpack(wat_ref[1, g]), xn)
                vt = _dot_nt(_unpack(wat_ref[2, g]), xn)
                for pp in range(4):
                    p = 4 * g + pp
                    sl = slice(RA * pp, RA * pp + RA)
                    phiq_ref[c, p] = pltpu.bitcast(_phi(pq[sl]), u32)
                    vext = jnp.concatenate([vt[sl], ones], axis=0).astype(bf16)
                    pend.append((p, vext, _phi(pk[sl])))
                if first and g < 3:
                    transpose_w(g, 2 * ct[g])
                    transpose_w(g, 2 * ct[g] + 1)
            for p, vext, phik in pend:
                kv_ref[p] += _dot_nt(vext, phik)
            return carry

        lax.fori_loop(0, NCH, body, 0, unroll=1 if first else 2)

    def seg_rows(sg, off=0, n=SEG):
        return pl.ds(pl.multiple_of(sg * SEG + off, 8), n)

    def a_finish(sr, sw, n):
        cols = slice(128 * n, 128 * n + 128)
        y = _dot(_unpack(oa_ref[pl.ds(pl.multiple_of(sr * (SEG // 2), SEG // 2), SEG // 2), :]),
                 _unpack(wop_ref[:, cols]))
        x = x_ref[seg_rows(sr), cols] + y
        x_ref[seg_rows(sw), cols] = x
        xa_ref[:, cols] = x

    def a_norm(first, sg, slot, i, chain):
        x = x_ref[seg_rows(sg, 8 * i, 8), :] if first else xa_ref[8 * i:8 * i + 8, :]
        xnb_ref[slot, 8 * i:8 * i + 8, :] = _ln_chained(x, chain)

    def a_phase2(first):
        if first:
            cp_w(2, NTR - 2).wait()
            cp_woa.wait()
        r = lax.broadcasted_iota(i32, (RA + 8, 2 * RA), 0)
        rb = jnp.where(((r >= DA) & (r < RA)) | (r >= RA + 4), 1, 0)
        same = rb == (lax.broadcasted_iota(i32, (RA + 8, 2 * RA), 1) & 1)
        for p in range(NPA):
            kvm_ref[p] = _pack(jnp.where(same, kv_ref[p], 0.0))

        def attend(c):
            top = lax.broadcasted_iota(i32, (8, TC), 0) < 4
            ot = []
            for p in range(NPA):
                ne = _dot(_unpack(kvm_ref[p]), _unpack(phiq_ref[c, p]))
                rc = 1.0 / (ne[RA:RA + 8] + 1e-6)
                sw = pltpu.roll(rc, 4, 0)
                ra, rb = jnp.where(top, rc, sw), jnp.where(top, sw, rc)
                ot.append(ne[0:RA] * jnp.concatenate([ra, ra, rc, rb, rb], axis=0))
            o = jnp.concatenate(ot, axis=0).T
            oa_ref[pl.ds(pl.multiple_of(c * (TC // 2), TC // 2), TC // 2), :] = _pack(o)

        if not first:
            for c in range(NCH):
                attend(c)
                if c == 2:
                    for n in range(D // 128):
                        a_finish(0, 0, n)
                    for i in range(4):
                        a_norm(False, 0, 0, i, [])
            return

        wop_ref[...] = pltpu.bitcast(wo_a[...], u32)
        attend(0)

        def body(c, carry):
            @pl.when(c == 2)
            def _():
                for n in range(3):
                    cp_w(n, NTR - 1).wait()

            @pl.when(c >= 2)
            def _():
                cp_w(3, c - 2).wait()

            lhs = [_unpack(oa_ref[pl.ds(pl.multiple_of(c * (TC // 2) + r // 2, 64), 64), :])
                   for r in range(0, TC, 128)]
            attend(jnp.minimum(c + 1, NCH - 1))
            t = jnp.maximum(c - 2, 0)
            transpose_w(jnp.where(c < 2, 2, t // 2), jnp.where(c < 2, NPB - 4, NPB - 2) + c % 2)
            pack_wo(jnp.where(c < 2, NTR, t))
            for r in range(0, TC, 128):
                x_ref[pl.ds(pl.multiple_of(c * TC + r, 128), 128), :] += _dot(lhs[r // 128], _unpack(wop_ref[...]))
            return carry

        lax.fori_loop(0, NCH, body, 0)

    def b_finish(first, sr, sw, slot, i, chain):
        x = x_ref[seg_rows(sr, 16 * i, 16), :] + yb_ref[slot, 16 * i:16 * i + 16, :]
        if first:
            x_ref[seg_rows(sw, 16 * i, 16), :] = x
            xb_ref[16 * i:16 * i + 16, :] = x
            xn = [_ln_chained(xb_ref[16 * i + k:16 * i + k + 8, :], chain) for k in (0, 8)]
            xna_ref[pl.ds(pl.multiple_of(sr * (SEG // 2) + 8 * i, 8), 8), :] = _pack(
                jnp.concatenate(xn, axis=0))
        else:
            xin_ref[pl.ds(pl.multiple_of(sr * SEG + 16 * i, 16), 16), :] = x.astype(bf16)

    def b_step(h, side, chain):
        st = {}

        def proj(p, which):
            if p == 0 and which == 0:
                y = _dot(h[:, 0:128], _unpack(wb_ref[0, 0, 0:64, :]))
                for k in range(1, D // 128):
                    y = y + _dot(h[:, 128 * k:128 * k + 128], _unpack(wb_ref[0, 0, 64 * k:64 * k + 64, :]))
            else:
                y = _dot(h, _unpack(wb_ref[which, p]))
            if which == 0:
                st[(p, 'qv')] = y[0:8] * SCALE
                y = jnp.concatenate([y[SEG:L], y[8:SEG]], axis=0)
                st[(p, 0)] = (jnp.concatenate([y[:, 0:128], y[:, 256:384]], axis=0).astype(bf16), y[:, 128:256])
                return
            y = jnp.concatenate([y[SEG:L], y[0:SEG]], axis=0)
            st[(p, 'kv', which)] = y[0:16]
            if which == 1:
                st[(p, 1)] = _split(y)
            else:
                lo = (lax.broadcasted_iota(i32, (L, PW), 1) & 64) == 0
                st[(p, 2)] = jnp.concatenate([jnp.where(lo, y, 0.0), jnp.where(lo, 0.0, y)], axis=0).astype(bf16)

        def do_qk(p):
            zeros = chain[:1] + st.pop('tie', [])
            del chain[:1]
            st[(p, 'p')] = _probs(st.pop((p, 0)), st.pop((p, 1)), zeros)

        def do_pv(p):
            cols = slice(p * PW, (p + 1) * PW)
            o = _dot(st.pop((p, 'p')), st.pop((p, 2)))
            o_ref[0:MEM, cols] = o[0:MEM]
            o_ref[2 * MEM:L, cols] = o[MEM:LM]

        def do_vpu(p):
            cols = slice(p * PW, (p + 1) * PW)
            lo = lax.broadcasted_iota(i32, (8, 128), 1) < 64
            row = lax.broadcasted_iota(i32, (8, 128), 0)
            q = st.pop((p, 'qv'))
            qa, qb = jnp.where(lo, q[:, 128:256], 0.0), jnp.where(lo, 0.0, q[:, 128:256])

            kk, vv = st.pop((p, 'kv', 1)), st.pop((p, 'kv', 2))
            sc = []
            for k in range(16):
                km = jnp.broadcast_to(kk[k:k + 1, 128:256], (8, 128))
                xa = jnp.sum(q[:, 0:128] * kk[k:k + 1, 0:128] + qa * km, axis=-1, keepdims=True)
                xb = jnp.sum(q[:, 256:384] * kk[k:k + 1, 256:384] + qb * km, axis=-1, keepdims=True)
                x = jnp.where(lo, xa, xb)
                sc.append(jnp.where(row >= k - MEM, x, -1000000000.0) if k > MEM else x)
            m = functools.reduce(jnp.maximum, sc)
            ev = [jnp.exp2(x - m) for x in sc]
            rr = 1.0 / functools.reduce(jnp.add, ev)
            z = _zero(m)
            ov = []
            for t in range(3):
                v = [vv[8 * b:8 * b + 8, 128 * t:128 * t + 128] + z for b in range(2)]
                ov.append(functools.reduce(
                    jnp.add, [ev[k] * v[k // 8][k % 8:k % 8 + 1] for k in range(16)]) * rr)
                z = _zero(ov[-1])
            o_ref[MEM:2 * MEM, cols] = jnp.concatenate(ov, axis=1)
            st['tie'] = [z[:, 0:2 * L]]

        def do_o(n):
            k0 = st.get('k', 0)
            k1 = st['k'] = k0 + n
            y = _dot(o_ref[:, k0 * 128:k1 * 128], _unpack(wo_ref[k0 * 64:k1 * 64, :]))
            st['y'] = y if 'y' not in st else st['y'] + y

        for s in range(NPB):
            proj(s, 0)
            if s >= 4:
                do_o(1)
            if s >= 1:
                do_qk(s - 1)
            proj(s, 1)
            if s >= 2:
                do_pv(s - 2)
            if s >= 1:
                do_vpu(s - 1)
            proj(s, 2)
            if s >= 4:
                do_o(1)
            for job in side[s]:
                job()
            assert st.get('k', 0) <= 3 * max(s - 2, 0)
        do_o(2)
        do_qk(NPB - 1)
        do_vpu(NPB - 1)
        do_o(4)
        do_pv(NPB - 2)
        do_o(7)
        assert st['k'] <= 3 * (NPB - 2)
        do_pv(NPB - 1)
        do_o(3 * (NPB - 1) - st['k'])
        do_o(3)
        return st['y']

    def layer_b(first):
        SPI = SPI1 if first else SPI2
        mem_ref[...] = mem0[...].astype(f32)
        yb_ref[1] = jnp.zeros((SEG, D), f32)
        if first:
            for i in range(4):
                a_norm(first, 0, 0, i, [])
            with jax.named_scope("wait_wo"):
                for j in range(NTR - 2, NTR):
                    cp_w(3, j).wait()
                    pack_wo(j)

        def body(j, carry):
            mem = mem_ref[...]
            for t in range(SPI):
                sg = j * SPI + t
                if not first and t % 2 == 0:
                    @pl.when(sg >= 4)
                    def _():
                        cp_rows(sg - 3, 2).start()

                sp = jnp.maximum(sg - 1, 0) if t == 0 else sg - 1
                sw = jnp.where(sg == 0, NSEG, sp) if t == 0 else sp
                sn = jnp.minimum(sg + 1, NSEG - 1) if t == SPI - 1 else sg + 1
                h = jnp.concatenate([xnb_ref[t % 2], mem], axis=0)
                chain = []
                side = [[] for _ in range(NPB)]
                for i in range(2):
                    side[1 + 2 * i].append(functools.partial(b_finish, first, sp, sw, (t + 1) % 2, i, chain))
                if not first:
                    for n in range(D // 128):
                        side[n].append(functools.partial(a_finish, sn, sg + 1, n))
                for i in range(4):
                    side[6 + 2 * i].append(functools.partial(a_norm, first, sn, (t + 1) % 2, i, chain))
                y = b_step(h, side, chain)
                mem = y[0:MEM]
                yb_ref[t % 2] = y[MEM:L]
            mem_ref[...] = mem
            return carry

        with jax.named_scope("b_loop"):
            lax.fori_loop(0, NSEG // SPI, body, 0)
        if not first:
            cp_rows(0, 1).start()
            cp_rows(NSEG - 3, 2).start()
        for i in range(2):
            b_finish(first, NSEG - 1, NSEG - 1, 1, i, [])

    for first in (True, False):
        kv_ref[...] = jnp.zeros(kv_ref.shape, f32)
        with jax.named_scope("a_p1"):
            a_phase1(first)
        with jax.named_scope("a_p2"):
            a_phase2(first)
        with jax.named_scope("layer_b"):
            layer_b(first)

    cp_rows(NSEG - 1, 1).start()
    cp_rows(0, NSEG).wait()


@jax.jit
def pallas_interleave_layers__linear_kernel_hedgehog__memory_aug_recurrent_mem_tr__prompt_kernel(
    A_x: jax.Array,
    A_wqkv: jax.Array,
    A_w_phi: jax.Array,
    A_wo: jax.Array,
    B_x: jax.Array,
    B_mem0: jax.Array,
    B_Wq: jax.Array,
    B_Wk: jax.Array,
    B_Wv: jax.Array,
    B_Wo: jax.Array,
    B_seg_len: jax.Array,
):
    del B_x, B_seg_len
    x = A_x.reshape(S, D)
    phi = A_w_phi.transpose(1, 2, 0)
    wqt = B_Wq.transpose(1, 2, 0).reshape(HD, D)
    wkt = B_Wk.transpose(1, 2, 0).reshape(HD, D)
    wvt = B_Wv.transpose(1, 2, 0).reshape(HD, D)
    wo = B_Wo.reshape(HD, D)
    hbm = pl.BlockSpec(memory_space=pl.ANY)
    out = pl.pallas_call(
        _kernel,
        out_shape=jax.ShapeDtypeStruct((S, D), bf16),
        in_specs=[hbm] * 9,
        out_specs=hbm,
        scratch_shapes=[
            pltpu.VMEM((S, D), bf16),
            pltpu.VMEM((3, D, D), bf16),
            pltpu.VMEM((DA, DA, HA), bf16),
            pltpu.VMEM((D, D), bf16),
            pltpu.VMEM((MEM, D), bf16),
            pltpu.VMEM((S + SEG, D), f32),
            pltpu.VMEM((S // 2, D), u32),
            pltpu.VMEM((2, SEG, D), f32),
            pltpu.VMEM((SEG, D), f32),
            pltpu.VMEM((SEG, D), f32),
            pltpu.VMEM((2, SEG, D), f32),
            pltpu.VMEM((S // 2, D), u32),
            pltpu.VMEM((3, GA, 80, D), u32),
            pltpu.VMEM((D // 2, D), u32),
            pltpu.VMEM((2, GA, 160, 256), f32),
            pltpu.VMEM((NCH, NPA, RA, TC), u32),
            pltpu.VMEM((NPA, RA + 8, 2 * RA), f32),
            pltpu.VMEM((NPA, (RA + 8) // 2, 2 * RA), u32),
            pltpu.VMEM((4, HD + 64, D), bf16),
            pltpu.VMEM((3, NPB + 2, D // 2, PW), u32),
            pltpu.VMEM(((HD + TRC) // 2, D), u32),
            pltpu.VMEM((MEM, D), f32),
            pltpu.VMEM((L, HD), f32),
            pltpu.SemaphoreType.DMA((20 + 4 * NTR,)),
        ],
        compiler_params=pltpu.CompilerParams(vmem_limit_bytes=120 * 1024 * 1024, disable_bounds_checks=True,
                                             disable_semaphore_checks=True),
    )(x, A_wqkv, phi, A_wo, B_mem0.reshape(MEM, D), wqt, wkt, wvt, wo)
    return out.reshape(1, S, D)
```

```python
import functools

import jax
import jax.numpy as jnp
from jax import lax
import jax.experimental.pallas as pl
import jax.experimental.pallas.tpu as pltpu

f32, bf16, u32, i32 = jnp.float32, jnp.bfloat16, jnp.uint32, jnp.int32

S, D = 2048, 640
HA, DA = 32, 20
NPA = HA // 2
RA = 2 * DA
GA = 4
TC = 256
NCH = S // TC
XCH = 256
HB, DB, MEM, SEG = 32, 192, 8, 32
HD = HB * DB
L = MEM + SEG
LM = L - 8
VBLK = (0, 192, 64, 256, 128, 320)
NPB = HB // 2
PW = 2 * DB
SCALE = DB ** -0.5 * 1.4426950408889634
TRC = 768
NTR = HD // TRC
NSEG = S // SEG
SPI1, SPI2 = 2, 4
assert NTR == NCH

_NN = (((1,), (0,)), ((), ()))
_NT = (((1,), (1,)), ((), ()))


def _dot(a, b):
    return lax.dot_general(a, b, _NN, precision=lax.Precision.DEFAULT, preferred_element_type=f32)


def _dot_nt(a, b):
    return lax.dot_general(a, b, _NT, precision=lax.Precision.DEFAULT, preferred_element_type=f32)


def _pack(x):
    return pltpu.bitcast(x.astype(bf16), u32)


def _unpack(x):
    return pltpu.bitcast(x, bf16)


def _ln(x):
    m = jnp.mean(x, axis=-1, keepdims=True)
    xc = x - m
    r = lax.rsqrt(jnp.mean(xc * xc, axis=-1, keepdims=True) + 1e-5)
    return x * r - m * r


def _ln_chained(x, chain):
    m = jnp.mean(x, axis=-1, keepdims=True)
    xc = x - m
    r = lax.rsqrt(jnp.mean(xc * xc, axis=-1, keepdims=True) + 1e-5)
    chain.append(jnp.minimum(r, 0.0))
    return x * r - m * r


def _fold(op, p):
    r = p[0:8]
    for j in range(1, 5):
        r = op(r, p[8 * j:8 * j + 8])
    r = op(r, pltpu.roll(r, 2, 0))
    return op(r, pltpu.roll(r, 4, 0))


def _tile5(r):
    return jnp.concatenate([r] * 5, axis=0)


def _phi(p):
    ep = jnp.exp(p - _tile5(_fold(jnp.maximum, p)))
    en = jnp.exp(_tile5(_fold(jnp.minimum, p)) - p)
    ep = ep * _tile5(1.0 / _fold(jnp.add, ep))
    en = en * _tile5(1.0 / _fold(jnp.add, en))
    return jnp.concatenate([ep, en], axis=0).astype(bf16)


def _split(k):
    lo = lax.broadcasted_iota(i32, (L, 128), 1) < 64
    z = jnp.zeros((L, 128), f32)
    mid = k[:, 128:256]
    outer = jnp.concatenate([k[:, 0:128], k[:, 256:384]], axis=0).astype(bf16)
    mid = jnp.concatenate([jnp.where(lo, mid, z), jnp.where(lo, z, mid)], axis=0).astype(bf16)
    return outer, mid


def _zero(x):
    return jnp.minimum(jnp.abs(x), 0.0)


def _probs(q, k, zeros):
    r = lax.broadcasted_iota(i32, (LM, 2 * L), 0)
    c = lax.broadcasted_iota(i32, (LM, 2 * L), 1)
    first = c < L
    so = _dot_nt(q[0], k[0])
    s = jnp.where(first, so[0:LM], so[LM:2 * LM]) + _dot_nt(q[1], k[1])
    s = s * SCALE
    if zeros:
        s = jnp.concatenate([functools.reduce(jnp.add, zeros, s[0:8]), s[8:LM]], axis=0)
    mask = (r < MEM) | (r + 8 >= jnp.where(first, c, c - L))
    s = jnp.where(mask, s, -1000000000.0)
    neg = jnp.full_like(s, -jnp.inf)
    ma = jnp.max(jnp.where(first, s, neg), axis=-1, keepdims=True)
    mb = jnp.max(jnp.where(first, neg, s), axis=-1, keepdims=True)
    e = jnp.exp2(s - jnp.where(first, ma, mb))
    z = jnp.zeros_like(e)
    sa = jnp.sum(jnp.where(first, e, z), axis=-1, keepdims=True)
    sb = jnp.sum(jnp.where(first, z, e), axis=-1, keepdims=True)
    return e * (1.0 / jnp.where(first, sa, sb))


def _kernel(x_hbm, wqkv_hbm, phi_hbm, woa_hbm, mem0_hbm, wqt_hbm, wkt_hbm, wvt_hbm, wo_hbm, out_hbm,
            xin_ref, wqkv, phi_ref, wo_a, mem0, x_ref, xna_ref, xnb_ref, xa_ref, xb_ref, yb_ref, oa_ref,
            wat_ref, wop_ref, lhs_ref, phiq_ref, kv_ref, kvm_ref, stage_ref, wb_ref, wo_ref, mem_ref, o_ref,
            sems):
    cp_phi = pltpu.make_async_copy(phi_hbm, phi_ref, sems.at[0])
    cp_mem0 = pltpu.make_async_copy(mem0_hbm, mem0, sems.at[1])
    cp_woa = pltpu.make_async_copy(woa_hbm, wo_a, sems.at[2])
    big = (wqt_hbm, wkt_hbm, wvt_hbm, wo_hbm)

    def cp_wqkv(n):
        return pltpu.make_async_copy(wqkv_hbm.at[:, pl.ds(pl.multiple_of(D * n, 128), D)], wqkv.at[n],
                                     sems.at[4 + n])

    def cp_x(j):
        rows = pl.ds(pl.multiple_of(j * XCH, XCH), XCH)
        return pltpu.make_async_copy(x_hbm.at[rows, :], xin_ref.at[rows, :], sems.at[12 + j])

    def cp_w(n, j):
        rows = pl.ds(pl.multiple_of(j * TRC, TRC), TRC)
        return pltpu.make_async_copy(big[n].at[rows, :], stage_ref.at[n, rows, :], sems.at[20 + n * NTR + j])

    def cp_rows(sg, nseg):
        rows = pl.ds(pl.multiple_of(sg * SEG, SEG), SEG * nseg)
        return pltpu.make_async_copy(xin_ref.at[rows, :], out_hbm.at[rows, :], sems.at[3])

    cp_phi.start()
    for n in range(3):
        cp_wqkv(n).start()
    for j in range(S // XCH):
        cp_x(j).start()
    cp_mem0.start()
    for j in range(NTR):
        if j == NTR - 1:
            cp_woa.start()
        for n in range(3):
            cp_w(n, j).start()
    for j in range(NTR):
        cp_w(3, j).start()

    def init_x(c, carry):
        with jax.named_scope("wait_x"):
            cp_x(c).wait()
        x = xin_ref[pl.ds(pl.multiple_of(c * XCH, XCH), XCH), :].astype(f32)
        x_ref[pl.ds(pl.multiple_of(c * XCH, XCH), XCH), :] = x
        xna_ref[pl.ds(pl.multiple_of(c * (XCH // 2), XCH // 2), XCH // 2), :] = _pack(_ln(x))
        return carry

    stage_ref[:, HD:HD + 64, :] = jnp.zeros((4, 64, D), bf16)

    with jax.named_scope("wait_phi"):
        cp_phi.wait()
    ecol = lax.broadcasted_iota(i32, (HA, D), 1) - DA * lax.broadcasted_iota(i32, (HA, D), 0)

    def scatter_phi(i, tp):
        for d in range(5):
            tp = tp + _dot(phi_ref[5 * i + d], jnp.where(ecol == 5 * i + d, 1.0, 0.0).astype(bf16))
        return tp

    tp = lax.fori_loop(0, DA // 5, scatter_phi, jnp.zeros((DA, D), f32))
    rep = jnp.where((lax.broadcasted_iota(i32, (RA, DA), 0) >> 1) == lax.broadcasted_iota(i32, (RA, DA), 1),
                    1.0, 0.0).astype(bf16)
    urep = _dot(rep, tp.astype(bf16))
    for g in range(GA):
        col = lax.broadcasted_iota(i32, (RA, 256), 1) + 128 * g
        par = lax.broadcasted_iota(i32, (RA, 256), 0) & 1
        for pp in range(4):
            lo = (8 * g + 2 * pp + par) * DA
            blk = jnp.where((col >= lo) & (col < lo + DA), urep[:, 128 * g:128 * g + 256], 0.0)
            lhs_ref[0, g, RA * pp:RA * pp + RA, :] = blk
        lhs_ref[1, g] = jnp.where(lax.broadcasted_iota(i32, (160, 256), 1) + 128 * g
                                  == lax.broadcasted_iota(i32, (160, 256), 0) + 160 * g, 1.0, 0.0)

    def prep(n, carry):
        with jax.named_scope("wait_wqkv"):
            cp_wqkv(n).wait()
        for g in range(GA):
            wat_ref[n, g] = _pack(_dot_nt(lhs_ref[n // 2, g].astype(bf16), wqkv[n, :, 128 * g:128 * g + 256]))
        return carry

    with jax.named_scope("prep"):
        lax.fori_loop(0, 3, prep, 0)
    with jax.named_scope("init_x"):
        lax.fori_loop(0, S // XCH, init_x, 0)
        cp_mem0.wait()

    def transpose_w(n, p):
        blocks = []
        for i in range(6):
            off = jnp.minimum(p * PW + jnp.where(n == 2, VBLK[i], 64 * i), HD)
            blocks.append(stage_ref[n, pl.ds(pl.multiple_of(off, 64), 64), :])
        wb_ref[n, p] = pltpu.bitcast(jnp.concatenate(blocks, axis=0).T, u32)

    def pack_wo(j):
        for i in range(12):
            src = pl.ds(pl.multiple_of(jnp.minimum(j * TRC + (i // 6) * PW + VBLK[i % 6], HD), 64), 64)
            wo_ref[pl.ds(pl.multiple_of(j * (TRC // 2) + 32 * i, 32), 32), :] = pltpu.bitcast(
                stage_ref[3, src, :], u32)

    def a_phase1(first):
        def body(c, carry):
            if first:
                ct = [jnp.where(c < lag, NTR, c - lag) for lag in (1, 1, 2)]

                @pl.when(c >= 2)
                def _():
                    cp_w(2, c - 2).wait()

                @pl.when(c >= 1)
                def _():
                    with jax.named_scope("wait_w"):
                        cp_w(0, c - 1).wait()
                        cp_w(1, c - 1).wait()

            xn = _unpack(xna_ref[pl.ds(pl.multiple_of(c * (TC // 2), TC // 2), TC // 2), :])
            ones = jnp.ones((8, TC), f32)
            pend = []
            for g in range(GA):
                pq = _dot_nt(_unpack(wat_ref[0, g]), xn)
                pk = _dot_nt(_unpack(wat_ref[1, g]), xn)
                vt = _dot_nt(_unpack(wat_ref[2, g]), xn)
                for pp in range(4):
                    p = 4 * g + pp
                    sl = slice(RA * pp, RA * pp + RA)
                    phiq_ref[c, p] = pltpu.bitcast(_phi(pq[sl]), u32)
                    vext = jnp.concatenate([vt[sl], ones], axis=0).astype(bf16)
                    pend.append((p, vext, _phi(pk[sl])))
                if first and g < 3:
                    transpose_w(g, 2 * ct[g])
                    transpose_w(g, 2 * ct[g] + 1)
            for p, vext, phik in pend:
                kv_ref[p] += _dot_nt(vext, phik)
            return carry

        lax.fori_loop(0, NCH, body, 0, unroll=1 if first else 2)

    def seg_rows(sg, off=0, n=SEG):
        return pl.ds(pl.multiple_of(sg * SEG + off, 8), n)

    def a_finish(sr, sw, n):
        cols = slice(128 * n, 128 * n + 128)
        y = _dot(_unpack(oa_ref[pl.ds(pl.multiple_of(sr * (SEG // 2), SEG // 2), SEG // 2), :]),
                 _unpack(wop_ref[:, cols]))
        x = x_ref[seg_rows(sr), cols] + y
        x_ref[seg_rows(sw), cols] = x
        xa_ref[:, cols] = x

    def a_norm(first, sg, slot, i, chain):
        x = x_ref[seg_rows(sg, 8 * i, 8), :] if first else xa_ref[8 * i:8 * i + 8, :]
        xnb_ref[slot, 8 * i:8 * i + 8, :] = _ln_chained(x, chain)

    def a_phase2(first):
        if first:
            cp_w(2, NTR - 2).wait()
            cp_woa.wait()
        r = lax.broadcasted_iota(i32, (RA + 8, 2 * RA), 0)
        rb = jnp.where(((r >= DA) & (r < RA)) | (r >= RA + 4), 1, 0)
        same = rb == (lax.broadcasted_iota(i32, (RA + 8, 2 * RA), 1) & 1)
        for p in range(NPA):
            kvm_ref[p] = _pack(jnp.where(same, kv_ref[p], 0.0))

        def attend(c):
            top = lax.broadcasted_iota(i32, (8, TC), 0) < 4
            ot = []
            for p in range(NPA):
                ne = _dot(_unpack(kvm_ref[p]), _unpack(phiq_ref[c, p]))
                rc = 1.0 / (ne[RA:RA + 8] + 1e-6)
                sw = pltpu.roll(rc, 4, 0)
                ra, rb = jnp.where(top, rc, sw), jnp.where(top, sw, rc)
                ot.append(ne[0:RA] * jnp.concatenate([ra, ra, rc, rb, rb], axis=0))
            o = jnp.concatenate(ot, axis=0).T
            oa_ref[pl.ds(pl.multiple_of(c * (TC // 2), TC // 2), TC // 2), :] = _pack(o)

        if not first:
            for c in range(NCH):
                attend(c)
                if c == 2:
                    for n in range(D // 128):
                        a_finish(0, 0, n)
                    for i in range(4):
                        a_norm(False, 0, 0, i, [])
            return

        wop_ref[...] = pltpu.bitcast(wo_a[...], u32)
        attend(0)

        def body(c, carry, last=False):
            @pl.when(c == 2)
            def _():
                for n in range(3):
                    cp_w(n, NTR - 1).wait()

            @pl.when(c >= 2)
            def _():
                cp_w(3, c - 2).wait()

            lhs = [_unpack(oa_ref[pl.ds(pl.multiple_of(c * (TC // 2) + r // 2, 64), 64), :])
                   for r in range(0, TC, 128)]
            if last:
                for i in range(4):
                    a_norm(True, 0, 0, i, [])
            else:
                attend(c + 1)
            t = jnp.maximum(c - 2, 0)
            transpose_w(jnp.where(c < 2, 2, t // 2), jnp.where(c < 2, NPB - 4, NPB - 2) + c % 2)
            pack_wo(jnp.where(c < 2, NTR, t))
            for r in range(0, TC, 128):
                x_ref[pl.ds(pl.multiple_of(c * TC + r, 128), 128), :] += _dot(lhs[r // 128], _unpack(wop_ref[...]))
            return carry

        lax.fori_loop(0, NCH - 1, body, 0)
        body(jnp.int32(NCH - 1), 0, last=True)

    def b_finish(first, sr, sw, slot, i, chain):
        x = x_ref[seg_rows(sr, 16 * i, 16), :] + yb_ref[slot, 16 * i:16 * i + 16, :]
        if first:
            x_ref[seg_rows(sw, 16 * i, 16), :] = x
            xb_ref[16 * i:16 * i + 16, :] = x
            xn = [_ln_chained(xb_ref[16 * i + k:16 * i + k + 8, :], chain) for k in (0, 8)]
            xna_ref[pl.ds(pl.multiple_of(sr * (SEG // 2) + 8 * i, 8), 8), :] = _pack(
                jnp.concatenate(xn, axis=0))
        else:
            xin_ref[pl.ds(pl.multiple_of(sr * SEG + 16 * i, 16), 16), :] = x.astype(bf16)

    def b_step(h, side, chain):
        st = {}

        def proj(p, which):
            if p == 0 and which == 0:
                y = _dot(h[:, 0:128], _unpack(wb_ref[0, 0, 0:64, :]))
                for k in range(1, D // 128):
                    y = y + _dot(h[:, 128 * k:128 * k + 128], _unpack(wb_ref[0, 0, 64 * k:64 * k + 64, :]))
            else:
                y = _dot(h, _unpack(wb_ref[which, p]))
            if which == 0:
                st[(p, 'qv')] = y[0:8] * SCALE
                y = jnp.concatenate([y[SEG:L], y[8:SEG]], axis=0)
                st[(p, 0)] = (jnp.concatenate([y[:, 0:128], y[:, 256:384]], axis=0).astype(bf16), y[:, 128:256])
                return
            y = jnp.concatenate([y[SEG:L], y[0:SEG]], axis=0)
            st[(p, 'kv', which)] = y[0:16]
            if which == 1:
                st[(p, 1)] = _split(y)
            else:
                lo = (lax.broadcasted_iota(i32, (L, PW), 1) & 64) == 0
                st[(p, 2)] = jnp.concatenate([jnp.where(lo, y, 0.0), jnp.where(lo, 0.0, y)], axis=0).astype(bf16)

        def do_qk(p):
            zeros = chain[:1] + st.pop('tie', [])
            del chain[:1]
            st[(p, 'p')] = _probs(st.pop((p, 0)), st.pop((p, 1)), zeros)

        def do_pv(p):
            cols = slice(p * PW, (p + 1) * PW)
            o = _dot(st.pop((p, 'p')), st.pop((p, 2)))
            o_ref[0:MEM, cols] = o[0:MEM]
            o_ref[2 * MEM:L, cols] = o[MEM:LM]

        def do_vpu(p):
            cols = slice(p * PW, (p + 1) * PW)
            lo = lax.broadcasted_iota(i32, (8, 128), 1) < 64
            row = lax.broadcasted_iota(i32, (8, 128), 0)
            q = st.pop((p, 'qv'))
            qa, qb = jnp.where(lo, q[:, 128:256], 0.0), jnp.where(lo, 0.0, q[:, 128:256])

            kk, vv = st.pop((p, 'kv', 1)), st.pop((p, 'kv', 2))
            sc = []
            for k in range(16):
                km = jnp.broadcast_to(kk[k:k + 1, 128:256], (8, 128))
                xa = jnp.sum(q[:, 0:128] * kk[k:k + 1, 0:128] + qa * km, axis=-1, keepdims=True)
                xb = jnp.sum(q[:, 256:384] * kk[k:k + 1, 256:384] + qb * km, axis=-1, keepdims=True)
                x = jnp.where(lo, xa, xb)
                sc.append(jnp.where(row >= k - MEM, x, -1000000000.0) if k > MEM else x)
            m = functools.reduce(jnp.maximum, sc)
            ev = [jnp.exp2(x - m) for x in sc]
            rr = 1.0 / functools.reduce(jnp.add, ev)
            z = _zero(m)
            ov = []
            for t in range(3):
                v = [vv[8 * b:8 * b + 8, 128 * t:128 * t + 128] + z for b in range(2)]
                ov.append(functools.reduce(
                    jnp.add, [ev[k] * v[k // 8][k % 8:k % 8 + 1] for k in range(16)]) * rr)
                z = _zero(ov[-1])
            o_ref[MEM:2 * MEM, cols] = jnp.concatenate(ov, axis=1)
            st['tie'] = [z[:, 0:2 * L]]

        def do_o(n):
            k0 = st.get('k', 0)
            k1 = st['k'] = k0 + n
            y = _dot(o_ref[:, k0 * 128:k1 * 128], _unpack(wo_ref[k0 * 64:k1 * 64, :]))
            st['y'] = y if 'y' not in st else st['y'] + y

        for s in range(NPB):
            proj(s, 0)
            if s >= 4:
                do_o(1)
            if s >= 1:
                do_qk(s - 1)
            proj(s, 1)
            if s >= 2:
                do_pv(s - 2)
            if s >= 1:
                do_vpu(s - 1)
            proj(s, 2)
            if s >= 4:
                do_o(1)
            for job in side[s]:
                job()
            assert st.get('k', 0) <= 3 * max(s - 2, 0)
        do_o(2)
        do_qk(NPB - 1)
        do_vpu(NPB - 1)
        do_o(4)
        do_pv(NPB - 2)
        do_o(7)
        assert st['k'] <= 3 * (NPB - 2)
        do_pv(NPB - 1)
        do_o(3 * (NPB - 1) - st['k'])
        do_o(3)
        return st['y']

    def layer_b(first):
        SPI = SPI1 if first else SPI2
        mem_ref[...] = mem0[...].astype(f32)
        yb_ref[1] = jnp.zeros((SEG, D), f32)
        if first:
            with jax.named_scope("wait_wo"):
                for j in range(NTR - 2, NTR):
                    cp_w(3, j).wait()
                    pack_wo(j)

        def body(j, carry):
            mem = mem_ref[...]
            for t in range(SPI):
                sg = j * SPI + t
                if not first and t % 2 == 0:
                    @pl.when(sg >= 4)
                    def _():
                        cp_rows(sg - 3, 2).start()

                sp = jnp.maximum(sg - 1, 0) if t == 0 else sg - 1
                sw = jnp.where(sg == 0, NSEG, sp) if t == 0 else sp
                sn = jnp.minimum(sg + 1, NSEG - 1) if t == SPI - 1 else sg + 1
                h = jnp.concatenate([xnb_ref[t % 2], mem], axis=0)
                chain = []
                side = [[] for _ in range(NPB)]
                for i in range(2):
                    side[1 + 2 * i].append(functools.partial(b_finish, first, sp, sw, (t + 1) % 2, i, chain))
                if not first:
                    for n in range(D // 128):
                        side[n].append(functools.partial(a_finish, sn, sg + 1, n))
                for i in range(4):
                    side[6 + 2 * i].append(functools.partial(a_norm, first, sn, (t + 1) % 2, i, chain))
                y = b_step(h, side, chain)
                mem = y[0:MEM]
                yb_ref[t % 2] = y[MEM:L]
            mem_ref[...] = mem
            return carry

        with jax.named_scope("b_loop"):
            lax.fori_loop(0, NSEG // SPI, body, 0)
        if not first:
            cp_rows(0, 1).start()
            cp_rows(NSEG - 3, 2).start()
        for i in range(2):
            b_finish(first, NSEG - 1, NSEG - 1, 1, i, [])

    for first in (True, False):
        kv_ref[...] = jnp.zeros(kv_ref.shape, f32)
        with jax.named_scope("a_p1"):
            a_phase1(first)
        with jax.named_scope("a_p2"):
            a_phase2(first)
        with jax.named_scope("layer_b"):
            layer_b(first)

    cp_rows(NSEG - 1, 1).start()
    cp_rows(0, NSEG).wait()


@jax.jit
def pallas_interleave_layers__linear_kernel_hedgehog__memory_aug_recurrent_mem_tr__prompt_kernel(
    A_x: jax.Array,
    A_wqkv: jax.Array,
    A_w_phi: jax.Array,
    A_wo: jax.Array,
    B_x: jax.Array,
    B_mem0: jax.Array,
    B_Wq: jax.Array,
    B_Wk: jax.Array,
    B_Wv: jax.Array,
    B_Wo: jax.Array,
    B_seg_len: jax.Array,
):
    del B_x, B_seg_len
    x = A_x.reshape(S, D)
    phi = A_w_phi.transpose(1, 2, 0)
    wqt = B_Wq.transpose(1, 2, 0).reshape(HD, D)
    wkt = B_Wk.transpose(1, 2, 0).reshape(HD, D)
    wvt = B_Wv.transpose(1, 2, 0).reshape(HD, D)
    wo = B_Wo.reshape(HD, D)
    hbm = pl.BlockSpec(memory_space=pl.ANY)
    out = pl.pallas_call(
        _kernel,
        out_shape=jax.ShapeDtypeStruct((S, D), bf16),
        in_specs=[hbm] * 9,
        out_specs=hbm,
        scratch_shapes=[
            pltpu.VMEM((S, D), bf16),
            pltpu.VMEM((3, D, D), bf16),
            pltpu.VMEM((DA, DA, HA), bf16),
            pltpu.VMEM((D, D), bf16),
            pltpu.VMEM((MEM, D), bf16),
            pltpu.VMEM((S + SEG, D), f32),
            pltpu.VMEM((S // 2, D), u32),
            pltpu.VMEM((2, SEG, D), f32),
            pltpu.VMEM((SEG, D), f32),
            pltpu.VMEM((SEG, D), f32),
            pltpu.VMEM((2, SEG, D), f32),
            pltpu.VMEM((S // 2, D), u32),
            pltpu.VMEM((3, GA, 80, D), u32),
            pltpu.VMEM((D // 2, D), u32),
            pltpu.VMEM((2, GA, 160, 256), f32),
            pltpu.VMEM((NCH, NPA, RA, TC), u32),
            pltpu.VMEM((NPA, RA + 8, 2 * RA), f32),
            pltpu.VMEM((NPA, (RA + 8) // 2, 2 * RA), u32),
            pltpu.VMEM((4, HD + 64, D), bf16),
            pltpu.VMEM((3, NPB + 2, D // 2, PW), u32),
            pltpu.VMEM(((HD + TRC) // 2, D), u32),
            pltpu.VMEM((MEM, D), f32),
            pltpu.VMEM((L, HD), f32),
            pltpu.SemaphoreType.DMA((20 + 4 * NTR,)),
        ],
        compiler_params=pltpu.CompilerParams(vmem_limit_bytes=120 * 1024 * 1024, disable_bounds_checks=True,
                                             disable_semaphore_checks=True),
    )(x, A_wqkv, phi, A_wo, B_mem0.reshape(MEM, D), wqt, wkt, wvt, wo)
    return out.reshape(1, S, D)
```

```python
import functools

import jax
import jax.numpy as jnp
from jax import lax
import jax.experimental.pallas as pl
import jax.experimental.pallas.tpu as pltpu

f32, bf16, u32, i32 = jnp.float32, jnp.bfloat16, jnp.uint32, jnp.int32

S, D = 2048, 640
HA, DA = 32, 20
NPA = HA // 2
RA = 2 * DA
GA = 4
TC = 256
NCH = S // TC
XCH = 256
HB, DB, MEM, SEG = 32, 192, 8, 32
HD = HB * DB
L = MEM + SEG
LM = L - 8
VBLK = (0, 192, 64, 256, 128, 320)
NPB = HB // 2
PW = 2 * DB
SCALE = DB ** -0.5 * 1.4426950408889634
TRC = 768
NTR = HD // TRC
NSEG = S // SEG
SPI1, SPI2 = 2, 4
assert NTR == NCH

_NN = (((1,), (0,)), ((), ()))
_NT = (((1,), (1,)), ((), ()))


def _dot(a, b):
    return lax.dot_general(a, b, _NN, precision=lax.Precision.DEFAULT, preferred_element_type=f32)


def _dot_nt(a, b):
    return lax.dot_general(a, b, _NT, precision=lax.Precision.DEFAULT, preferred_element_type=f32)


def _pack(x):
    return pltpu.bitcast(x.astype(bf16), u32)


def _unpack(x):
    return pltpu.bitcast(x, bf16)


def _ln(x):
    m = jnp.mean(x, axis=-1, keepdims=True)
    xc = x - m
    r = lax.rsqrt(jnp.mean(xc * xc, axis=-1, keepdims=True) + 1e-5)
    return x * r - m * r


def _ln_chained(x, chain):
    m = jnp.mean(x, axis=-1, keepdims=True)
    xc = x - m
    r = lax.rsqrt(jnp.mean(xc * xc, axis=-1, keepdims=True) + 1e-5)
    chain.append(jnp.minimum(r, 0.0))
    return x * r - m * r


def _fold(op, p):
    r = p[0:8]
    for j in range(1, 5):
        r = op(r, p[8 * j:8 * j + 8])
    r = op(r, pltpu.roll(r, 2, 0))
    return op(r, pltpu.roll(r, 4, 0))


def _tile5(r):
    return jnp.concatenate([r] * 5, axis=0)


def _phi(p):
    ep = jnp.exp(p - _tile5(_fold(jnp.maximum, p)))
    en = jnp.exp(_tile5(_fold(jnp.minimum, p)) - p)
    ep = ep * _tile5(1.0 / _fold(jnp.add, ep))
    en = en * _tile5(1.0 / _fold(jnp.add, en))
    return jnp.concatenate([ep, en], axis=0).astype(bf16)


def _split(k):
    lo = lax.broadcasted_iota(i32, (L, 128), 1) < 64
    z = jnp.zeros((L, 128), f32)
    mid = k[:, 128:256]
    outer = jnp.concatenate([k[:, 0:128], k[:, 256:384]], axis=0).astype(bf16)
    mid = jnp.concatenate([jnp.where(lo, mid, z), jnp.where(lo, z, mid)], axis=0).astype(bf16)
    return outer, mid


def _zero(x):
    return jnp.minimum(jnp.abs(x), 0.0)


def _probs(q, k, zeros):
    r = lax.broadcasted_iota(i32, (LM, 2 * L), 0)
    c = lax.broadcasted_iota(i32, (LM, 2 * L), 1)
    first = c < L
    so = _dot_nt(q[0], k[0])
    s = jnp.where(first, so[0:LM], so[LM:2 * LM]) + _dot_nt(q[1], k[1])
    s = s * SCALE
    if zeros:
        s = jnp.concatenate([functools.reduce(jnp.add, zeros, s[0:8]), s[8:LM]], axis=0)
    mask = (r < MEM) | (r + 8 >= jnp.where(first, c, c - L))
    s = jnp.where(mask, s, -1000000000.0)
    neg = jnp.full_like(s, -jnp.inf)
    ma = jnp.max(jnp.where(first, s, neg), axis=-1, keepdims=True)
    mb = jnp.max(jnp.where(first, neg, s), axis=-1, keepdims=True)
    e = jnp.exp2(s - jnp.where(first, ma, mb))
    z = jnp.zeros_like(e)
    sa = jnp.sum(jnp.where(first, e, z), axis=-1, keepdims=True)
    sb = jnp.sum(jnp.where(first, z, e), axis=-1, keepdims=True)
    return e * (1.0 / jnp.where(first, sa, sb))


def _kernel(x_hbm, wqkv_hbm, phi_hbm, woa_hbm, mem0_hbm, wqt_hbm, wkt_hbm, wvt_hbm, wo_hbm, out_hbm,
            xin_ref, wqkv, phi_ref, wo_a, mem0, x_ref, xna_ref, xnb_ref, xa_ref, xb_ref, yb_ref, oa_ref,
            wat_ref, wop_ref, lhs_ref, phiq_ref, kv_ref, kvm_ref, stage_ref, wb_ref, wo_ref, o_ref, sems):
    cp_phi = pltpu.make_async_copy(phi_hbm, phi_ref, sems.at[0])
    cp_mem0 = pltpu.make_async_copy(mem0_hbm, mem0, sems.at[1])
    cp_woa = pltpu.make_async_copy(woa_hbm, wo_a, sems.at[2])
    big = (wqt_hbm, wkt_hbm, wvt_hbm, wo_hbm)

    def cp_wqkv(n):
        return pltpu.make_async_copy(wqkv_hbm.at[:, pl.ds(pl.multiple_of(D * n, 128), D)], wqkv.at[n],
                                     sems.at[4 + n])

    def cp_x(j):
        rows = pl.ds(pl.multiple_of(j * XCH, XCH), XCH)
        return pltpu.make_async_copy(x_hbm.at[rows, :], xin_ref.at[rows, :], sems.at[12 + j])

    def cp_w(n, j):
        rows = pl.ds(pl.multiple_of(j * TRC, TRC), TRC)
        return pltpu.make_async_copy(big[n].at[rows, :], stage_ref.at[n, rows, :], sems.at[20 + n * NTR + j])

    def cp_rows(sg, nseg):
        rows = pl.ds(pl.multiple_of(sg * SEG, SEG), SEG * nseg)
        return pltpu.make_async_copy(xin_ref.at[rows, :], out_hbm.at[rows, :], sems.at[3])

    cp_phi.start()
    for n in range(3):
        cp_wqkv(n).start()
    for j in range(S // XCH):
        cp_x(j).start()
    cp_mem0.start()
    for j in range(NTR):
        if j == NTR - 1:
            cp_woa.start()
        for n in range(3):
            cp_w(n, j).start()
    for j in range(NTR):
        cp_w(3, j).start()

    def init_x(c, carry):
        with jax.named_scope("wait_x"):
            cp_x(c).wait()
        x = xin_ref[pl.ds(pl.multiple_of(c * XCH, XCH), XCH), :].astype(f32)
        x_ref[pl.ds(pl.multiple_of(c * XCH, XCH), XCH), :] = x
        xna_ref[pl.ds(pl.multiple_of(c * (XCH // 2), XCH // 2), XCH // 2), :] = _pack(_ln(x))
        return carry

    stage_ref[:, HD:HD + 64, :] = jnp.zeros((4, 64, D), bf16)

    with jax.named_scope("wait_phi"):
        cp_phi.wait()
    ecol = lax.broadcasted_iota(i32, (HA, D), 1) - DA * lax.broadcasted_iota(i32, (HA, D), 0)

    def scatter_phi(i, tp):
        for d in range(5):
            tp = tp + _dot(phi_ref[5 * i + d], jnp.where(ecol == 5 * i + d, 1.0, 0.0).astype(bf16))
        return tp

    tp = lax.fori_loop(0, DA // 5, scatter_phi, jnp.zeros((DA, D), f32))
    rep = jnp.where((lax.broadcasted_iota(i32, (RA, DA), 0) >> 1) == lax.broadcasted_iota(i32, (RA, DA), 1),
                    1.0, 0.0).astype(bf16)
    urep = _dot(rep, tp.astype(bf16))
    for g in range(GA):
        col = lax.broadcasted_iota(i32, (RA, 256), 1) + 128 * g
        par = lax.broadcasted_iota(i32, (RA, 256), 0) & 1
        for pp in range(4):
            lo = (8 * g + 2 * pp + par) * DA
            blk = jnp.where((col >= lo) & (col < lo + DA), urep[:, 128 * g:128 * g + 256], 0.0)
            lhs_ref[0, g, RA * pp:RA * pp + RA, :] = blk
        lhs_ref[1, g] = jnp.where(lax.broadcasted_iota(i32, (160, 256), 1) + 128 * g
                                  == lax.broadcasted_iota(i32, (160, 256), 0) + 160 * g, 1.0, 0.0)

    def prep(n, carry):
        with jax.named_scope("wait_wqkv"):
            cp_wqkv(n).wait()
        for g in range(GA):
            wat_ref[n, g] = _pack(_dot_nt(lhs_ref[n // 2, g].astype(bf16), wqkv[n, :, 128 * g:128 * g + 256]))
        return carry

    with jax.named_scope("prep"):
        lax.fori_loop(0, 3, prep, 0)
    with jax.named_scope("init_x"):
        lax.fori_loop(0, S // XCH, init_x, 0)
        cp_mem0.wait()

    def transpose_w(n, p):
        blocks = []
        for i in range(6):
            off = jnp.minimum(p * PW + jnp.where(n == 2, VBLK[i], 64 * i), HD)
            blocks.append(stage_ref[n, pl.ds(pl.multiple_of(off, 64), 64), :])
        wb_ref[n, p] = pltpu.bitcast(jnp.concatenate(blocks, axis=0).T, u32)

    def pack_wo(j):
        for i in range(12):
            src = pl.ds(pl.multiple_of(jnp.minimum(j * TRC + (i // 6) * PW + VBLK[i % 6], HD), 64), 64)
            wo_ref[pl.ds(pl.multiple_of(j * (TRC // 2) + 32 * i, 32), 32), :] = pltpu.bitcast(
                stage_ref[3, src, :], u32)

    def a_phase1(first):
        def body(c, carry):
            if first:
                ct = [jnp.where(c < lag, NTR, c - lag) for lag in (1, 1, 2)]

                @pl.when(c >= 2)
                def _():
                    cp_w(2, c - 2).wait()

                @pl.when(c >= 1)
                def _():
                    with jax.named_scope("wait_w"):
                        cp_w(0, c - 1).wait()
                        cp_w(1, c - 1).wait()

            xn = _unpack(xna_ref[pl.ds(pl.multiple_of(c * (TC // 2), TC // 2), TC // 2), :])
            ones = jnp.ones((8, TC), f32)
            pend = []
            for g in range(GA):
                pq = _dot_nt(_unpack(wat_ref[0, g]), xn)
                pk = _dot_nt(_unpack(wat_ref[1, g]), xn)
                vt = _dot_nt(_unpack(wat_ref[2, g]), xn)
                for pp in range(4):
                    p = 4 * g + pp
                    sl = slice(RA * pp, RA * pp + RA)
                    phiq_ref[c, p] = pltpu.bitcast(_phi(pq[sl]), u32)
                    vext = jnp.concatenate([vt[sl], ones], axis=0).astype(bf16)
                    pend.append((p, vext, _phi(pk[sl])))
                if first and g < 3:
                    transpose_w(g, 2 * ct[g])
                    transpose_w(g, 2 * ct[g] + 1)
            for p, vext, phik in pend:
                kv_ref[p] += _dot_nt(vext, phik)
            return carry

        lax.fori_loop(0, NCH, body, 0, unroll=1 if first else 2)

    def seg_rows(sg, off=0, n=SEG):
        return pl.ds(pl.multiple_of(sg * SEG + off, 8), n)

    def a_finish(sr, sw, n):
        cols = slice(128 * n, 128 * n + 128)
        y = _dot(_unpack(oa_ref[pl.ds(pl.multiple_of(sr * (SEG // 2), SEG // 2), SEG // 2), :]),
                 _unpack(wop_ref[:, cols]))
        x = x_ref[seg_rows(sr), cols] + y
        x_ref[seg_rows(sw), cols] = x
        xa_ref[:, cols] = x

    def a_norm(first, sg, i, chain):
        x = x_ref[seg_rows(sg, 8 * i, 8), :] if first else xa_ref[8 * i:8 * i + 8, :]
        xnb_ref[8 * i:8 * i + 8, :] = _ln_chained(x, chain)

    def a_phase2(first):
        if first:
            cp_w(2, NTR - 2).wait()
            cp_woa.wait()
        r = lax.broadcasted_iota(i32, (RA + 8, 2 * RA), 0)
        rb = jnp.where(((r >= DA) & (r < RA)) | (r >= RA + 4), 1, 0)
        same = rb == (lax.broadcasted_iota(i32, (RA + 8, 2 * RA), 1) & 1)
        for p in range(NPA):
            kvm_ref[p] = _pack(jnp.where(same, kv_ref[p], 0.0))

        def attend(c):
            top = lax.broadcasted_iota(i32, (8, TC), 0) < 4
            ot = []
            for p in range(NPA):
                ne = _dot(_unpack(kvm_ref[p]), _unpack(phiq_ref[c, p]))
                rc = 1.0 / (ne[RA:RA + 8] + 1e-6)
                sw = pltpu.roll(rc, 4, 0)
                ra, rb = jnp.where(top, rc, sw), jnp.where(top, sw, rc)
                ot.append(ne[0:RA] * jnp.concatenate([ra, ra, rc, rb, rb], axis=0))
            o = jnp.concatenate(ot, axis=0).T
            oa_ref[pl.ds(pl.multiple_of(c * (TC // 2), TC // 2), TC // 2), :] = _pack(o)

        if not first:
            for c in range(NCH):
                attend(c)
                if c == 2:
                    for n in range(D // 128):
                        a_finish(0, 0, n)
                    for i in range(4):
                        a_norm(False, 0, i, [])
            return

        wop_ref[...] = pltpu.bitcast(wo_a[...], u32)
        attend(0)

        def body(c, carry, last=False):
            @pl.when(c == 2)
            def _():
                for n in range(3):
                    cp_w(n, NTR - 1).wait()

            @pl.when(c >= 2)
            def _():
                cp_w(3, c - 2).wait()

            lhs = [_unpack(oa_ref[pl.ds(pl.multiple_of(c * (TC // 2) + r // 2, 64), 64), :])
                   for r in range(0, TC, 128)]
            if last:
                for i in range(4):
                    a_norm(True, 0, i, [])
            else:
                attend(c + 1)
            t = jnp.maximum(c - 2, 0)
            transpose_w(jnp.where(c < 2, 2, t // 2), jnp.where(c < 2, NPB - 4, NPB - 2) + c % 2)
            pack_wo(jnp.where(c < 2, NTR, t))
            for r in range(0, TC, 128):
                x_ref[pl.ds(pl.multiple_of(c * TC + r, 128), 128), :] += _dot(lhs[r // 128], _unpack(wop_ref[...]))
            return carry

        lax.fori_loop(0, NCH - 1, body, 0)
        body(jnp.int32(NCH - 1), 0, last=True)

    def b_finish(first, sr, sw, i, chain):
        x = x_ref[seg_rows(sr, 16 * i, 16), :] + yb_ref[16 * i:16 * i + 16, :]
        if first:
            x_ref[seg_rows(sw, 16 * i, 16), :] = x
            xb_ref[16 * i:16 * i + 16, :] = x
            xn = [_ln_chained(xb_ref[16 * i + k:16 * i + k + 8, :], chain) for k in (0, 8)]
            xna_ref[pl.ds(pl.multiple_of(sr * (SEG // 2) + 8 * i, 8), 8), :] = _pack(
                jnp.concatenate(xn, axis=0))
        else:
            xin_ref[pl.ds(pl.multiple_of(sr * SEG + 16 * i, 16), 16), :] = x.astype(bf16)

    def b_step(h, side, chain):
        st = {}

        def proj(p, which):
            if p == 0 and which == 0:
                y = _dot(h[:, 0:128], _unpack(wb_ref[0, 0, 0:64, :]))
                for k in range(1, D // 128):
                    y = y + _dot(h[:, 128 * k:128 * k + 128], _unpack(wb_ref[0, 0, 64 * k:64 * k + 64, :]))
            else:
                y = _dot(h, _unpack(wb_ref[which, p]))
            if which == 0:
                st[(p, 'qv')] = y[0:8] * SCALE
                y = jnp.concatenate([y[SEG:L], y[8:SEG]], axis=0)
                st[(p, 0)] = (jnp.concatenate([y[:, 0:128], y[:, 256:384]], axis=0).astype(bf16), y[:, 128:256])
                return
            y = jnp.concatenate([y[SEG:L], y[0:SEG]], axis=0)
            st[(p, 'kv', which)] = y[0:16]
            if which == 1:
                st[(p, 1)] = _split(y)
            else:
                lo = (lax.broadcasted_iota(i32, (L, PW), 1) & 64) == 0
                st[(p, 2)] = jnp.concatenate([jnp.where(lo, y, 0.0), jnp.where(lo, 0.0, y)], axis=0).astype(bf16)

        def do_qk(p):
            zeros = chain[:1] + st.pop('tie', [])
            del chain[:1]
            st[(p, 'p')] = _probs(st.pop((p, 0)), st.pop((p, 1)), zeros)

        def do_pv(p):
            cols = slice(p * PW, (p + 1) * PW)
            o = _dot(st.pop((p, 'p')), st.pop((p, 2)))
            o_ref[0:MEM, cols] = o[0:MEM]
            o_ref[2 * MEM:L, cols] = o[MEM:LM]

        def do_vpu(p):
            cols = slice(p * PW, (p + 1) * PW)
            lo = lax.broadcasted_iota(i32, (8, 128), 1) < 64
            row = lax.broadcasted_iota(i32, (8, 128), 0)
            q = st.pop((p, 'qv'))
            qa, qb = jnp.where(lo, q[:, 128:256], 0.0), jnp.where(lo, 0.0, q[:, 128:256])

            kk, vv = st.pop((p, 'kv', 1)), st.pop((p, 'kv', 2))
            sc = []
            for k in range(16):
                km = jnp.broadcast_to(kk[k:k + 1, 128:256], (8, 128))
                xa = jnp.sum(q[:, 0:128] * kk[k:k + 1, 0:128] + qa * km, axis=-1, keepdims=True)
                xb = jnp.sum(q[:, 256:384] * kk[k:k + 1, 256:384] + qb * km, axis=-1, keepdims=True)
                x = jnp.where(lo, xa, xb)
                sc.append(jnp.where(row >= k - MEM, x, -1000000000.0) if k > MEM else x)
            m = functools.reduce(jnp.maximum, sc)
            ev = [jnp.exp2(x - m) for x in sc]
            rr = 1.0 / functools.reduce(jnp.add, ev)
            z = _zero(m)
            ov = []
            for t in range(3):
                v = [vv[8 * b:8 * b + 8, 128 * t:128 * t + 128] + z for b in range(2)]
                ov.append(functools.reduce(
                    jnp.add, [ev[k] * v[k // 8][k % 8:k % 8 + 1] for k in range(16)]) * rr)
                z = _zero(ov[-1])
            o_ref[MEM:2 * MEM, cols] = jnp.concatenate(ov, axis=1)
            st['tie'] = [z[:, 0:2 * L]]

        def do_o(n):
            k0 = st.get('k', 0)
            k1 = st['k'] = k0 + n
            y = _dot(o_ref[:, k0 * 128:k1 * 128], _unpack(wo_ref[k0 * 64:k1 * 64, :]))
            st['y'] = y if 'y' not in st else st['y'] + y

        for s in range(NPB):
            proj(s, 0)
            if s >= 4:
                do_o(1)
            if s >= 1:
                do_qk(s - 1)
            proj(s, 1)
            if s >= 2:
                do_pv(s - 2)
            if s >= 1:
                do_vpu(s - 1)
            proj(s, 2)
            if s >= 4:
                do_o(1)
            for job in side[s]:
                job()
            assert st.get('k', 0) <= 3 * max(s - 2, 0)
        do_o(2)
        do_qk(NPB - 1)
        do_vpu(NPB - 1)
        do_o(4)
        do_pv(NPB - 2)
        do_o(7)
        assert st['k'] <= 3 * (NPB - 2)
        do_pv(NPB - 1)
        do_o(3 * (NPB - 1) - st['k'])
        do_o(3)
        return st['y']

    def layer_b(first):
        yb_ref[...] = jnp.zeros((SEG, D), f32)
        if first:
            with jax.named_scope("wait_wo"):
                for j in range(NTR - 2, NTR):
                    cp_w(3, j).wait()
                    pack_wo(j)

        def body(sg, mem):
            if not first:
                @pl.when(sg >= 2)
                def _():
                    cp_rows(sg - 2, 1).start()

            sp = jnp.maximum(sg - 1, 0)
            sw = jnp.where(sg == 0, NSEG, sp)
            sn = jnp.minimum(sg + 1, NSEG - 1)
            h = jnp.concatenate([xnb_ref[...], mem], axis=0)
            chain = []
            side = [[] for _ in range(NPB)]
            for i in range(2):
                side[1 + 2 * i].append(functools.partial(b_finish, first, sp, sw, i, chain))
            if not first:
                for n in range(D // 128):
                    side[n].append(functools.partial(a_finish, sn, sg + 1, n))
            for i in range(4):
                side[6 + 2 * i].append(functools.partial(a_norm, first, sn, i, chain))
            y = b_step(h, side, chain)
            yb_ref[...] = y[MEM:L]
            return y[0:MEM]

        with jax.named_scope("b_loop"):
            lax.fori_loop(0, NSEG, body, mem0[...].astype(f32), unroll=SPI1 if first else SPI2)
        if not first:
            cp_rows(NSEG - 2, 1).start()
        for i in range(2):
            b_finish(first, NSEG - 1, NSEG - 1, i, [])

    for first in (True, False):
        kv_ref[...] = jnp.zeros(kv_ref.shape, f32)
        with jax.named_scope("a_p1"):
            a_phase1(first)
        with jax.named_scope("a_p2"):
            a_phase2(first)
        with jax.named_scope("layer_b"):
            layer_b(first)

    cp_rows(NSEG - 1, 1).start()
    cp_rows(0, NSEG).wait()


@jax.jit
def pallas_interleave_layers__linear_kernel_hedgehog__memory_aug_recurrent_mem_tr__prompt_kernel(
    A_x: jax.Array,
    A_wqkv: jax.Array,
    A_w_phi: jax.Array,
    A_wo: jax.Array,
    B_x: jax.Array,
    B_mem0: jax.Array,
    B_Wq: jax.Array,
    B_Wk: jax.Array,
    B_Wv: jax.Array,
    B_Wo: jax.Array,
    B_seg_len: jax.Array,
):
    del B_x, B_seg_len
    x = A_x.reshape(S, D)
    phi = A_w_phi.transpose(1, 2, 0)
    wqt = B_Wq.transpose(1, 2, 0).reshape(HD, D)
    wkt = B_Wk.transpose(1, 2, 0).reshape(HD, D)
    wvt = B_Wv.transpose(1, 2, 0).reshape(HD, D)
    wo = B_Wo.reshape(HD, D)
    hbm = pl.BlockSpec(memory_space=pl.ANY)
    out = pl.pallas_call(
        _kernel,
        out_shape=jax.ShapeDtypeStruct((S, D), bf16),
        in_specs=[hbm] * 9,
        out_specs=hbm,
        scratch_shapes=[
            pltpu.VMEM((S, D), bf16),
            pltpu.VMEM((3, D, D), bf16),
            pltpu.VMEM((DA, DA, HA), bf16),
            pltpu.VMEM((D, D), bf16),
            pltpu.VMEM((MEM, D), bf16),
            pltpu.VMEM((S + SEG, D), f32),
            pltpu.VMEM((S // 2, D), u32),
            pltpu.VMEM((SEG, D), f32),
            pltpu.VMEM((SEG, D), f32),
            pltpu.VMEM((SEG, D), f32),
            pltpu.VMEM((SEG, D), f32),
            pltpu.VMEM((S // 2, D), u32),
            pltpu.VMEM((3, GA, 80, D), u32),
            pltpu.VMEM((D // 2, D), u32),
            pltpu.VMEM((2, GA, 160, 256), f32),
            pltpu.VMEM((NCH, NPA, RA, TC), u32),
            pltpu.VMEM((NPA, RA + 8, 2 * RA), f32),
            pltpu.VMEM((NPA, (RA + 8) // 2, 2 * RA), u32),
            pltpu.VMEM((4, HD + 64, D), bf16),
            pltpu.VMEM((3, NPB + 2, D // 2, PW), u32),
            pltpu.VMEM(((HD + TRC) // 2, D), u32),
            pltpu.VMEM((L, HD), f32),
            pltpu.SemaphoreType.DMA((20 + 4 * NTR,)),
        ],
        compiler_params=pltpu.CompilerParams(vmem_limit_bytes=120 * 1024 * 1024, disable_bounds_checks=True,
                                             disable_semaphore_checks=True),
    )(x, A_wqkv, phi, A_wo, B_mem0.reshape(MEM, D), wqt, wkt, wvt, wo)
    return out.reshape(1, S, D)
```

```python
import functools

import jax
import jax.numpy as jnp
from jax import lax
import jax.experimental.pallas as pl
import jax.experimental.pallas.tpu as pltpu

f32, bf16, u32, i32 = jnp.float32, jnp.bfloat16, jnp.uint32, jnp.int32

S, D = 2048, 640
HA, DA = 32, 20
NPA = HA // 2
RA = 2 * DA
GA = 4
TC = 256
NCH = S // TC
XCH = 512
HB, DB, MEM, SEG = 32, 192, 8, 32
HD = HB * DB
L = MEM + SEG
LM = L - 8
VBLK = (0, 192, 64, 256, 128, 320)
NPB = HB // 2
PW = 2 * DB
SCALE = DB ** -0.5 * 1.4426950408889634
TRC = 768
NTR = HD // TRC
NSEG = S // SEG
assert NTR == NCH

_NN = (((1,), (0,)), ((), ()))
_NT = (((1,), (1,)), ((), ()))


def _dot(a, b):
    return lax.dot_general(a, b, _NN, precision=lax.Precision.DEFAULT, preferred_element_type=f32)


def _dot_nt(a, b):
    return lax.dot_general(a, b, _NT, precision=lax.Precision.DEFAULT, preferred_element_type=f32)


def _pack(x):
    return pltpu.bitcast(x.astype(bf16), u32)


def _unpack(x):
    return pltpu.bitcast(x, bf16)


def _ln(x):
    m = jnp.mean(x, axis=-1, keepdims=True)
    xc = x - m
    r = lax.rsqrt(jnp.mean(xc * xc, axis=-1, keepdims=True) + 1e-5)
    return x * r - m * r


def _ln_chained(x, chain):
    m = jnp.mean(x, axis=-1, keepdims=True)
    xc = x - m
    r = lax.rsqrt(jnp.mean(xc * xc, axis=-1, keepdims=True) + 1e-5)
    chain.append(jnp.minimum(r, 0.0))
    return x * r - m * r


def _fold(op, p):
    r = p[0:8]
    for j in range(1, 5):
        r = op(r, p[8 * j:8 * j + 8])
    r = op(r, pltpu.roll(r, 2, 0))
    return op(r, pltpu.roll(r, 4, 0))


def _tile5(r):
    return jnp.concatenate([r] * 5, axis=0)


def _phi(p):
    ep = jnp.exp(p - _tile5(_fold(jnp.maximum, p)))
    en = jnp.exp(_tile5(_fold(jnp.minimum, p)) - p)
    ep = ep * _tile5(1.0 / _fold(jnp.add, ep))
    en = en * _tile5(1.0 / _fold(jnp.add, en))
    return jnp.concatenate([ep, en], axis=0).astype(bf16)


def _split(k):
    lo = lax.broadcasted_iota(i32, (L, 128), 1) < 64
    z = jnp.zeros((L, 128), f32)
    mid = k[:, 128:256]
    outer = jnp.concatenate([k[:, 0:128], k[:, 256:384]], axis=0).astype(bf16)
    mid = jnp.concatenate([jnp.where(lo, mid, z), jnp.where(lo, z, mid)], axis=0).astype(bf16)
    return outer, mid


def _zero(x):
    return jnp.minimum(jnp.abs(x), 0.0)


def _probs(q, k, zeros):
    r = lax.broadcasted_iota(i32, (LM, 2 * L), 0)
    c = lax.broadcasted_iota(i32, (LM, 2 * L), 1)
    first = c < L
    so = _dot_nt(q[0], k[0])
    s = jnp.where(first, so[0:LM], so[LM:2 * LM]) + _dot_nt(q[1], k[1])
    s = s * SCALE
    if zeros:
        s = jnp.concatenate([functools.reduce(jnp.add, zeros, s[0:8]), s[8:LM]], axis=0)
    mask = (r < MEM) | (r + 8 >= jnp.where(first, c, c - L))
    s = jnp.where(mask, s, -1000000000.0)
    neg = jnp.full_like(s, -jnp.inf)
    ma = jnp.max(jnp.where(first, s, neg), axis=-1, keepdims=True)
    mb = jnp.max(jnp.where(first, neg, s), axis=-1, keepdims=True)
    e = jnp.exp2(s - jnp.where(first, ma, mb))
    z = jnp.zeros_like(e)
    sa = jnp.sum(jnp.where(first, e, z), axis=-1, keepdims=True)
    sb = jnp.sum(jnp.where(first, z, e), axis=-1, keepdims=True)
    return e * (1.0 / jnp.where(first, sa, sb))


def _kernel(x_hbm, wqkv_hbm, phi_hbm, woa_hbm, mem0_hbm, wqt_hbm, wkt_hbm, wvt_hbm, wo_hbm, out_hbm,
            xin_ref, wqkv, phi_ref, wo_a, mem0, x_ref, xna_ref, xnb_ref, xa_ref, xb_ref, yb_ref, oa_ref,
            wat_ref, wop_ref, lhs_ref, phiq_ref, kv_ref, kvm_ref, stage_ref, wb_ref, wo_ref, o_ref, sems):
    cp_phi = pltpu.make_async_copy(phi_hbm, phi_ref, sems.at[0])
    cp_mem0 = pltpu.make_async_copy(mem0_hbm, mem0, sems.at[1])
    cp_woa = pltpu.make_async_copy(woa_hbm, wo_a, sems.at[2])
    big = (wqt_hbm, wkt_hbm, wvt_hbm, wo_hbm)

    def cp_wqkv(n):
        return pltpu.make_async_copy(wqkv_hbm.at[:, pl.ds(pl.multiple_of(D * n, 128), D)], wqkv.at[n],
                                     sems.at[4 + n])

    def cp_x(j):
        rows = pl.ds(pl.multiple_of(j * XCH, XCH), XCH)
        return pltpu.make_async_copy(x_hbm.at[rows, :], xin_ref.at[rows, :], sems.at[12 + j])

    def cp_w(n, j):
        rows = pl.ds(pl.multiple_of(j * TRC, TRC), TRC)
        return pltpu.make_async_copy(big[n].at[rows, :], stage_ref.at[n, rows, :], sems.at[20 + n * NTR + j])

    def cp_rows(sg, nseg):
        rows = pl.ds(pl.multiple_of(sg * SEG, SEG), SEG * nseg)
        return pltpu.make_async_copy(xin_ref.at[rows, :], out_hbm.at[rows, :], sems.at[3])

    cp_phi.start()
    for n in range(3):
        cp_wqkv(n).start()
    for j in range(S // XCH):
        cp_x(j).start()
    cp_mem0.start()
    for j in range(NTR):
        if j == NTR - 1:
            cp_woa.start()
        for n in range(3):
            cp_w(n, j).start()
    for j in range(NTR):
        cp_w(3, j).start()

    def init_x(c, carry):
        with jax.named_scope("wait_x"):
            cp_x(c).wait()
        x = xin_ref[pl.ds(pl.multiple_of(c * XCH, XCH), XCH), :].astype(f32)
        xna_ref[pl.ds(pl.multiple_of(c * (XCH // 2), XCH // 2), XCH // 2), :] = _pack(_ln(x))
        return carry

    stage_ref[:, HD:HD + 64, :] = jnp.zeros((4, 64, D), bf16)

    with jax.named_scope("wait_phi"):
        cp_phi.wait()
    ecol = lax.broadcasted_iota(i32, (HA, D), 1) - DA * lax.broadcasted_iota(i32, (HA, D), 0)

    def scatter_phi(i, tp):
        for d in range(5):
            tp = tp + _dot(phi_ref[5 * i + d], jnp.where(ecol == 5 * i + d, 1.0, 0.0).astype(bf16))
        return tp

    tp = lax.fori_loop(0, DA // 5, scatter_phi, jnp.zeros((DA, D), f32))
    rep = jnp.where((lax.broadcasted_iota(i32, (RA, DA), 0) >> 1) == lax.broadcasted_iota(i32, (RA, DA), 1),
                    1.0, 0.0).astype(bf16)
    urep = _dot(rep, tp.astype(bf16))
    for g in range(GA):
        col = lax.broadcasted_iota(i32, (RA, 256), 1) + 128 * g
        par = lax.broadcasted_iota(i32, (RA, 256), 0) & 1
        for pp in range(4):
            lo = (8 * g + 2 * pp + par) * DA
            blk = jnp.where((col >= lo) & (col < lo + DA), urep[:, 128 * g:128 * g + 256], 0.0)
            lhs_ref[0, g, RA * pp:RA * pp + RA, :] = blk
        lhs_ref[1, g] = jnp.where(lax.broadcasted_iota(i32, (160, 256), 1) + 128 * g
                                  == lax.broadcasted_iota(i32, (160, 256), 0) + 160 * g, 1.0, 0.0)

    def prep(n, carry):
        with jax.named_scope("wait_wqkv"):
            cp_wqkv(n).wait()
        for g in range(GA):
            wat_ref[n, g] = _pack(_dot_nt(lhs_ref[n // 2, g].astype(bf16), wqkv[n, :, 128 * g:128 * g + 256]))
        return carry

    with jax.named_scope("prep"):
        lax.fori_loop(0, 3, prep, 0)

    def transpose_w(n, p):
        blocks = []
        for i in range(6):
            off = jnp.minimum(p * PW + jnp.where(n == 2, VBLK[i], 64 * i), HD)
            blocks.append(stage_ref[n, pl.ds(pl.multiple_of(off, 64), 64), :])
        wb_ref[n, p] = pltpu.bitcast(jnp.concatenate(blocks, axis=0).T, u32)

    def pack_wo(j):
        for i in range(12):
            src = pl.ds(pl.multiple_of(jnp.minimum(j * TRC + (i // 6) * PW + VBLK[i % 6], HD), 64), 64)
            wo_ref[pl.ds(pl.multiple_of(j * (TRC // 2) + 32 * i, 32), 32), :] = pltpu.bitcast(
                stage_ref[3, src, :], u32)

    def a_phase1(first):
        def body(c, carry):
            if first:
                ct = [jnp.where(c < lag, NTR, c - lag) for lag in (1, 1, 2)]

                @pl.when(c >= 2)
                def _():
                    cp_w(2, c - 2).wait()

                @pl.when(c >= 1)
                def _():
                    with jax.named_scope("wait_w"):
                        cp_w(0, c - 1).wait()
                        cp_w(1, c - 1).wait()

            xn = _unpack(xna_ref[pl.ds(pl.multiple_of(c * (TC // 2), TC // 2), TC // 2), :])
            ones = jnp.ones((8, TC), f32)
            pend = []
            for g in range(GA):
                pq = _dot_nt(_unpack(wat_ref[0, g]), xn)
                pk = _dot_nt(_unpack(wat_ref[1, g]), xn)
                vt = _dot_nt(_unpack(wat_ref[2, g]), xn)
                for pp in range(4):
                    p = 4 * g + pp
                    sl = slice(RA * pp, RA * pp + RA)
                    phiq_ref[c, p] = pltpu.bitcast(_phi(pq[sl]), u32)
                    vext = jnp.concatenate([vt[sl], ones], axis=0).astype(bf16)
                    pend.append((p, vext, _phi(pk[sl])))
                if first and g < 3:
                    transpose_w(g, 2 * ct[g])
                    transpose_w(g, 2 * ct[g] + 1)
            for p, vext, phik in pend:
                kv_ref[p] += _dot_nt(vext, phik)
            return carry

        if not first:
            lax.fori_loop(0, NCH, body, 0, unroll=2)
            return

        def part(q, carry):
            init_x(q, 0)
            lax.fori_loop(2 * q, 2 * q + 2, body, 0)
            return carry

        lax.fori_loop(0, S // XCH, part, 0)

    def seg_rows(sg, off=0, n=SEG):
        return pl.ds(pl.multiple_of(sg * SEG + off, 8), n)

    def a_finish(sr, sw, n):
        cols = slice(128 * n, 128 * n + 128)
        y = _dot(_unpack(oa_ref[pl.ds(pl.multiple_of(sr * (SEG // 2), SEG // 2), SEG // 2), :]),
                 _unpack(wop_ref[:, cols]))
        x = x_ref[seg_rows(sr), cols] + y
        x_ref[seg_rows(sw), cols] = x
        xa_ref[:, cols] = x

    def a_norm(first, sg, i, chain):
        x = x_ref[seg_rows(sg, 8 * i, 8), :] if first else xa_ref[8 * i:8 * i + 8, :]
        xnb_ref[8 * i:8 * i + 8, :] = _ln_chained(x, chain)

    def a_phase2(first):
        r = lax.broadcasted_iota(i32, (RA + 8, 2 * RA), 0)
        rb = jnp.where(((r >= DA) & (r < RA)) | (r >= RA + 4), 1, 0)
        same = rb == (lax.broadcasted_iota(i32, (RA + 8, 2 * RA), 1) & 1)
        for p in range(NPA):
            kvm_ref[p] = _pack(jnp.where(same, kv_ref[p], 0.0))

        def attend(c):
            top = lax.broadcasted_iota(i32, (8, TC), 0) < 4
            ot = []
            for p in range(NPA):
                ne = _dot(_unpack(kvm_ref[p]), _unpack(phiq_ref[c, p]))
                rc = 1.0 / (ne[RA:RA + 8] + 1e-6)
                sw = pltpu.roll(rc, 4, 0)
                ra, rb = jnp.where(top, rc, sw), jnp.where(top, sw, rc)
                ot.append(ne[0:RA] * jnp.concatenate([ra, ra, rc, rb, rb], axis=0))
            o = jnp.concatenate(ot, axis=0).T
            oa_ref[pl.ds(pl.multiple_of(c * (TC // 2), TC // 2), TC // 2), :] = _pack(o)

        if not first:
            wop_ref[...] = pltpu.bitcast(wo_a[...], u32)
            for c in range(NCH):
                attend(c)
                if c == 2:
                    for n in range(D // 128):
                        a_finish(0, 0, n)
                    for i in range(4):
                        a_norm(False, 0, i, [])
            return

        attend(0)
        cp_mem0.wait()
        cp_w(2, NTR - 2).wait()
        cp_woa.wait()

        def body(c, carry, last=False):
            @pl.when(c == 2)
            def _():
                for n in range(3):
                    cp_w(n, NTR - 1).wait()

            @pl.when(c >= 2)
            def _():
                cp_w(3, c - 2).wait()

            if last:
                cp_w(3, NTR - 2).wait()
            lhs = [_unpack(oa_ref[pl.ds(pl.multiple_of(c * (TC // 2) + r // 2, 64), 64), :])
                   for r in range(0, TC, 128)]
            if last:
                pack_wo(NTR - 2)
                for i in range(4):
                    a_norm(True, 0, i, [])
            else:
                attend(c + 1)
            t = jnp.maximum(c - 2, 0)
            transpose_w(jnp.where(c < 2, 2, t // 2), jnp.where(c < 2, NPB - 4, NPB - 2) + c % 2)
            pack_wo(jnp.where(c < 2, NTR, t))
            for r in range(0, TC, 128):
                rows = pl.ds(pl.multiple_of(c * TC + r, 128), 128)
                x_ref[rows, :] = xin_ref[rows, :].astype(f32) + _dot(lhs[r // 128], wo_a[...])
            return carry

        lax.fori_loop(0, NCH - 1, body, 0)
        body(jnp.int32(NCH - 1), 0, last=True)

    def b_finish(first, sr, sw, i, chain):
        x = x_ref[seg_rows(sr, 16 * i, 16), :] + yb_ref[16 * i:16 * i + 16, :]
        if first:
            x_ref[seg_rows(sw, 16 * i, 16), :] = x
            xb_ref[16 * i:16 * i + 16, :] = x
            xn = [_ln_chained(xb_ref[16 * i + k:16 * i + k + 8, :], chain) for k in (0, 8)]
            xna_ref[pl.ds(pl.multiple_of(sr * (SEG // 2) + 8 * i, 8), 8), :] = _pack(
                jnp.concatenate(xn, axis=0))
        else:
            xin_ref[pl.ds(pl.multiple_of(sr * SEG + 16 * i, 16), 16), :] = x.astype(bf16)

    def b_step(h, side, chain):
        st = {}

        def proj(p, which):
            if p == 0 and which == 0:
                y = _dot(h[:, 0:128], _unpack(wb_ref[0, 0, 0:64, :]))
                for k in range(1, D // 128):
                    y = y + _dot(h[:, 128 * k:128 * k + 128], _unpack(wb_ref[0, 0, 64 * k:64 * k + 64, :]))
            else:
                y = _dot(h, _unpack(wb_ref[which, p]))
            if which == 0:
                st[(p, 'qv')] = y[0:8] * SCALE
                y = jnp.concatenate([y[SEG:L], y[8:SEG]], axis=0)
                st[(p, 0)] = (jnp.concatenate([y[:, 0:128], y[:, 256:384]], axis=0).astype(bf16), y[:, 128:256])
                return
            y = jnp.concatenate([y[SEG:L], y[0:SEG]], axis=0)
            st[(p, 'kv', which)] = y[0:16]
            if which == 1:
                st[(p, 1)] = _split(y)
            else:
                lo = (lax.broadcasted_iota(i32, (L, PW), 1) & 64) == 0
                st[(p, 2)] = jnp.concatenate([jnp.where(lo, y, 0.0), jnp.where(lo, 0.0, y)], axis=0).astype(bf16)

        def do_qk(p):
            zeros = chain[:1] + st.pop('tie', [])
            del chain[:1]
            st[(p, 'p')] = _probs(st.pop((p, 0)), st.pop((p, 1)), zeros)

        def do_pv(p):
            cols = slice(p * PW, (p + 1) * PW)
            o = _dot(st.pop((p, 'p')), st.pop((p, 2)))
            o_ref[0:MEM, cols] = o[0:MEM]
            o_ref[2 * MEM:L, cols] = o[MEM:LM]

        def do_vpu(p):
            cols = slice(p * PW, (p + 1) * PW)
            lo = lax.broadcasted_iota(i32, (8, 128), 1) < 64
            row = lax.broadcasted_iota(i32, (8, 128), 0)
            q = st.pop((p, 'qv'))
            qa, qb = jnp.where(lo, q[:, 128:256], 0.0), jnp.where(lo, 0.0, q[:, 128:256])

            kk, vv = st.pop((p, 'kv', 1)), st.pop((p, 'kv', 2))
            sc = []
            for k in range(16):
                km = jnp.broadcast_to(kk[k:k + 1, 128:256], (8, 128))
                xa = jnp.sum(q[:, 0:128] * kk[k:k + 1, 0:128] + qa * km, axis=-1, keepdims=True)
                xb = jnp.sum(q[:, 256:384] * kk[k:k + 1, 256:384] + qb * km, axis=-1, keepdims=True)
                x = jnp.where(lo, xa, xb)
                sc.append(jnp.where(row >= k - MEM, x, -1000000000.0) if k > MEM else x)
            m = functools.reduce(jnp.maximum, sc)
            ev = [jnp.exp2(x - m) for x in sc]
            rr = 1.0 / functools.reduce(jnp.add, ev)
            z = _zero(m)
            ov = []
            for t in range(3):
                v = [vv[8 * b:8 * b + 8, 128 * t:128 * t + 128] + z for b in range(2)]
                ov.append(functools.reduce(
                    jnp.add, [ev[k] * v[k // 8][k % 8:k % 8 + 1] for k in range(16)]) * rr)
                z = _zero(ov[-1])
            o_ref[MEM:2 * MEM, cols] = jnp.concatenate(ov, axis=1)
            st['tie'] = [z[:, 0:2 * L]]

        def do_o(n):
            k0 = st.get('k', 0)
            k1 = st['k'] = k0 + n
            y = _dot(o_ref[:, k0 * 128:k1 * 128], _unpack(wo_ref[k0 * 64:k1 * 64, :]))
            st['y'] = y if 'y' not in st else st['y'] + y

        for s in range(NPB):
            proj(s, 0)
            if s >= 4:
                do_o(1)
            if s >= 1:
                do_qk(s - 1)
            proj(s, 1)
            if s >= 2:
                do_pv(s - 2)
            if s >= 1:
                do_vpu(s - 1)
            proj(s, 2)
            if s >= 4:
                do_o(1)
            for job in side[s]:
                job()
            assert st.get('k', 0) <= 3 * max(s - 2, 0)
        do_o(2)
        do_qk(NPB - 1)
        do_vpu(NPB - 1)
        do_o(4)
        do_pv(NPB - 2)
        do_o(7)
        assert st['k'] <= 3 * (NPB - 2)
        do_pv(NPB - 1)
        do_o(3 * (NPB - 1) - st['k'])
        do_o(3)
        return st['y']

    def layer_b(first):
        yb_ref[...] = jnp.zeros((SEG, D), f32)
        if first:
            with jax.named_scope("wait_wo"):
                cp_w(3, NTR - 1).wait()
            pack_wo(NTR - 1)

        def body(sg, mem):
            if not first:
                @pl.when(sg >= 2)
                def _():
                    cp_rows(sg - 2, 1).start()

            sp = jnp.maximum(sg - 1, 0)
            sw = jnp.where(sg == 0, NSEG, sp)
            sn = jnp.minimum(sg + 1, NSEG - 1)
            h = jnp.concatenate([xnb_ref[...], mem], axis=0)
            chain = []
            side = [[] for _ in range(NPB)]
            for i in range(2):
                side[1 + 2 * i].append(functools.partial(b_finish, first, sp, sw, i, chain))
            if not first:
                for n in range(D // 128):
                    side[n].append(functools.partial(a_finish, sn, sg + 1, n))
            for i in range(4):
                side[6 + 2 * i].append(functools.partial(a_norm, first, sn, i, chain))
            y = b_step(h, side, chain)
            yb_ref[...] = y[MEM:L]
            return y[0:MEM]

        with jax.named_scope("b_loop"):
            mem = mem0[...].astype(f32)
            if first:
                mem = lax.fori_loop(0, 4, body, mem)
                lax.fori_loop(4, NSEG, body, mem, unroll=3)
            else:
                lax.fori_loop(0, NSEG, body, mem, unroll=4)
        if not first:
            cp_rows(NSEG - 2, 1).start()
        for i in range(2):
            b_finish(first, NSEG - 1, NSEG - 1, i, [])

    for first in (True, False):
        kv_ref[...] = jnp.zeros(kv_ref.shape, f32)
        with jax.named_scope("a_p1"):
            a_phase1(first)
        with jax.named_scope("a_p2"):
            a_phase2(first)
        with jax.named_scope("layer_b"):
            layer_b(first)

    cp_rows(NSEG - 1, 1).start()
    cp_rows(0, NSEG).wait()


@jax.jit
def pallas_interleave_layers__linear_kernel_hedgehog__memory_aug_recurrent_mem_tr__prompt_kernel(
    A_x: jax.Array,
    A_wqkv: jax.Array,
    A_w_phi: jax.Array,
    A_wo: jax.Array,
    B_x: jax.Array,
    B_mem0: jax.Array,
    B_Wq: jax.Array,
    B_Wk: jax.Array,
    B_Wv: jax.Array,
    B_Wo: jax.Array,
    B_seg_len: jax.Array,
):
    del B_x, B_seg_len
    x = A_x.reshape(S, D)
    phi = A_w_phi.transpose(1, 2, 0)
    wqt = B_Wq.transpose(1, 2, 0).reshape(HD, D)
    wkt = B_Wk.transpose(1, 2, 0).reshape(HD, D)
    wvt = B_Wv.transpose(1, 2, 0).reshape(HD, D)
    wo = B_Wo.reshape(HD, D)
    hbm = pl.BlockSpec(memory_space=pl.ANY)
    out = pl.pallas_call(
        _kernel,
        out_shape=jax.ShapeDtypeStruct((S, D), bf16),
        in_specs=[hbm] * 9,
        out_specs=hbm,
        scratch_shapes=[
            pltpu.VMEM((S, D), bf16),
            pltpu.VMEM((3, D, D), bf16),
            pltpu.VMEM((DA, DA, HA), bf16),
            pltpu.VMEM((D, D), bf16),
            pltpu.VMEM((MEM, D), bf16),
            pltpu.VMEM((S + SEG, D), f32),
            pltpu.VMEM((S // 2, D), u32),
            pltpu.VMEM((SEG, D), f32),
            pltpu.VMEM((SEG, D), f32),
            pltpu.VMEM((SEG, D), f32),
            pltpu.VMEM((SEG, D), f32),
            pltpu.VMEM((S // 2, D), u32),
            pltpu.VMEM((3, GA, 80, D), u32),
            pltpu.VMEM((D // 2, D), u32),
            pltpu.VMEM((2, GA, 160, 256), f32),
            pltpu.VMEM((NCH, NPA, RA, TC), u32),
            pltpu.VMEM((NPA, RA + 8, 2 * RA), f32),
            pltpu.VMEM((NPA, (RA + 8) // 2, 2 * RA), u32),
            pltpu.VMEM((4, HD + 64, D), bf16),
            pltpu.VMEM((3, NPB + 2, D // 2, PW), u32),
            pltpu.VMEM(((HD + TRC) // 2, D), u32),
            pltpu.VMEM((L, HD), f32),
            pltpu.SemaphoreType.DMA((20 + 4 * NTR,)),
        ],
        compiler_params=pltpu.CompilerParams(vmem_limit_bytes=120 * 1024 * 1024, disable_bounds_checks=True,
                                             disable_semaphore_checks=True),
    )(x, A_wqkv, phi, A_wo, B_mem0.reshape(MEM, D), wqt, wkt, wvt, wo)
    return out.reshape(1, S, D)
```
